```python
import jax
import jax.numpy as jnp

def _softmax(x, axis=-1):
    return jax.nn.softmax(x, axis=axis)

def _gelu(x):
    return jax.nn.gelu(x, approximate=True)

def _silu(x):
    return jax.nn.silu(x)

def _sigmoid(x):
    return jax.nn.sigmoid(x)

def _layernorm(x, axis=-1, eps=1e-05):
    m = jnp.mean(x, axis=axis, keepdims=True)
    v = jnp.var(x, axis=axis, keepdims=True)
    return (x - m) / jnp.sqrt(v + eps)

def _scatter_add(tgt, idx, src, axis=0):
    return tgt.at[idx].add(src)

def _segment_sum(src, seg, n):
    return jax.ops.segment_sum(src, seg, n)

class _Rng:

    def __init__(self, key):
        self._k = key

    def _next(self):
        self._k, sub = jax.random.split(self._k)
        return sub

    def normal(self, shape):
        return jax.random.normal(self._next(), shape, dtype=jnp.bfloat16)

    def randint(self, lo, hi, shape):
        return jax.random.randint(self._next(), shape, lo, hi, dtype=jnp.int32)

    def uniform(self, shape, lo=0.0, hi=1.0):
        return jax.random.uniform(self._next(), shape, jnp.bfloat16, lo, hi)

    def permutation(self, n):
        return jax.random.permutation(self._next(), n)
kernel_name = 'concat_heads__ssm_conv_h3__memory_aug_infini_attn__prompt'

def setup_inputs():
    _rng = _Rng(jax.random.key(int.from_bytes(__import__("os").urandom(4), "little")))
    _w = lambda a: (lambda t: t.astype(jnp.bfloat16) if jnp.issubdtype(t.dtype, jnp.floating) else t)(jnp.asarray(a))

    def _A_setup():
        B, S, D = (1, 2048, 640)
        ks = 4
        return {'q': _w((lambda *s: _rng.normal(s) * 0.05)(B, S, D)), 'k': _w((lambda *s: _rng.normal(s) * 0.05)(B, S, D)), 'v': _w((lambda *s: _rng.normal(s) * 0.05)(B, S, D)), 'shift_k': _w((lambda *s: _rng.normal(s) * 0.05)(D, ks) * 0.5), 'ssm_k': _w((lambda *s: _rng.normal(s) * 0.05)(D, S) * (1.0 / S ** 0.5)), 'ssm_D': _w((lambda *s: _rng.normal(s) * 0.05)(D))}
    _A_in = _A_setup()

    def _B_setup():
        B, S, D, H = (1, 2048, 640, 32)
        N = 4
        L = max(1, S // N)
        sc = D ** (-0.5)
        return {'x': _w((lambda *s: _rng.normal(s) * 0.05)(B, N * L, D)), 'wq': _w((lambda *s: _rng.normal(s) * 0.05)(D, D) * sc), 'wk': _w((lambda *s: _rng.normal(s) * 0.05)(D, D) * sc), 'wv': _w((lambda *s: _rng.normal(s) * 0.05)(D, D) * sc), 'wo': _w((lambda *s: _rng.normal(s) * 0.05)(D, D) * sc), 'beta': _w((lambda *s: _rng.normal(s) * 0.05)(H))}
    _B_in = _B_setup()
    return {'A_q': _A_in['q'], 'A_k': _A_in['k'], 'A_v': _A_in['v'], 'A_shift_k': _A_in['shift_k'], 'A_ssm_k': _A_in['ssm_k'], 'A_ssm_D': _A_in['ssm_D'], 'B_x': _B_in['x'], 'B_wq': _B_in['wq'], 'B_wk': _B_in['wk'], 'B_wv': _B_in['wv'], 'B_wo': _B_in['wo'], 'B_beta': _B_in['beta']}

def reference(A_q, A_k, A_v, A_shift_k, A_ssm_k, A_ssm_D, B_x, B_wq, B_wk, B_wv, B_wo, B_beta):

    def _A_ref(q, k, v, shift_k, ssm_k, ssm_D):
        B, S, D = q.shape
        ks = shift_k.shape[-1]
        k_pad = jnp.pad(k, ((0, 0), (ks - 1, 0), (0, 0)))
        k_shift = jnp.zeros_like(k)
        for t in range(ks):
            k_shift = k_shift + k_pad[:, t:t + S, :] * shift_k[:, ks - 1 - t][None, None, :]
        kv = k_shift * v
        L = 2 * S
        kv_pad = jnp.pad(kv, ((0, 0), (0, S), (0, 0)))
        kf_pad = jnp.pad(ssm_k, ((0, 0), (0, S)))
        kv_f = (lambda x, axes=(-2, -1): jnp.fft.rfft2(x.astype(jnp.float32), axes=axes))(kv_pad[:, None, :, :], axes=(1, 2))
        kf_f = (lambda x, axes=(-2, -1): jnp.fft.rfft2(x.astype(jnp.float32), axes=axes))(kf_pad[:, None, :], axes=(1, 2))
        kf_f = (lambda x, *d: x.transpose(*d))(kf_f, 1, 2, 0)
        y_f = kv_f * kf_f[None, :, :, :]
        y = (lambda x, s, axes=(-2, -1): jnp.fft.irfft2(x, s=s, axes=axes).astype(jnp.bfloat16))(y_f, (1, L), axes=(1, 2))[:, 0, :S, :]
        y = y + kv * ssm_D[None, None, :]
        return q * y

    def _B_ref(x, wq, wk, wv, wo, beta):
        B, S, D = x.shape
        H = 32
        Dh = D // H
        N = 4
        L = S // N
        q = (lambda x, *d: x.transpose(*d))((x @ wq).reshape(B, S, H, Dh), 0, 2, 1, 3).reshape(B, H, N, L, Dh)
        k = (lambda x, *d: x.transpose(*d))((x @ wk).reshape(B, S, H, Dh), 0, 2, 1, 3).reshape(B, H, N, L, Dh)
        v = (lambda x, *d: x.transpose(*d))((x @ wv).reshape(B, S, H, Dh), 0, 2, 1, 3).reshape(B, H, N, L, Dh)
        phi = lambda t: jnp.where(t > 0, t + 1.0, jnp.exp(t))
        scale = Dh ** (-0.5)
        ar = jnp.arange(L)
        mask = (lambda x, dt: x.astype(dt))(ar[:, None] < ar[None, :], x.dtype) * -1000000000.0
        g = _sigmoid(beta).reshape(1, H, 1, 1)
        M = jnp.einsum('bhd,bhe->bhde', q[:, :, 0, 0, :] * 0.0, q[:, :, 0, 0, :] * 0.0)
        z = q[:, :, 0, 0, :] * 0.0
        outs = []
        for s in range(N):
            qs, ks, vs = (q[:, :, s].copy(), k[:, :, s].copy(), v[:, :, s].copy())
            logits = jnp.einsum('bhqd,bhkd->bhqk', qs, ks) * scale + mask
            p = _softmax(logits, axis=-1)
            a_dot = jnp.einsum('bhqk,bhkd->bhqd', p, vs)
            pq = phi(qs)
            num = jnp.einsum('bhld,bhde->bhle', pq, M)
            den = jnp.einsum('bhld,bhd->bhl', pq, z)[..., None] + 1e-06
            a_mem = num / den
            o = g * a_mem + (1.0 - g) * a_dot
            outs.append(o)
            pk = phi(ks)
            M = M + jnp.einsum('bhld,bhle->bhde', pk, vs)
            z = z + jnp.einsum('bhld->bhd', pk)
        o = (lambda x, *d: x.transpose(*d))(jnp.stack(outs, 2).reshape(B, H, S, Dh), 0, 2, 1, 3).reshape(B, S, D)
        return o @ wo
    a = _A_ref(A_q, A_k, A_v, A_shift_k, A_ssm_k, A_ssm_D)
    b = _B_ref(B_x, B_wq, B_wk, B_wv, B_wo, B_beta)
    return jnp.concatenate([a, b], axis=-1)
```

```python
import math

import jax
import jax.numpy as jnp
import ml_dtypes
import numpy as np
from jax import lax
from jax.experimental import pallas as pl
from jax.experimental.pallas import tpu as pltpu

S = 2048
D = 640
NT = D // 128
DH = 20
NG = 8
SEG = 512
M1, M2 = 32, 64

bf16 = jnp.bfloat16
f32 = jnp.float32
u32 = jnp.uint32
i32 = jnp.int32

LOG2E = math.log2(math.e)


def _neg(a):
    return None if a is None else (-a[0], a[1])


def _add(a, b):
    if a is None:
        return b
    if b is None:
        return a
    if a[0] == b[0]:
        return (a[0], a[1] + b[1])
    if a[0] > 0:
        return (1, a[1] - b[1])
    return (1, b[1] - a[1])


def _sub(a, b):
    return _add(a, _neg(b))


def _scale(a, c):
    if a is None or abs(c) < 1e-12:
        return None
    if abs(abs(c) - 1.0) < 1e-12:
        return a if c > 0 else _neg(a)
    return (a[0], a[1] * float(c))


def _cmul(z, ang):
    c, s = math.cos(ang), math.sin(ang)
    x, y = z
    if x is not None and y is not None and abs(abs(c) - abs(s)) < 1e-12:
        r = 1.0 if c * s > 0 else -1.0
        if r > 0:
            return (_scale(_sub(x, y), c), _scale(_add(y, x), c))
        return (_scale(_add(x, y), c), _scale(_sub(y, x), c))
    return (_sub(_scale(x, c), _scale(y, s)), _add(_scale(y, c), _scale(x, s)))


def _cadd(a, b):
    return (_add(a[0], b[0]), _add(a[1], b[1]))


def _csub(a, b):
    return (_sub(a[0], b[0]), _sub(a[1], b[1]))


def _fft_dif(z):
    n = len(z)
    if n == 1:
        return list(z)
    if n == 2:
        return [_cadd(z[0], z[1]), _csub(z[0], z[1])]
    q = n // 4
    u, v1, v3 = [None] * (2 * q), [], []
    for j in range(q):
        a, b, c, d = z[j], z[j + q], z[j + 2 * q], z[j + 3 * q]
        u[j], u[j + q] = _cadd(a, c), _cadd(b, d)
        t1, t2 = _csub(a, c), _csub(b, d)
        mi_t2 = (t2[1], _neg(t2[0]))
        v1.append(_cmul(_cadd(t1, mi_t2), -2 * math.pi * j / n))
        v3.append(_cmul(_csub(t1, mi_t2), -6 * math.pi * j / n))
    out = [None] * n
    out[0::2] = _fft_dif(u)
    out[1::4] = _fft_dif(v1)
    out[3::4] = _fft_dif(v3)
    return out


def _ifft_dit(z):
    n = len(z)
    if n == 1:
        return list(z)
    if n == 2:
        return [_cadd(z[0], z[1]), _csub(z[0], z[1])]
    q = n // 4
    e, o1, o3 = _ifft_dit(z[0::2]), _ifft_dit(z[1::4]), _ifft_dit(z[3::4])
    out = [None] * n
    for j in range(q):
        a = _cmul(o1[j], 2 * math.pi * j / n)
        b = _cmul(o3[j], 6 * math.pi * j / n)
        s, d = _cadd(a, b), _csub(a, b)
        i_d = (_neg(d[1]), d[0])
        out[j], out[j + 2 * q] = _cadd(e[j], s), _csub(e[j], s)
        out[j + q], out[j + 3 * q] = _cadd(e[j + q], i_d), _csub(e[j + q], i_d)
    return out


def _stage1_fwd(xs):
    z = [_cmul(((1, x), None), -2 * math.pi * n / (4 * M1)) for n, x in enumerate(xs)]
    return _fft_dif(z)


def _stage1_inv(us):
    z = _ifft_dit([((1, re), (1, im)) for re, im in us])
    return [_cmul(w, 2 * math.pi * n / (4 * M1))[0] for n, w in enumerate(z)]


def _pack_rows(m):
    b = np.asarray(m, np.float32).astype(ml_dtypes.bfloat16).view(np.uint16).astype(np.uint32)
    return np.ascontiguousarray(b[..., 0::2, :] | (b[..., 1::2, :] << 16))


def _dft_tables():
    signs = [(re[0], im[0]) for re, im in _stage1_fwd([1.0] * M1)]
    r = np.arange(128)
    part = (r // 8) % 2
    nat = 8 * (r // 16) + r % 8
    eo = 16 * (r // 32) + 2 * (r % 8) + (r // 16) % 2
    fwd = np.zeros((M1, 128, 128))
    inv = np.zeros((M1, 128, 128))
    for k1 in range(M1):
        freq = k1 + M1 * nat + 0.25
        ph = 2 * np.pi * freq[:, None] * eo[None, :] / S
        same = part[:, None] == part[None, :]
        cross = np.where(part[:, None] == 0, 1.0, -1.0)
        sg = np.where(part == 0, signs[k1][0], signs[k1][1])
        fwd[k1] = np.where(same, np.cos(ph), cross * np.sin(ph)) * sg[None, :]
        ph = 2 * np.pi * nat[:, None] * freq[None, :] / S
        inv[k1] = np.where(same, np.cos(ph), -cross * np.sin(ph)) / S
    return _pack_rows(fwd), _pack_rows(inv)


_G_FWD, _G_INV = _dft_tables()
_INV_SIGNS = [y[0] for y in _stage1_inv([(1.0, 1.0)] * M1)]


def _pk(x):
    return pltpu.bitcast(x, u32)


def _upk(x):
    return pltpu.bitcast(x, bf16)


def _even(x):
    return pltpu.bitcast(x << 16, f32)


def _odd(x):
    return pltpu.bitcast(x & jnp.uint32(0xFFFF0000), f32)


def _dot(a, b):
    return jnp.dot(a, b, preferred_element_type=f32)


def _dot_t(a, b):
    return lax.dot_general(a, b, (((1,), (1,)), ((), ())), preferred_element_type=f32)


def _phi(t):
    return jnp.where(t > 0, t + 1.0, jnp.exp2(t * LOG2E))


def _recip(x):
    r = pltpu.reciprocal(x, approx=True)
    return r * (2.0 - x * r)


def _ds(start, size, align=8):
    return pl.ds(pl.multiple_of(start, align), size)


def _kernel(
    q_hbm, k_hbm, v_hbm, shift_ref, h_hbm, d_ref,
    x_hbm, wq_hbm, wk_hbm, wv_hbm, wo_hbm, beta_ref, gf_hbm, gi_hbm,
    out_hbm,
    x_b, wq_b, wk_b, wv_b, wo_b, k_b, v_b, h_b, q_b, gf_v, gi_v, oa_b, ob_b,
    wt_v, ht_v, kv_v, par_v, yx_v, yh_v, ua_v, ub_v,
    kt_v, kg_v, qt_v, pqt_v, vt_v, ot_v, on_a, on_b,
    sa_v, ma_v, sb_v, mb_v, mem_v, gate_v, zero_s, sems,
):
    x_v, wq_v, wk_v, wv_v, wo_v = (r.bitcast(u32) for r in (x_b, wq_b, wk_b, wv_b, wo_b))
    k_v, v_v, h_v, q_v, oa_v, ob_v = (r.bitcast(u32) for r in (k_b, v_b, h_b, q_b, oa_b, ob_b))

    n_sem = [0]

    def group(pairs):
        sem = sems.at[n_sem[0]]
        n_sem[0] += 1
        return [pltpu.make_async_copy(src, dst, sem) for src, dst in pairs]

    def cols(t):
        return pl.ds(128 * t, 128)

    def weight(hbm, buf):
        return group([(hbm.at[:, cols(t)], buf.at[t]) for t in range(NT)])

    def xrows(r0, n):
        return group([(x_hbm.at[pl.ds(r0, n), cols(t)], x_b.at[t, pl.ds(r0, n)]) for t in range(NT)])

    c_wk, c_wq, c_wv, c_wo = (weight(a, b) for a, b in
                              ((wk_hbm, wk_b), (wq_hbm, wq_b), (wv_hbm, wv_b), (wo_hbm, wo_b)))
    c_x = [xrows(0, 512), xrows(512, 768), xrows(1280, 768)]
    c_h = [group([(h_hbm.at[cols(t)], h_b.at[t])]) for t in range(NT)]
    c_kv = [group([(k_hbm.at[:, cols(t)], k_b.at[t, pl.ds(16, S)]),
                   (v_hbm.at[:, cols(t)], v_b.at[t])]) for t in range(NT)]
    c_g = group([(gf_hbm, gf_v), (gi_hbm, gi_v)])
    c_q = group([(q_hbm.at[:, cols(t)], q_b.at[t]) for t in range(NT)])
    c_oa = [group([(oa_b.at[t], out_hbm.at[:, cols(t)])]) for t in range(NT)]
    c_ob = [group([(ob_b.at[t, pl.ds(SEG * s, SEG)], out_hbm.at[pl.ds(SEG * s, SEG), cols(NT + t)])
                   for t in range(NT)]) for s in range(S // SEG)]

    def start(cs):
        for c in cs:
            c.start()

    def wait(cs):
        for c in cs:
            c.wait()

    def wait_when(cond, cs):
        pl.when(cond)(lambda: wait(cs))

    for cs in (c_wq, c_wv, c_wk, c_x[0], c_h[0], c_x[1], c_kv[0], c_h[1], c_kv[1], c_h[2], c_x[2],
               c_kv[2], c_h[3], c_kv[3], c_h[4], c_kv[4], c_g, c_q, c_wo):
        start(cs)

    sub8 = lax.broadcasted_iota(i32, (8, 128), 0)
    lane8 = lax.broadcasted_iota(i32, (8, 128), 1)

    zero_s[0] = 0
    zero_s[1] = 0
    taps = shift_ref[...].astype(f32)
    skip = d_ref[...].astype(f32).reshape(1, D)
    for t in range(NT):
        for j in range(4):
            par_v[t, j] = jnp.broadcast_to(taps[j:j + 1, 128 * t:128 * t + 128], (8, 128))
        par_v[t, 4] = jnp.where(sub8 == 0, skip[:, 128 * t:128 * t + 128], 0.0)
        k_v[t, 0:8, :] = jnp.zeros((8, 128), u32)
    beta = beta_ref[...].astype(f32).reshape(1, 4 * NG)
    gate = 1.0 / (1.0 + jnp.exp(-beta))
    for h in range(4 * NG):
        gate_v[h] = jnp.broadcast_to(gate[:, h:h + 1], (8, 128))

    wait(c_wq)
    wait(c_wv)
    for ft in range(NT):
        for kt in range(NT):
            wt_v[ft, kt, 0:64, :] = _pk(_upk(wq_v[ft, 64 * kt:64 * kt + 64, :]).T)
            wt_v[ft, kt, 64:128, :] = _pk(_upk(wv_v[ft, 64 * kt:64 * kt + 64, :]).T)

    q_scale = DH ** -0.5 * LOG2E

    def project(tile0, ntiles, ft):
        wt = _upk(jnp.concatenate([wt_v[ft, kt] for kt in range(NT)], axis=1))
        wk = _upk(wk_v[ft])
        rows = _ds(ft * 64, 64)
        for j in range(ntiles):
            tok = _ds((tile0 + j) * 64, 64)
            xt = _upk(jnp.concatenate([x_v[kt, tok, :] for kt in range(NT)], axis=1))
            qv = _dot_t(wt, xt)
            qt_v[tile0 + j, rows, :] = _pk((qv[:128] * q_scale).astype(bf16))
            pqt_v[tile0 + j, rows, :] = _pk(_phi(qv[:128]).astype(bf16))
            vt_v[tile0 + j, rows, :] = _pk(qv[128:].astype(bf16))
            kt_v[ft, tok, :] = _pk(_dot(xt, wk).astype(bf16))

    def transpose_filter(ct, t0, n):
        for t in range(n):
            blk = h_v[ct, :, _ds((t0 + t) * 128, 128, 128)]
            ht_v[ct, _ds((t0 + t) * 64, 64), :] = _pk(_upk(blk).T)

    def forward_unit(ct, bb):
        r0 = pl.multiple_of(bb * 8, 8)
        w = [par_v[ct, j] for j in range(4)]
        for n1 in range(M1):
            base = r0 + 32 * n1
            p0, p1, p2 = (k_v[ct, pl.ds(base + 8 - j, 8), :] for j in range(3))
            e0, o0, e1, o1, o2 = _even(p0), _odd(p0), _even(p1), _odd(p1), _odd(p2)
            vv = v_v[ct, _ds(base, 8), :]
            kv_v[0, n1] = (w[0] * e0 + w[1] * o1 + w[2] * e1 + w[3] * o2) * _even(vv)
            kv_v[1, n1] = (w[0] * o0 + w[1] * e0 + w[2] * o1 + w[3] * e1) * _odd(vv)

        def emit(dst, par, xs):
            for k1, (re, im) in enumerate(_stage1_fwd(xs)):
                y = jnp.concatenate([re[1], im[1]], axis=0).astype(bf16)
                dst[ct, k1, _ds(bb * 16 + 8 * par, 8), :] = _pk(y)

        for par in range(2):
            unpack = _odd if par else _even
            hs = [unpack(ht_v[ct, _ds(r0 + 32 * n1, 8), :]) for n1 in range(M1)]
            if par == 0:
                hs[0] = hs[0] + jnp.where(bb == 0, par_v[ct, 4], 0.0)
            emit(yh_v, par, hs)
        for par in range(2):
            emit(yx_v, par, [kv_v[par, n1] for n1 in range(M1)])

    wait(c_wk)
    wait(c_x[0])
    wait(c_h[0])

    def phase1a(ft, c):
        project(0, 4, ft)
        return c

    lax.fori_loop(0, NT, phase1a, 0)
    transpose_filter(0, 0, 16)

    def phase1b(i, c):
        wait_when(i == 0, c_x[1])
        wait_when(i == NT, c_x[2])
        for ct in range(NT):
            wait_when(i == 2 * ct, c_kv[ct] + (c_h[ct + 1] if ct + 1 < NT else []))
        ct = i // 2
        project(4 + 6 * (i // NT), 6, i % NT)
        for u in range(2):
            forward_unit(ct, 2 * (i % 2) + u)
        transpose_filter(jnp.minimum(ct + 1, NT - 1), 8 * (i % 2), 8)
        return c

    lax.fori_loop(0, 2 * NT, phase1b, 0)

    def spectral(ct, u_out, z):
        def fwd(k1):
            g = _upk(gf_v[k1])
            x = _dot(g, _upk(yx_v[ct, k1]))
            h = _dot(g, _upk(yh_v[ct, k1]))
            rows = []
            for a in range(8):
                xr, xi = x[16 * a:16 * a + 8], x[16 * a + 8:16 * a + 16]
                hr, hi = h[16 * a:16 * a + 8], h[16 * a + 8:16 * a + 16]
                rows += [xr * hr - xi * hi, xr * hi + xi * hr]
            return jnp.concatenate(rows, axis=0).astype(bf16)

        zs = {}
        for k1 in range(M1 + 4):
            if k1 < M1:
                zs[k1] = fwd(k1)
            if k1 >= 4:
                u_out[z, k1 - 4] = _dot(_upk(gi_v[k1 - 4]), zs.pop(k1 - 4))

    def inverse(ct, u_in, z):
        for bb in range(4):
            halves = []
            for a in (2 * bb, 2 * bb + 1):
                us = [(u_in[z, k1, 16 * a:16 * a + 8, :], u_in[z, k1, 16 * a + 8:16 * a + 16, :])
                      for k1 in range(M1)]
                halves.append([y[1] for y in _stage1_inv(us)])
            for n1 in range(M1):
                rows = pl.ds(32 * n1 + 8 * bb, 8)
                y = jnp.concatenate([halves[0][n1], halves[1][n1]], axis=0)
                y = y * _upk(q_v[ct, rows, :]).astype(f32)
                if _INV_SIGNS[n1] < 0:
                    y = -y
                oa_v[ct, rows, :] = _pk(y.astype(bf16))

    def align_keys(r0, n):
        rows = _ds(r0, n)
        lane = lax.broadcasted_iota(i32, (n, 128), 1)
        for g in range(NG):
            t, off = divmod(80 * g, 128)
            x = kt_v[t, rows, :]
            if off > 48:
                x = jnp.where(lane >= off, x, kt_v[t + 1, rows, :])
            kg_v[g, rows, :] = pltpu.roll(x, 128 - off, 1) if off else x

    wait(c_g)
    z0, z1 = zero_s[0], zero_s[1]
    spectral(0, ua_v, z0)
    align_keys(0, 256)
    wait(c_q)

    def phase2(i, c):
        z0, z1 = zero_s[0], zero_s[1]

        @pl.when(i > 0)
        def _():
            start(c_oa[0])

        spectral(2 * i + 1, ub_v, z0)
        inverse(2 * i, ua_v, z1)
        spectral(2 * i + 2, ua_v, z0)
        inverse(2 * i + 1, ub_v, z1)
        align_keys(256 + 384 * i, 384)
        return c

    lax.fori_loop(0, 2, phase2, 0)
    for t in range(1, 4):
        start(c_oa[t])

    prow = lax.broadcasted_iota(i32, (16, 128), 0)
    base = {3: 0, 2: 4, 1: 7, 0: 9}
    steps = [(j, t) for j in (3, 2, 1, 0) for t in range(j + 1)]

    def attend(uq, s_out, m_out, zo, up, s_in, m_in, zi, memory):
        ri = lax.broadcasted_iota(i32, (128, 128), 0)
        ci = lax.broadcasted_iota(i32, (128, 128), 1)
        bias = jnp.where(ri <= ci, 0.0, -1e9 * LOG2E).astype(f32)
        if uq is not None:
            sq, gq = uq // NG, uq % NG
        if up is not None:
            sp, gp = up // NG, up % NG
            gates = [gate_v[4 * gp + i] for i in range(4)]
        weights, run_max, acc = {}, {}, {}

        def q_weights(j):
            if j not in weights:
                ws = []
                for i in range(4):
                    own = (prow >= 2 * i) & (prow < 2 * i + 10)
                    qw = jnp.where(own, qt_v[4 * sq + j, _ds(40 * gq + 8 * i, 16), :], jnp.uint32(0))
                    parts = [jnp.zeros((8 * i, 128), u32)] if i else []
                    ws.append(jnp.concatenate(parts + [qw, jnp.zeros((48 - 8 * i, 128), u32)], axis=0))
                weights[j] = _upk(jnp.concatenate(ws, axis=1))
            return weights[j]

        def v_rows(i, t):
            free = prow >= 12 if i < 2 else prow < 4
            return _upk(jnp.where(free, jnp.uint32(0x3F803F80), vt_v[4 * sp + t, _ds(40 * gp + 8 * i, 16), :]))

        if memory:
            prev = 4 * (sp - 1)
            upd = None
            for t in range(4):
                pk_t = _phi(_upk(kg_v[gp, _ds((prev + t) * 64, 64), :]).astype(f32)).astype(bf16)
                lhs = jnp.concatenate([vt_v[prev + t, _ds(40 * gp, 40), :],
                                       jnp.full((8, 128), 0x3F803F80, u32)], axis=0)
                d = _dot(_upk(lhs), pk_t)
                upd = d if upd is None else upd + d
            m = mem_v[gp] + upd[:88]
            mem_v[gp] = m
            own = [(lane8 >= DH * i) & (lane8 < DH * i + DH) for i in range(4)]
            rows = []
            for r in range(10):
                lo, hi = (8 * r) // DH, (8 * r + 7) // DH
                blk = m[8 * r:8 * r + 8]
                a = jnp.where(own[lo], blk * gates[lo], 0.0)
                if hi != lo:
                    a = jnp.where(sub8 < 4, a, jnp.where(own[hi], blk * gates[hi], 0.0))
                rows.append(a)
            rows += [jnp.where(own[i], m[80:88], 0.0) for i in range(4)]
            mem_lhs = jnp.concatenate(rows, axis=0).astype(bf16)

        def memory_read(j):
            w = jnp.concatenate([pqt_v[4 * sp + j, _ds(40 * gp, 40), :], jnp.zeros((24, 128), u32)], axis=0)
            r = _dot(mem_lhs, _upk(w))
            inv = [_recip(r[80 + 8 * i:88 + 8 * i] + 1e-6) for i in range(4)]
            rows = []
            for b in range(10):
                lo, hi = (8 * b) // DH, (8 * b + 7) // DH
                rows.append(r[8 * b:8 * b + 8] * (inv[lo] if lo == hi else jnp.where(sub8 < 4, inv[lo], inv[hi])))
            return rows

        def finish(j):
            a = []
            for i in range(4):
                o = acc[(j, i)]
                r = _recip(o[24:32] if i < 2 else o[0:8]) * (1.0 - gates[i])
                a.append([o[8 * b:8 * b + 8] * r for b in range(4)])
            low = sub8 < 4
            rows = [a[0][0], a[0][1], jnp.where(low, a[0][2], a[1][0]), a[1][1], a[1][2],
                    a[2][1], a[2][2], jnp.where(low, a[2][3], a[3][1]), a[3][2], a[3][3]]
            if memory:
                rows = [x + y for x, y in zip(rows, memory_read(j))]
            ot_v[4 * sp + j, _ds(40 * gp, 40), :] = _pk(jnp.concatenate(rows, axis=0).astype(bf16))

        for j, t in steps:
            if uq is not None:
                keys = _upk(kg_v[gq, _ds(256 * sq + 64 * t, 64), :])
                logits = _dot(keys, q_weights(j))
            if up is not None:
                ps = [jnp.exp2(s_in[zi, i, base[j] + t].reshape(16, 8, 128) - m_in[zi, j, i][None])
                      .reshape(128, 128).astype(bf16) for i in range(4)]
            if uq is not None:
                for i in range(4):
                    st = logits[:, 128 * i:128 * i + 128]
                    if t == j:
                        st = st + bias
                    s_out[zo, i, base[j] + t] = st
                    mx = jnp.max(st.reshape(16, 8, 128), axis=0)
                    run_max[(j, i)] = mx if t == 0 else jnp.maximum(run_max[(j, i)], mx)
                    if t == j:
                        m_out[zo, j, i] = jnp.broadcast_to(
                            jnp.max(run_max[(j, i)], axis=0, keepdims=True), (8, 128))
            if up is not None:
                for i in range(4):
                    d = _dot(v_rows(i, t), ps[i])
                    acc[(j, i)] = d if t == 0 else acc[(j, i)] + d
                if t == j:
                    finish(j)

    mem_v[...] = jnp.zeros(mem_v.shape, f32)
    z0, z1 = zero_s[0], zero_s[1]
    attend(0, sa_v, ma_v, z0, None, None, None, None, False)
    inverse(NT - 1, ua_v, z1)
    start(c_oa[NT - 1])

    def attend_pair(memory, last=False):
        def body(i, c):
            z0, z1 = zero_s[0], zero_s[1]
            attend(2 * i + 1, sb_v, mb_v, z0, 2 * i, sa_v, ma_v, z1, memory)
            attend(None if last else 2 * i + 2, sa_v, ma_v, z0, 2 * i + 1, sb_v, mb_v, z1, memory)
            return c
        return body

    lax.fori_loop(0, 4, attend_pair(False), 0)
    lax.fori_loop(4, 15, attend_pair(True), 0)
    attend_pair(True, last=True)(15, 0)

    def transpose_heads(s, dst, z):
        for j in range(4):
            for ft in range(NT):
                dst[z, ft, 64 * j:64 * j + 64, :] = _pk(_upk(ot_v[4 * s + j, 64 * ft:64 * ft + 64, :]).T)

    def out_project(s, src, z):
        lhs = _upk(jnp.concatenate([src[z, ft] for ft in range(NT)], axis=1))
        for nt in range(NT):
            ob_v[nt, _ds(256 * s, 256), :] = _pk(_dot(lhs, _upk(wo_v[nt])).astype(bf16))

    wait(c_wo)
    z0, z1 = zero_s[0], zero_s[1]
    transpose_heads(0, on_a, z0)
    for s in range(S // SEG):
        src, dst = (on_a, on_b) if s % 2 == 0 else (on_b, on_a)
        if s + 1 < S // SEG:
            transpose_heads(s + 1, dst, z0)
        out_project(s, src, z1)
        start(c_ob[s])
    for cs in c_oa + c_ob:
        wait(cs)


@jax.jit
def pallas_concat_heads__ssm_conv_h3__memory_aug_infini_attn__prompt_kernel(
    A_q: jax.Array,
    A_k: jax.Array,
    A_v: jax.Array,
    A_shift_k: jax.Array,
    A_ssm_k: jax.Array,
    A_ssm_D: jax.Array,
    B_x: jax.Array,
    B_wq: jax.Array,
    B_wk: jax.Array,
    B_wv: jax.Array,
    B_wo: jax.Array,
    B_beta: jax.Array,
):
    hbm = pl.BlockSpec(memory_space=pl.ANY)
    vmem = pl.BlockSpec(memory_space=pltpu.VMEM)
    V = pltpu.VMEM
    scratch = [
        V((NT, S, 128), bf16),
        V((NT, D, 128), bf16), V((NT, D, 128), bf16),
        V((NT, D, 128), bf16), V((NT, D, 128), bf16),
        V((NT, S + 16, 128), bf16), V((NT, S, 128), bf16),
        V((NT, 128, S), bf16), V((NT, S, 128), bf16),
        V((M1, 64, 128), u32), V((M1, 64, 128), u32),
        V((NT, S, 128), bf16), V((NT, S, 128), bf16),
        V((NT, NT, 128, 128), u32),
        V((NT, S // 2, 128), u32),
        V((2, M1, 8, 128), f32),
        V((NT, 5, 8, 128), f32),
        V((NT, M1, 64, 128), u32), V((NT, M1, 64, 128), u32),
        V((1, M1, 128, 128), f32), V((1, M1, 128, 128), f32),
        V((NT, S // 2, 128), u32), V((NG, S // 2, 128), u32),
        V((16, D // 2, 128), u32), V((16, D // 2, 128), u32),
        V((16, D // 2, 128), u32), V((16, D // 2, 128), u32),
        V((1, NT, SEG // 2, 128), u32), V((1, NT, SEG // 2, 128), u32),
        V((1, 4, 10, 128, 128), f32), V((1, 4, 4, 8, 128), f32),
        V((1, 4, 10, 128, 128), f32), V((1, 4, 4, 8, 128), f32),
        V((NG, 88, 128), f32),
        V((4 * NG, 8, 128), f32),
        pltpu.SMEM((2,), i32),
        pltpu.SemaphoreType.DMA((32,)),
    ]
    out = pl.pallas_call(
        _kernel,
        out_shape=jax.ShapeDtypeStruct((S, 2 * D), bf16),
        in_specs=[hbm, hbm, hbm, vmem, hbm, vmem, hbm, hbm, hbm, hbm, hbm, vmem, hbm, hbm],
        out_specs=hbm,
        scratch_shapes=scratch,
        compiler_params=pltpu.CompilerParams(vmem_limit_bytes=110 * 2**20),
    )(
        A_q.reshape(S, D), A_k.reshape(S, D), A_v.reshape(S, D), A_shift_k.T, A_ssm_k, A_ssm_D,
        B_x.reshape(S, D), B_wq, B_wk, B_wv, B_wo, B_beta, _G_FWD, _G_INV,
    )
    return out.reshape(1, S, 2 * D)
```

```python
import functools
import math

import jax
import jax.numpy as jnp
import ml_dtypes
import numpy as np
from jax import lax
from jax.experimental import pallas as pl
from jax.experimental.pallas import tpu as pltpu

S = 2048
D = 640
NT = D // 128
DH = 20
NG = 8
SEG = 512
M1, M2 = 32, 64

bf16 = jnp.bfloat16
f32 = jnp.float32
u32 = jnp.uint32
i32 = jnp.int32

LOG2E = math.log2(math.e)
PACE1 = 2
PACE2 = 4
LEAD1 = 4
FREE1 = 600
LEAD2 = 4
FREE2 = 400
TAIL2 = 4
MID2 = 8
LOOK2 = 3
LAG1 = 3
LAG2 = 0


def _neg(a):
    return None if a is None else (-a[0], a[1])


def _add(a, b):
    if a is None:
        return b
    if b is None:
        return a
    if a[0] == b[0]:
        return (a[0], a[1] + b[1])
    if a[0] > 0:
        return (1, a[1] - b[1])
    return (1, b[1] - a[1])


def _sub(a, b):
    return _add(a, _neg(b))


def _scale(a, c):
    if a is None or abs(c) < 1e-12:
        return None
    if abs(abs(c) - 1.0) < 1e-12:
        return a if c > 0 else _neg(a)
    return (a[0], a[1] * float(c))


def _cmul(z, ang):
    c, s = math.cos(ang), math.sin(ang)
    x, y = z
    if x is not None and y is not None and abs(abs(c) - abs(s)) < 1e-12:
        r = 1.0 if c * s > 0 else -1.0
        if r > 0:
            return (_scale(_sub(x, y), c), _scale(_add(y, x), c))
        return (_scale(_add(x, y), c), _scale(_sub(y, x), c))
    return (_sub(_scale(x, c), _scale(y, s)), _add(_scale(y, c), _scale(x, s)))


def _cadd(a, b):
    return (_add(a[0], b[0]), _add(a[1], b[1]))


def _csub(a, b):
    return (_sub(a[0], b[0]), _sub(a[1], b[1]))


def _dif_step(a, b, c, d, j, n):
    t1, t2 = _csub(a, c), _csub(b, d)
    mi_t2 = (t2[1], _neg(t2[0]))
    return (_cadd(a, c), _cadd(b, d),
            _cmul(_cadd(t1, mi_t2), -2 * math.pi * j / n),
            _cmul(_csub(t1, mi_t2), -6 * math.pi * j / n))


def _dit_step(e0, e1, o1, o3, j, n):
    a, b = _cmul(o1, 2 * math.pi * j / n), _cmul(o3, 6 * math.pi * j / n)
    s, d = _cadd(a, b), _csub(a, b)
    i_d = (_neg(d[1]), d[0])
    return _cadd(e0, s), _cadd(e1, i_d), _csub(e0, s), _csub(e1, i_d)


def _fft(z):
    n = len(z)
    if n == 1:
        return list(z)
    if n == 2:
        return [_cadd(z[0], z[1]), _csub(z[0], z[1])]
    q = n // 4
    steps = [_dif_step(*z[j::q], j, n) for j in range(q)]
    out = [None] * n
    out[0::2] = _fft([s[0] for s in steps] + [s[1] for s in steps])
    out[1::4] = _fft([s[2] for s in steps])
    out[3::4] = _fft([s[3] for s in steps])
    return out


def _ifft(z):
    n = len(z)
    if n == 1:
        return list(z)
    if n == 2:
        return [_cadd(z[0], z[1]), _csub(z[0], z[1])]
    q = n // 4
    e, o1, o3 = _ifft(z[0::2]), _ifft(z[1::4]), _ifft(z[3::4])
    out = [None] * n
    for j in range(q):
        out[j::q] = _dit_step(e[j], e[j + q], o1[j], o3[j], j, n)
    return out


_SUBS = ((0, 8, 0, 4), (8, 8, 1, 4), (16, 8, 3, 4), (24, 4, 2, 8), (28, 4, 6, 8))


def _fwd_first(j, xs):
    z = [_cmul(((1, x), None), -2 * math.pi * (j + 4 * m) / (4 * M1)) for m, x in enumerate(xs)]
    lo, hi = _dif_step(*z[0::2], j, 32), _dif_step(*z[1::2], j + 4, 32)
    mid = _dif_step(lo[0], hi[0], lo[1], hi[1], j, 16)
    return {j: mid[0], j + 4: mid[1], 8 + j: lo[2], 12 + j: hi[2],
            16 + j: lo[3], 20 + j: hi[3], 24 + j: mid[2], 28 + j: mid[3]}


def _inv_last(j, w):
    mid = _dit_step(w[j], w[j + 4], w[24 + j], w[28 + j], j, 16)
    lo = _dit_step(mid[0], mid[2], w[8 + j], w[16 + j], j, 32)
    hi = _dit_step(mid[1], mid[3], w[12 + j], w[20 + j], j + 4, 32)
    z = [None] * 8
    z[0::2], z[1::2] = lo, hi
    return [_cmul(v, 2 * math.pi * (j + 4 * m) / (4 * M1))[0] for m, v in enumerate(z)]


def _slots(j):
    return (j, j + 4, 8 + j, 12 + j, 16 + j, 20 + j, 24 + j, 28 + j)


def _codelet_signs():
    one = (1, 1.0)
    mid = {}
    for j in range(4):
        mid.update(_fwd_first(j, [1.0] * 8))
    mid = {s: (v[0][0], v[1][0]) for s, v in mid.items()}
    out = {}
    for s0, n, k0, dk in _SUBS:
        ys = _fft([((mid[s0 + i][0], 1.0), (mid[s0 + i][1], 1.0)) for i in range(n)])
        out.update({k0 + dk * i: (y[0][0], y[1][0]) for i, y in enumerate(ys)})
    imid = {}
    for s0, n, _, _ in _SUBS:
        imid.update({s0 + i: (w[0][0], w[1][0]) for i, w in enumerate(_ifft([(one, one)] * n))})
    return mid, out, imid


_FWD_MID_SIGNS, _FWD_SIGNS, _INV_MID_SIGNS = _codelet_signs()


class _Pacer:
    def __init__(self, never, blocks, slots, lead=0, free=0, lag=2):
        self.never, self.blocks, self.slots, self.lag = never, list(blocks), slots - lead, lag
        self.total = sum(b[0] for b in self.blocks) - free
        self.slot, self.spent, self.results = -lead, 0, []

    def note(self, result):
        self.results.append(result[:8])

    def _run_block(self):
        cost, fn, release, word = self.blocks.pop(0)
        self.spent += cost
        if release is not None and len(self.results) >= self.lag > 0:
            release(self.results[-self.lag])
        fn()
        return word

    def pace(self, x, every):
        parts = [x[8 * r:8 * r + 8] for r in range(x.shape[0] // 8)]
        for r in range(0, len(parts), every):
            self.slot += 1
            words = []
            while self.blocks and ((self.spent + self.blocks[0][0] / 2) * self.slots
                                   <= self.total * min(self.slot, self.slots)):
                word = self._run_block()
                if word not in words:
                    words.append(word)
            for word in words:
                parts[r] = jnp.where(self.never, word(), parts[r])
        return jnp.concatenate(parts, axis=0)

    def run(self, pieces):
        for piece in pieces:
            piece(self)
        while self.blocks:
            self._run_block()


def _pack_rows(m):
    b = np.asarray(m, np.float32).astype(ml_dtypes.bfloat16).view(np.uint16).astype(np.uint32)
    return np.ascontiguousarray(b[..., 0::2, :] | (b[..., 1::2, :] << 16))


def _dft_tables():
    r = np.arange(128)
    part = (r // 8) % 2
    nat = 8 * (r // 16) + r % 8
    eo = 16 * (r // 32) + 2 * (r % 8) + (r // 16) % 2
    fwd = np.zeros((M1, 128, 128))
    inv = np.zeros((M1, 128, 128))
    for k1 in range(M1):
        freq = k1 + M1 * nat + 0.25
        ph = 2 * np.pi * freq[:, None] * eo[None, :] / S
        same = part[:, None] == part[None, :]
        cross = np.where(part[:, None] == 0, 1.0, -1.0)
        sg = np.where(part == 0, _FWD_SIGNS[k1][0], _FWD_SIGNS[k1][1])
        fwd[k1] = np.where(same, np.cos(ph), cross * np.sin(ph)) * sg[None, :]
        ph = 2 * np.pi * nat[:, None] * freq[None, :] / S
        inv[k1] = np.where(same, np.cos(ph), -cross * np.sin(ph)) / S
    return _pack_rows(fwd), _pack_rows(inv)


_G_FWD, _G_INV = _dft_tables()


def _pk(x):
    return pltpu.bitcast(x, u32)


def _upk(x):
    return pltpu.bitcast(x, bf16)


def _even(x):
    return pltpu.bitcast(x << 16, f32)


def _odd(x):
    return pltpu.bitcast(x & jnp.uint32(0xFFFF0000), f32)


def _dot(a, b):
    return jnp.dot(a, b, preferred_element_type=f32)


def _dot_t(a, b):
    return lax.dot_general(a, b, (((1,), (1,)), ((), ())), preferred_element_type=f32)


def _phi(t):
    return jnp.where(t > 0, t + 1.0, jnp.exp2(t * LOG2E))


def _recip(x):
    r = pltpu.reciprocal(x, approx=True)
    return r * (2.0 - x * r)


def _ds(start, size, align=8):
    return pl.ds(pl.multiple_of(start, align), size)


def _kernel(
    q_hbm, k_hbm, v_hbm, shift_ref, h_hbm, d_ref,
    x_hbm, wq_hbm, wk_hbm, wv_hbm, wo_hbm, beta_ref, gf_hbm, gi_hbm,
    out_hbm,
    x_b, wq_b, wk_b, wv_b, wo_b, k_b, v_b, h_b, q_b, gf_v, gi_v, oa_b, ob_b,
    wt_v, ht_v, mx_v, mh_v, kv_v, par_v, yx_b, yh_b, ua_v, ub_v,
    kt_b, kg_v, qt_b, pqt_b, vt_b, ot_b, on_a, on_b,
    sa_v, ma_v, sb_v, mb_v, mem_v, gate_v, zero_s, sems,
):
    x_v, wq_v, wk_v, wv_v, wo_v = (r.bitcast(u32) for r in (x_b, wq_b, wk_b, wv_b, wo_b))
    k_v, v_v, h_v, q_v = (r.bitcast(u32) for r in (k_b, v_b, h_b, q_b))
    yx_v, yh_v, kt_v, oa_v = (r.bitcast(u32) for r in (yx_b, yh_b, kt_b, oa_b))
    qt_v, pqt_v, vt_v, ot_v = (r.bitcast(u32) for r in (qt_b, pqt_b, vt_b, ot_b))

    n_sem = [0]

    def group(pairs):
        sem = sems.at[n_sem[0]]
        n_sem[0] += 1
        return [pltpu.make_async_copy(src, dst, sem) for src, dst in pairs]

    def cols(t):
        return pl.ds(128 * t, 128)

    def weight(hbm, buf):
        return group([(hbm.at[:, cols(t)], buf.at[t]) for t in range(NT)])

    def xrows(r0, n):
        return group([(x_hbm.at[pl.ds(r0, n), cols(t)], x_b.at[t, pl.ds(r0, n)]) for t in range(NT)])

    c_wk, c_wq, c_wv, c_wo = (weight(a, b) for a, b in
                              ((wk_hbm, wk_b), (wq_hbm, wq_b), (wv_hbm, wv_b), (wo_hbm, wo_b)))
    c_x = [xrows(0, 512), xrows(512, 768), xrows(1280, 768)]
    c_h = [group([(h_hbm.at[cols(t)], h_b.at[t])]) for t in range(NT)]
    c_kv = [group([(k_hbm.at[:, cols(t)], k_b.at[t, pl.ds(16, S)]),
                   (v_hbm.at[:, cols(t)], v_b.at[t])]) for t in range(NT)]
    c_g = group([(gf_hbm, gf_v), (gi_hbm, gi_v)])
    c_q = group([(q_hbm.at[:, cols(t)], q_b.at[t]) for t in range(NT)])
    c_oa = [group([(oa_b.at[t], out_hbm.at[:, cols(t)])]) for t in range(NT)]
    c_ob = [group([(ob_b.at[t, pl.ds(SEG * s, SEG)], out_hbm.at[pl.ds(SEG * s, SEG), cols(NT + t)])
                   for t in range(NT)]) for s in range(S // SEG)]

    def start(cs):
        for c in cs:
            c.start()

    def wait(cs):
        for c in cs:
            c.wait()

    def wait_when(cond, cs):
        pl.when(cond)(lambda: wait(cs))

    for cs in (c_wq, c_wv, c_wk, c_x[0], c_h[0], c_x[1], c_kv[0], c_h[1], c_kv[1], c_h[2], c_x[2],
               c_kv[2], c_h[3], c_kv[3], c_h[4], c_kv[4], c_g, c_q, c_wo):
        start(cs)

    sub8 = lax.broadcasted_iota(i32, (8, 128), 0)
    lane8 = lax.broadcasted_iota(i32, (8, 128), 1)

    zero_s[0] = 0
    zero_s[1] = 0
    zero_s[2] = 0
    taps = shift_ref[...].astype(f32)
    skip = d_ref[...].astype(f32).reshape(1, D)
    for t in range(NT):
        for j in range(4):
            par_v[t, j] = jnp.broadcast_to(taps[j:j + 1, 128 * t:128 * t + 128], (8, 128))
        par_v[t, 4] = jnp.where(sub8 == 0, skip[:, 128 * t:128 * t + 128], 0.0)
        k_v[t, 0:8, :] = jnp.zeros((8, 128), u32)
    beta = beta_ref[...].astype(f32).reshape(1, 4 * NG)
    gate = 1.0 / (1.0 + jnp.exp(-beta))
    for h in range(4 * NG):
        gate_v[h] = jnp.broadcast_to(gate[:, h:h + 1], (8, 128))

    wait(c_wq)
    wait(c_wv)
    for ft in range(NT):
        for kt in range(NT):
            wt_v[ft, kt, 0:64, :] = _pk(_upk(wq_v[ft, 64 * kt:64 * kt + 64, :]).T)
            wt_v[ft, kt, 64:128, :] = _pk(_upk(wv_v[ft, 64 * kt:64 * kt + 64, :]).T)

    q_scale = DH ** -0.5 * LOG2E

    def project(tile0, ntiles, ft):
        rows = _ds(ft * 128, 128, 128)

        def x_tile(j, pace=None):
            tok = _ds((tile0 + j) * 64, 64)
            parts = [x_v[kt, tok, :] for kt in range(NT)]
            if pace is not None:
                parts[0] = pace.pace(parts[0], PACE1)
            return _upk(jnp.concatenate(parts, axis=1))

        def w_t(half, pace):
            parts = [wt_v[ft, kt, 64 * half:64 * half + 64, :] for kt in range(NT)]
            parts[0] = pace.pace(parts[0], PACE1)
            return _upk(jnp.concatenate(parts, axis=1))

        def q_piece(j, pace):
            q = _dot_t(w_t(0, pace), x_tile(j))
            pace.note(q)
            qt_b[tile0 + j, rows, :] = (q * q_scale).astype(bf16)
            pqt_b[tile0 + j, rows, :] = _phi(q).astype(bf16)

        def v_piece(j, pace):
            v = _dot_t(w_t(1, pace), x_tile(j))
            pace.note(v)
            vt_b[tile0 + j, rows, :] = v.astype(bf16)

        def k_piece(j, pace):
            k = _dot(x_tile(j, pace), _upk(wk_v[ft]))
            pace.note(k)
            kt_b[ft, _ds((tile0 + j) * 128, 128, 128), :] = k.astype(bf16)

        return [functools.partial(f, j) for j in range(ntiles) for f in (k_piece, q_piece, v_piece)]

    class Spare:
        def __init__(self, view, *idx):
            self.view, self.idx = view, idx
            view[(*idx, slice(0, 8), slice(None))] = jnp.zeros((8, 128), view.dtype)

        def word(self):
            return pltpu.bitcast(self.view[(*self.idx, _ds(zero_s[2], 8), slice(None))], u32)

        def release(self, value):
            self.view[(*self.idx, _ds(zero_s[2] + 8, 8), slice(None))] = pltpu.bitcast(value, self.view.dtype)

    sp_ht, sp_k, sp_kv = Spare(ht_v, NT), Spare(k_v, NT), Spare(kv_v, 2)
    sp_mx, sp_mh, sp_yx, sp_yh = Spare(mx_v, 2), Spare(mh_v, 2), Spare(yx_v, NT, 0), Spare(yh_v, NT, 0)
    sp_oa, sp_kt, sp_kg = Spare(oa_v, NT), Spare(kt_v, NT), Spare(kg_v, NG)
    sp_ua, sp_ub = Spare(ua_v, 0, M1), Spare(ub_v, 0, M1)

    def block(cost, src, dst, fn, *args):
        return (cost, functools.partial(fn, *args), src.release if src else None, dst.word)

    def transpose_filter(ct, t0, n):
        def one(t):
            ht_v[ct, _ds((t0 + t) * 64, 64), :] = _pk(_upk(h_v[ct, :, _ds((t0 + t) * 128, 128, 128)]).T)

        return [block(20, None, sp_ht, one, t) for t in range(n)]

    def forward_unit(ct, bb):
        r0 = pl.multiple_of(bb * 8, 8)

        def short_conv(n1):
            w = [par_v[ct, j] for j in range(4)]
            base = r0 + 32 * n1
            p0, p1, p2 = (k_v[ct, pl.ds(base + 8 - j, 8), :] for j in range(3))
            e0, o0, e1, o1, o2 = _even(p0), _odd(p0), _even(p1), _odd(p1), _odd(p2)
            vv = v_v[ct, _ds(base, 8), :]
            return ((w[0] * e0 + w[1] * o1 + w[2] * e1 + w[3] * o2) * _even(vv),
                    (w[0] * o0 + w[1] * e0 + w[2] * o1 + w[3] * e1) * _odd(vv))

        def park(mid, par, vals):
            for s, (re, im) in vals.items():
                mid[par, pl.ds(16 * s, 8), :] = re[1]
                mid[par, pl.ds(16 * s + 8, 8), :] = im[1]

        def conv(n1s):
            for n1 in n1s:
                for par, y in enumerate(short_conv(n1)):
                    kv_v[par, pl.ds(8 * n1, 8), :] = y

        def first_x(j, par):
            xs = [kv_v[par, _ds(8 * (j + 4 * m) + zero_s[2], 8), :] for m in range(8)]
            park(mx_v, par, _fwd_first(j, xs))

        def first_h(j, par):
            xs = [(_odd if par else _even)(ht_v[ct, _ds(r0 + 32 * (j + 4 * m), 8), :]) for m in range(8)]
            if par == 0 and j == 0:
                xs[0] = xs[0] + jnp.where(bb == 0, par_v[ct, 4], 0.0)
            park(mh_v, par, _fwd_first(j, xs))

        def second(mid, dst, par, subs):
            for s0, n, k0, dk in subs:
                zs = [((_FWD_MID_SIGNS[s][0], mid[par, _ds(16 * s + zero_s[2], 8), :]),
                       (_FWD_MID_SIGNS[s][1], mid[par, _ds(16 * s + 8 + zero_s[2], 8), :]))
                      for s in range(s0, s0 + n)]
                for i, (re, im) in enumerate(_fft(zs)):
                    y = jnp.concatenate([re[1], im[1]], axis=0).astype(bf16)
                    dst[ct, k0 + dk * i, _ds(bb * 32 + 16 * par, 16, 16), :] = y

        def seconds(mid, dst, sp_src, sp_dst):
            return [block(64 if len(subs) == 1 else 40, sp_src, sp_dst, second, mid, dst, par, subs)
                    for par in range(2) for subs in (_SUBS[0:1], _SUBS[1:2], _SUBS[2:3], _SUBS[3:5])]

        def firsts(fn, sp_src, sp_dst):
            return [block(105, sp_src, sp_dst, fn, j, par) for par in range(2) for j in range(4)]

        convs = [block(92, sp_k, sp_kv, conv, range(n, n + 4)) for n in range(0, M1, 4)]
        return (firsts(first_h, sp_ht, sp_mh) + convs + seconds(mh_v, yh_b, sp_mh, sp_yh)
                + firsts(first_x, sp_kv, sp_mx) + seconds(mx_v, yx_b, sp_mx, sp_yx))

    def pacer(blocks, slots, lead=0, free=0, lag=0):
        return _Pacer(sub8 < zero_s[2], blocks, slots, lead, free, lag)

    wait(c_wk)
    wait(c_x[0])
    wait(c_h[0])

    def phase1a(ft, c):
        pacer(transpose_filter(0, jnp.minimum(4 * ft, 12), 4), 8).run(project(0, 4, ft))
        return c

    lax.fori_loop(0, NT, phase1a, 0)

    def phase1b(i, c):
        wait_when(i == 0, c_x[1])
        wait_when(i == NT, c_x[2])
        for ct in range(NT):
            wait_when(i == 2 * ct, c_kv[ct] + (c_h[ct + 1] if ct + 1 < NT else []))
        ct = i // 2
        blocks = []
        for u in range(2):
            blocks += forward_unit(ct, 2 * (i % 2) + u)
            blocks += transpose_filter(jnp.minimum(ct + 1, NT - 1), 8 * (i % 2) + 4 * u, 4)
        pacer(blocks, 18 * 8 // PACE1, LEAD1, FREE1, LAG1).run(project(4 + 6 * (i // NT), 6, i % NT))
        return c

    lax.fori_loop(0, 2 * NT, phase1b, 0)

    def spectral(ct, u_out, z):
        zs = {}

        def fwd(k1, pace):
            g = _upk(pace.pace(gf_v[k1], PACE2))
            x = _dot(g, _upk(yx_v[ct, k1]))
            h = _dot(g, _upk(yh_v[ct, k1]))
            rows = []
            for a in range(8):
                xr, xi = x[16 * a:16 * a + 8], x[16 * a + 8:16 * a + 16]
                hr, hi = h[16 * a:16 * a + 8], h[16 * a + 8:16 * a + 16]
                rows += [xr * hr - xi * hi, xr * hi + xi * hr]
            pace.note(x)
            zs[k1] = jnp.concatenate(rows, axis=0).astype(bf16)

        def inv(k1, pace):
            u_out[z, k1] = _dot(_upk(pace.pace(gi_v[k1], PACE2)), zs.pop(k1))

        pieces = []
        for k1 in range(M1 + LOOK2):
            if k1 < M1:
                pieces.append(functools.partial(fwd, k1))
            if k1 >= LOOK2:
                pieces.append(functools.partial(inv, k1 - LOOK2))
        return pieces

    def inverse(ct, u_in, z):
        def first(mid, a, subs):
            for s0, n, k0, dk in subs:
                zs = [((1, u_in[z, k, 16 * a:16 * a + 8, :]), (1, u_in[z, k, 16 * a + 8:16 * a + 16, :]))
                      for k in range(k0, M1, dk)]
                for i, (re, im) in enumerate(_ifft(zs)):
                    mid[a % 2, pl.ds(16 * (s0 + i), 8), :] = re[1]
                    mid[a % 2, pl.ds(16 * (s0 + i) + 8, 8), :] = im[1]

        def last(mid, bb, j, par):
            w = {s: ((_INV_MID_SIGNS[s][0], mid[par, _ds(16 * s + zero_s[2], 8), :]),
                     (_INV_MID_SIGNS[s][1], mid[par, _ds(16 * s + 8 + zero_s[2], 8), :]))
                 for s in _slots(j)}
            for m, (sign, y) in enumerate(_inv_last(j, w)):
                n1 = j + 4 * m
                if par == 0:
                    kv_v[0, pl.ds(8 * n1, 8), :] = y
                    continue
                gate_q = _upk(q_v[ct, pl.ds(32 * n1 + 8 * bb, 8), :]).astype(f32)
                y = jnp.concatenate([kv_v[0, _ds(8 * n1 + zero_s[2], 8), :], y], axis=0) * gate_q
                oa_b[ct, pl.ds(64 * n1 + 16 * bb, 16), :] = (y if sign > 0 else -y).astype(bf16)

        blocks = []
        sp_u = sp_ua if u_in is ua_v else sp_ub
        for bb in range(4):
            mid, sp_mid = (mh_v, sp_mh) if bb % 2 else (mx_v, sp_mx)
            blocks += [block(56 if len(subs) == 1 else 32, sp_u, sp_mid, first, mid, a, subs)
                       for a in (2 * bb, 2 * bb + 1)
                       for subs in (_SUBS[0:1], _SUBS[1:2], _SUBS[2:3], _SUBS[3:5])]
            blocks += [block(125 if par else 85, sp_mid, sp_oa if par else sp_kv, last, mid, bb, j, par)
                       for par in range(2) for j in range(4)]
        return blocks

    def align_keys(r0, n):
        def one(r):
            rows = _ds(r0 + r, 16)
            lane = lax.broadcasted_iota(i32, (16, 128), 1)
            for g in range(NG):
                t, off = divmod(80 * g, 128)
                x = kt_v[t, rows, :]
                if off > 48:
                    x = jnp.where(lane >= off, x, kt_v[t + 1, rows, :])
                kg_v[g, rows, :] = pltpu.roll(x, 128 - off, 1) if off else x

        return [block(1, sp_kt, sp_kg, one, r) for r in range(0, n, 16)]

    wait(c_g)
    pacer(align_keys(0, S // 2), 64).run(spectral(0, ua_v, zero_s[0]))
    wait(c_q)

    def phase2(i, c):
        z0, z1 = zero_s[0], zero_s[1]

        @pl.when(i > 0)
        def _():
            start(c_oa[0] + c_oa[1])

        pacer(inverse(2 * i, ua_v, z1), 64 * 8 // PACE2 - TAIL2, LEAD2, 0, LAG2).run(spectral(2 * i + 1, ub_v, z0))
        pacer(inverse(2 * i + 1, ub_v, z1), 64 * 8 // PACE2, MID2, FREE2, LAG2).run(spectral(2 * i + 2, ua_v, z0))
        return c

    lax.fori_loop(0, 2, phase2, 0)
    start(c_oa[2] + c_oa[3])

    prow = lax.broadcasted_iota(i32, (16, 128), 0)
    base = {3: 0, 2: 4, 1: 7, 0: 9}
    steps = [(j, t) for j in (3, 2, 1, 0) for t in range(j + 1)]

    def attend(uq, s_out, m_out, zo, up, s_in, m_in, zi, memory, pace=None):
        ri = lax.broadcasted_iota(i32, (128, 128), 0)
        ci = lax.broadcasted_iota(i32, (128, 128), 1)
        bias = jnp.where(ri <= ci, 0.0, -1e9 * LOG2E).astype(f32)
        if uq is not None:
            sq, gq = uq // NG, uq % NG
        if up is not None:
            sp, gp = up // NG, up % NG
            gates = [gate_v[4 * gp + i] for i in range(4)]
        weights, run_max, acc = {}, {}, {}

        def q_weights(j):
            if j not in weights:
                ws = []
                for i in range(4):
                    own = (prow >= 2 * i) & (prow < 2 * i + 10)
                    qw = jnp.where(own, qt_v[4 * sq + j, _ds(40 * gq + 8 * i, 16), :], jnp.uint32(0))
                    parts = [jnp.zeros((8 * i, 128), u32)] if i else []
                    ws.append(jnp.concatenate(parts + [qw, jnp.zeros((48 - 8 * i, 128), u32)], axis=0))
                weights[j] = _upk(jnp.concatenate(ws, axis=1))
            return weights[j]

        def v_rows(i, t):
            free = prow >= 12 if i < 2 else prow < 4
            return _upk(jnp.where(free, jnp.uint32(0x3F803F80), vt_v[4 * sp + t, _ds(40 * gp + 8 * i, 16), :]))

        if memory:
            prev = 4 * (sp - 1)
            upd = None
            for t in range(4):
                pk_t = _phi(_upk(kg_v[gp, _ds((prev + t) * 64, 64), :]).astype(f32)).astype(bf16)
                lhs = jnp.concatenate([vt_v[prev + t, _ds(40 * gp, 40), :],
                                       jnp.full((8, 128), 0x3F803F80, u32)], axis=0)
                d = _dot(_upk(lhs), pk_t)
                upd = d if upd is None else upd + d
            m = mem_v[gp] + upd[:88]
            mem_v[gp] = m
            own = [(lane8 >= DH * i) & (lane8 < DH * i + DH) for i in range(4)]
            rows = []
            for r in range(10):
                lo, hi = (8 * r) // DH, (8 * r + 7) // DH
                blk = m[8 * r:8 * r + 8]
                a = jnp.where(own[lo], blk * gates[lo], 0.0)
                if hi != lo:
                    a = jnp.where(sub8 < 4, a, jnp.where(own[hi], blk * gates[hi], 0.0))
                rows.append(a)
            rows += [jnp.where(own[i], m[80:88], 0.0) for i in range(4)]
            mem_lhs = jnp.concatenate(rows, axis=0).astype(bf16)

        def memory_read(j):
            w = jnp.concatenate([pqt_v[4 * sp + j, _ds(40 * gp, 40), :], jnp.zeros((24, 128), u32)], axis=0)
            r = _dot(mem_lhs, _upk(w))
            inv = [_recip(r[80 + 8 * i:88 + 8 * i] + 1e-6) for i in range(4)]
            rows = []
            for b in range(10):
                lo, hi = (8 * b) // DH, (8 * b + 7) // DH
                rows.append(r[8 * b:8 * b + 8] * (inv[lo] if lo == hi else jnp.where(sub8 < 4, inv[lo], inv[hi])))
            return rows

        def finish(j):
            a = []
            for i in range(4):
                o = acc[(j, i)]
                r = _recip(o[24:32] if i < 2 else o[0:8]) * (1.0 - gates[i])
                a.append([o[8 * b:8 * b + 8] * r for b in range(4)])
            low = sub8 < 4
            rows = [a[0][0], a[0][1], jnp.where(low, a[0][2], a[1][0]), a[1][1], a[1][2],
                    a[2][1], a[2][2], jnp.where(low, a[2][3], a[3][1]), a[3][2], a[3][3]]
            if memory:
                rows = [x + y for x, y in zip(rows, memory_read(j))]
            ot_b[4 * sp + j, _ds(80 * gp, 80, 16), :] = jnp.concatenate(rows, axis=0).astype(bf16)

        for j, t in steps:
            if uq is not None:
                keys = kg_v[gq, _ds(256 * sq + 64 * t, 64), :]
                keys = _upk(pace.pace(keys, 2) if pace else keys)
                logits = _dot(keys, q_weights(j))
            if up is not None:
                ps = [jnp.exp2(s_in[zi, i, base[j] + t].reshape(16, 8, 128) - m_in[zi, j, i][None])
                      .reshape(128, 128).astype(bf16) for i in range(4)]
            if uq is not None:
                for i in range(4):
                    st = logits[:, 128 * i:128 * i + 128]
                    if t == j:
                        st = st + bias
                    s_out[zo, i, base[j] + t] = st
                    mx = jnp.max(st.reshape(16, 8, 128), axis=0)
                    run_max[(j, i)] = mx if t == 0 else jnp.maximum(run_max[(j, i)], mx)
                    if t == j:
                        m_out[zo, j, i] = jnp.broadcast_to(
                            jnp.max(run_max[(j, i)], axis=0, keepdims=True), (8, 128))
            if up is not None:
                for i in range(4):
                    d = _dot(v_rows(i, t), ps[i])
                    acc[(j, i)] = d if t == 0 else acc[(j, i)] + d
                if t == j:
                    finish(j)

    mem_v[...] = jnp.zeros(mem_v.shape, f32)
    z0, z1 = zero_s[0], zero_s[1]
    pacer(inverse(NT - 1, ua_v, z1), 40).run(
        [lambda p: attend(0, sa_v, ma_v, z0, None, None, None, None, False, p)])
    start(c_oa[NT - 1])

    def attend_pair(memory, last=False):
        def body(i, c):
            z0, z1 = zero_s[0], zero_s[1]
            attend(2 * i + 1, sb_v, mb_v, z0, 2 * i, sa_v, ma_v, z1, memory)
            attend(None if last else 2 * i + 2, sa_v, ma_v, z0, 2 * i + 1, sb_v, mb_v, z1, memory)
            return c
        return body

    lax.fori_loop(0, 4, attend_pair(False), 0)
    lax.fori_loop(4, 15, attend_pair(True), 0)
    attend_pair(True, last=True)(15, 0)

    def transpose_heads(s, dst, z):
        for j in range(4):
            for ft in range(NT):
                dst[z, ft, 64 * j:64 * j + 64, :] = _pk(_upk(ot_v[4 * s + j, 64 * ft:64 * ft + 64, :]).T)

    def out_project(s, src, z):
        lhs = _upk(jnp.concatenate([src[z, ft] for ft in range(NT)], axis=1))
        for nt in range(NT):
            ob_b[nt, pl.ds(SEG * s, SEG), :] = _dot(lhs, _upk(wo_v[nt])).astype(bf16)

    wait(c_wo)
    z0, z1 = zero_s[0], zero_s[1]
    transpose_heads(0, on_a, z0)
    for s in range(S // SEG):
        src, dst = (on_a, on_b) if s % 2 == 0 else (on_b, on_a)
        if s + 1 < S // SEG:
            transpose_heads(s + 1, dst, z0)
        out_project(s, src, z1)
        start(c_ob[s])
    for cs in c_oa + c_ob:
        wait(cs)


@jax.jit
def pallas_concat_heads__ssm_conv_h3__memory_aug_infini_attn__prompt_kernel(
    A_q: jax.Array,
    A_k: jax.Array,
    A_v: jax.Array,
    A_shift_k: jax.Array,
    A_ssm_k: jax.Array,
    A_ssm_D: jax.Array,
    B_x: jax.Array,
    B_wq: jax.Array,
    B_wk: jax.Array,
    B_wv: jax.Array,
    B_wo: jax.Array,
    B_beta: jax.Array,
):
    hbm = pl.BlockSpec(memory_space=pl.ANY)
    vmem = pl.BlockSpec(memory_space=pltpu.VMEM)
    V = pltpu.VMEM
    scratch = [
        V((NT, S, 128), bf16),
        V((NT, D, 128), bf16), V((NT, D, 128), bf16),
        V((NT, D, 128), bf16), V((NT, D, 128), bf16),
        V((NT + 1, S + 16, 128), bf16), V((NT, S, 128), bf16),
        V((NT, 128, S), bf16), V((NT, S, 128), bf16),
        V((M1, 64, 128), u32), V((M1, 64, 128), u32),
        V((NT + 1, S, 128), bf16), V((NT, S, 128), bf16),
        V((NT, NT, 128, 128), u32),
        V((NT + 1, S // 2, 128), u32),
        V((3, 16 * M1, 128), f32), V((3, 16 * M1, 128), f32),
        V((3, 8 * M1, 128), f32),
        V((NT, 5, 8, 128), f32),
        V((NT + 1, M1, 128, 128), bf16), V((NT + 1, M1, 128, 128), bf16),
        V((1, M1 + 1, 128, 128), f32), V((1, M1 + 1, 128, 128), f32),
        V((NT + 1, S, 128), bf16), V((NG + 1, S // 2, 128), u32),
        V((16, D, 128), bf16), V((16, D, 128), bf16),
        V((16, D, 128), bf16), V((16, D, 128), bf16),
        V((1, NT, SEG // 2, 128), u32), V((1, NT, SEG // 2, 128), u32),
        V((1, 4, 10, 128, 128), f32), V((1, 4, 4, 8, 128), f32),
        V((1, 4, 10, 128, 128), f32), V((1, 4, 4, 8, 128), f32),
        V((NG, 88, 128), f32),
        V((4 * NG, 8, 128), f32),
        pltpu.SMEM((3,), i32),
        pltpu.SemaphoreType.DMA((32,)),
    ]
    out = pl.pallas_call(
        _kernel,
        out_shape=jax.ShapeDtypeStruct((S, 2 * D), bf16),
        in_specs=[hbm, hbm, hbm, vmem, hbm, vmem, hbm, hbm, hbm, hbm, hbm, vmem, hbm, hbm],
        out_specs=hbm,
        scratch_shapes=scratch,
        compiler_params=pltpu.CompilerParams(vmem_limit_bytes=110 * 2**20),
    )(
        A_q.reshape(S, D), A_k.reshape(S, D), A_v.reshape(S, D), A_shift_k.T, A_ssm_k, A_ssm_D,
        B_x.reshape(S, D), B_wq, B_wk, B_wv, B_wo, B_beta, _G_FWD, _G_INV,
    )
    return out.reshape(1, S, 2 * D)
```

```python
import functools
import math

import jax
import jax.numpy as jnp
import ml_dtypes
import numpy as np
from jax import lax
from jax.experimental import pallas as pl
from jax.experimental.pallas import tpu as pltpu

S = 2048
D = 640
NT = D // 128
DH = 20
NG = 8
SEG = 512
M1, M2 = 32, 64

bf16 = jnp.bfloat16
f32 = jnp.float32
u32 = jnp.uint32
i32 = jnp.int32

LOG2E = math.log2(math.e)
PACE0 = 4
LAG0 = 0
PACE1 = 2
LEAD1 = 4
FREE1 = 400
LAG1 = 2
TR1 = 0
HALVES = ((0,), (1,))
PACE2 = 4
LEAD2 = 4
FREE2 = 0
LOOK2 = 5
LAG2 = 4
LAG2F = 4
NF2 = 3
NI2 = 1
NS4 = 3
PACE4 = 4
FREE4 = 0
OUT_CHUNKS = ((0, 4), (4, 8), (8, 12), (12, 15), (15, 16))
LAG4 = 0


def _neg(a):
    return None if a is None else (-a[0], a[1])


def _add(a, b):
    if a is None:
        return b
    if b is None:
        return a
    if a[0] == b[0]:
        return (a[0], a[1] + b[1])
    if a[0] > 0:
        return (1, a[1] - b[1])
    return (1, b[1] - a[1])


def _sub(a, b):
    return _add(a, _neg(b))


def _scale(a, c):
    if a is None or abs(c) < 1e-12:
        return None
    if abs(abs(c) - 1.0) < 1e-12:
        return a if c > 0 else _neg(a)
    return (a[0], a[1] * float(c))


def _cmul(z, ang):
    c, s = math.cos(ang), math.sin(ang)
    x, y = z
    if x is not None and y is not None and abs(abs(c) - abs(s)) < 1e-12:
        r = 1.0 if c * s > 0 else -1.0
        if r > 0:
            return (_scale(_sub(x, y), c), _scale(_add(y, x), c))
        return (_scale(_add(x, y), c), _scale(_sub(y, x), c))
    return (_sub(_scale(x, c), _scale(y, s)), _add(_scale(y, c), _scale(x, s)))


def _cadd(a, b):
    return (_add(a[0], b[0]), _add(a[1], b[1]))


def _csub(a, b):
    return (_sub(a[0], b[0]), _sub(a[1], b[1]))


def _dif_step(a, b, c, d, j, n):
    t1, t2 = _csub(a, c), _csub(b, d)
    mi_t2 = (t2[1], _neg(t2[0]))
    return (_cadd(a, c), _cadd(b, d),
            _cmul(_cadd(t1, mi_t2), -2 * math.pi * j / n),
            _cmul(_csub(t1, mi_t2), -6 * math.pi * j / n))


def _dit_step(e0, e1, o1, o3, j, n):
    a, b = _cmul(o1, 2 * math.pi * j / n), _cmul(o3, 6 * math.pi * j / n)
    s, d = _cadd(a, b), _csub(a, b)
    i_d = (_neg(d[1]), d[0])
    return _cadd(e0, s), _cadd(e1, i_d), _csub(e0, s), _csub(e1, i_d)


def _fft(z):
    n = len(z)
    if n == 1:
        return list(z)
    if n == 2:
        return [_cadd(z[0], z[1]), _csub(z[0], z[1])]
    q = n // 4
    steps = [_dif_step(*z[j::q], j, n) for j in range(q)]
    out = [None] * n
    out[0::2] = _fft([s[0] for s in steps] + [s[1] for s in steps])
    out[1::4] = _fft([s[2] for s in steps])
    out[3::4] = _fft([s[3] for s in steps])
    return out


def _ifft(z):
    n = len(z)
    if n == 1:
        return list(z)
    if n == 2:
        return [_cadd(z[0], z[1]), _csub(z[0], z[1])]
    q = n // 4
    e, o1, o3 = _ifft(z[0::2]), _ifft(z[1::4]), _ifft(z[3::4])
    out = [None] * n
    for j in range(q):
        out[j::q] = _dit_step(e[j], e[j + q], o1[j], o3[j], j, n)
    return out


_SUBS = ((0, 8, 0, 4), (8, 8, 1, 4), (16, 8, 3, 4), (24, 4, 2, 8), (28, 4, 6, 8))


def _fwd_first(j, xs):
    z = [_cmul(((1, x), None), -2 * math.pi * (j + 4 * m) / (4 * M1)) for m, x in enumerate(xs)]
    lo, hi = _dif_step(*z[0::2], j, 32), _dif_step(*z[1::2], j + 4, 32)
    mid = _dif_step(lo[0], hi[0], lo[1], hi[1], j, 16)
    return {j: mid[0], j + 4: mid[1], 8 + j: lo[2], 12 + j: hi[2],
            16 + j: lo[3], 20 + j: hi[3], 24 + j: mid[2], 28 + j: mid[3]}


def _inv_last(j, w):
    mid = _dit_step(w[j], w[j + 4], w[24 + j], w[28 + j], j, 16)
    lo = _dit_step(mid[0], mid[2], w[8 + j], w[16 + j], j, 32)
    hi = _dit_step(mid[1], mid[3], w[12 + j], w[20 + j], j + 4, 32)
    z = [None] * 8
    z[0::2], z[1::2] = lo, hi
    return [_cmul(v, 2 * math.pi * (j + 4 * m) / (4 * M1))[0] for m, v in enumerate(z)]


def _slots(j):
    return (j, j + 4, 8 + j, 12 + j, 16 + j, 20 + j, 24 + j, 28 + j)


def _codelet_signs():
    one = (1, 1.0)
    mid = {}
    for j in range(4):
        mid.update(_fwd_first(j, [1.0] * 8))
    mid = {s: (v[0][0], v[1][0]) for s, v in mid.items()}
    out = {}
    for s0, n, k0, dk in _SUBS:
        ys = _fft([((mid[s0 + i][0], 1.0), (mid[s0 + i][1], 1.0)) for i in range(n)])
        out.update({k0 + dk * i: (y[0][0], y[1][0]) for i, y in enumerate(ys)})
    imid = {}
    for s0, n, _, _ in _SUBS:
        imid.update({s0 + i: (w[0][0], w[1][0]) for i, w in enumerate(_ifft([(one, one)] * n))})
    return mid, out, imid


_FWD_MID_SIGNS, _FWD_SIGNS, _INV_MID_SIGNS = _codelet_signs()


class _Pacer:
    def __init__(self, never, blocks, slots, lead=0, free=0, lag=2):
        self.never, self.blocks, self.slots, self.lag = never, list(blocks), slots - lead, lag
        self.total = sum(b[0] for b in self.blocks) - free
        self.slot, self.spent, self.results = -lead, 0, []

    def note(self, result):
        self.results.append(result[:8])

    def _run_block(self):
        cost, fn, release, word = self.blocks.pop(0)
        self.spent += cost
        if release is not None and len(self.results) >= self.lag > 0:
            release(self.results[-self.lag])
        fn()
        return word

    def pace(self, x, every):
        parts = [x[8 * r:8 * r + 8] for r in range(x.shape[0] // 8)]
        for r in range(0, len(parts), every):
            self.slot += 1
            words = []
            while self.blocks and ((self.spent + self.blocks[0][0] / 2) * self.slots
                                   <= self.total * min(self.slot, self.slots)):
                word = self._run_block()
                if word not in words:
                    words.append(word)
            for word in words:
                parts[r] = jnp.where(self.never, word(), parts[r])
        return jnp.concatenate(parts, axis=0)

    def run(self, pieces):
        for piece in pieces:
            piece(self)
        while self.blocks:
            self._run_block()


def _pack_rows(m):
    b = np.asarray(m, np.float32).astype(ml_dtypes.bfloat16).view(np.uint16).astype(np.uint32)
    return np.ascontiguousarray(b[..., 0::2, :] | (b[..., 1::2, :] << 16))


def _dft_tables():
    r = np.arange(128)
    part = (r // 8) % 2
    nat = 8 * (r // 16) + r % 8
    eo = 16 * (r // 32) + 2 * (r % 8) + (r // 16) % 2
    fwd = np.zeros((M1, 128, 128))
    inv = np.zeros((M1, 128, 128))
    for k1 in range(M1):
        freq = k1 + M1 * nat + 0.25
        ph = 2 * np.pi * freq[:, None] * eo[None, :] / S
        same = part[:, None] == part[None, :]
        cross = np.where(part[:, None] == 0, 1.0, -1.0)
        sg = np.where(part == 0, _FWD_SIGNS[k1][0], _FWD_SIGNS[k1][1])
        fwd[k1] = np.where(same, np.cos(ph), cross * np.sin(ph)) * sg[None, :]
        ph = 2 * np.pi * nat[:, None] * freq[None, :] / S
        inv[k1] = np.where(same, np.cos(ph), -cross * np.sin(ph)) / S
    return _pack_rows(fwd), _pack_rows(inv)


_G_FWD, _G_INV = _dft_tables()


def _pk(x):
    return pltpu.bitcast(x, u32)


def _upk(x):
    return pltpu.bitcast(x, bf16)


def _even(x):
    return pltpu.bitcast(x << 16, f32)


def _odd(x):
    return pltpu.bitcast(x & jnp.uint32(0xFFFF0000), f32)


def _dot(a, b):
    return jnp.dot(a, b, preferred_element_type=f32)


def _dot_t(a, b):
    return lax.dot_general(a, b, (((1,), (1,)), ((), ())), preferred_element_type=f32)


def _phi(t):
    return jnp.where(t > 0, t + 1.0, jnp.exp2(t * LOG2E))


def _recip(x):
    r = pltpu.reciprocal(x, approx=True)
    return r * (2.0 - x * r)


def _ds(start, size, align=8):
    return pl.ds(pl.multiple_of(start, align), size)


def _kernel(
    q_hbm, k_hbm, v_hbm, shift_ref, h_hbm, d_ref,
    x_hbm, wq_hbm, wk_hbm, wv_hbm, wo_hbm, beta_ref, gf_hbm, gi_hbm,
    out_hbm,
    x_b, wq_b, wk_b, wv_b, wo_b, k_b, v_b, h_b, q_b, gf_v, gi_v,
    oa0_b, oa1_b, oa2_b, oa3_b, oa4_b, ob_b,
    wt_v, ht_v, mx_v, mh_v, kv_v, par_v, yx_b, yh_b, u0_v, u1_v, u2_v, u3_v, u4_v,
    k0_b, k1_b, k2_b, k3_b, kg_v, qt_b, pqt_b, vt_b, ot_b, on0_v, on1_v, on2_v, on3_v,
    sa_v, ma_v, sb_v, mb_v, mem_v, gate_v, zero_s, sems,
):
    u_v = (u0_v, u1_v, u2_v, u3_v, u4_v)
    kt_b = (k0_b, k1_b, k2_b, k3_b)
    oa_b = (oa0_b, oa1_b, oa2_b, oa3_b, oa4_b)
    x_v, wq_v, wk_v, wv_v, wo_v = (r.bitcast(u32) for r in (x_b, wq_b, wk_b, wv_b, wo_b))
    k_v, v_v, h_v, q_v = (r.bitcast(u32) for r in (k_b, v_b, h_b, q_b))
    yx_v, yh_v = (r.bitcast(u32) for r in (yx_b, yh_b))
    oa_v = [r.bitcast(u32) for r in oa_b]
    kt_v = [r.bitcast(u32) for r in kt_b]
    qt_v, pqt_v, vt_v, ot_v = (r.bitcast(u32) for r in (qt_b, pqt_b, vt_b, ot_b))

    n_sem = [0]

    def group(pairs):
        sem = sems.at[n_sem[0]]
        n_sem[0] += 1
        return [pltpu.make_async_copy(src, dst, sem) for src, dst in pairs]

    def cols(t):
        return pl.ds(128 * t, 128)

    def weight(hbm, buf):
        return group([(hbm.at[:, cols(t)], buf.at[t]) for t in range(NT)])

    def xrows(r0, n):
        return group([(x_hbm.at[pl.ds(r0, n), cols(t)], x_b.at[t, pl.ds(r0, n)]) for t in range(NT)])

    c_wk = [group([(wk_hbm.at[:, cols(t)], wk_b.at[t])]) for t in range(NT)]
    c_wq, c_wv, c_wo = (weight(a, b) for a, b in ((wq_hbm, wq_b), (wv_hbm, wv_b), (wo_hbm, wo_b)))
    c_x = [xrows(SEG * s, SEG) for s in range(S // SEG)]
    c_h = [group([(h_hbm.at[cols(t)], h_b.at[t])]) for t in range(NT)]
    c_kv = [group([(k_hbm.at[:, cols(t)], k_b.at[t, pl.ds(16, S)]),
                   (v_hbm.at[:, cols(t)], v_b.at[t])]) for t in range(NT)]
    c_g = group([(gf_hbm, gf_v), (gi_hbm, gi_v)])
    c_q = group([(q_hbm.at[:, cols(t)], q_b.at[t]) for t in range(NT)])
    c_oa = [group([(oa_b[t].at[0], out_hbm.at[:, cols(t)])]) for t in range(NT)]
    c_ob = [group([(ob_b.at[t, pl.ds(128 * t0, 128 * (t1 - t0))],
                    out_hbm.at[pl.ds(128 * t0, 128 * (t1 - t0)), cols(NT + t)]) for t in range(NT)])
            for t0, t1 in OUT_CHUNKS]

    def start(cs):
        for c in cs:
            c.start()

    def wait(cs):
        for c in cs:
            c.wait()

    def wait_when(cond, cs):
        pl.when(cond)(lambda: wait(cs))

    for cs in (c_wk[0], c_x[0], *c_wk[1:], c_x[1], c_x[2], c_wq, c_x[3], c_wv, c_h[0], c_kv[0], c_h[1],
               c_kv[1], c_h[2], c_kv[2], c_h[3], c_kv[3], c_h[4], c_kv[4], c_g, c_q, c_wo):
        start(cs)

    sub8 = lax.broadcasted_iota(i32, (8, 128), 0)
    lane8 = lax.broadcasted_iota(i32, (8, 128), 1)

    zero_s[0] = 0
    zero_s[1] = 0
    zero_s[2] = 0
    taps = shift_ref[...].astype(f32)
    skip = d_ref[...].astype(f32).reshape(1, D)
    for t in range(NT):
        for j in range(4):
            par_v[t, j] = jnp.broadcast_to(taps[j:j + 1, 128 * t:128 * t + 128], (8, 128))
        par_v[t, 4] = jnp.where(sub8 == 0, skip[:, 128 * t:128 * t + 128], 0.0)
        k_v[t, 0:8, :] = jnp.zeros((8, 128), u32)
    beta = beta_ref[...].astype(f32).reshape(1, 4 * NG)
    gate = 1.0 / (1.0 + jnp.exp(-beta))
    for h in range(4 * NG):
        gate_v[h] = jnp.broadcast_to(gate[:, h:h + 1], (8, 128))

    q_scale = DH ** -0.5 * LOG2E

    def project_k(tile, ft, pace):
        parts = [x_v[kt, pl.ds(64 * tile, 64), :] for kt in range(NT)]
        parts[0] = pace.pace(parts[0], PACE0)
        k = _dot(_upk(jnp.concatenate(parts, axis=1)), _upk(wk_v[ft]))
        pace.note(k)
        kt_b[tile // 4][ft, pl.ds(128 * (tile % 4), 128), :] = k.astype(bf16)

    def project_qv(tile, ft, halves, pace):
        xt = _upk(jnp.concatenate([x_v[kt, _ds(tile * 64, 64), :] for kt in range(NT)], axis=1))
        lo, hi = 64 * halves[0], 64 * halves[-1] + 64
        parts = [wt_v[ft, kt, lo:hi, :] for kt in range(NT)]
        parts[0] = pace.pace(parts[0], PACE1)
        r = _dot_t(_upk(jnp.concatenate(parts, axis=1)), xt)
        pace.note(r)
        rows = pl.ds(128 * ft, 128)
        for i, half in enumerate(halves):
            y = r[128 * i:128 * i + 128]
            if half == 0:
                qt_b[tile, rows, :] = (y * q_scale).astype(bf16)
                pqt_b[tile, rows, :] = _phi(y).astype(bf16)
            else:
                vt_b[tile, rows, :] = y.astype(bf16)

    class Spare:
        def __init__(self, view, *idx):
            self.view, self.idx = view, idx
            view[(*idx, slice(0, 8), slice(None))] = jnp.zeros((8, 128), view.dtype)

        def word(self):
            return pltpu.bitcast(self.view[(*self.idx, _ds(zero_s[2], 8), slice(None))], u32)

        def release(self, value):
            self.view[(*self.idx, _ds(zero_s[2] + 8, 8), slice(None))] = pltpu.bitcast(value, self.view.dtype)

    sp_ht, sp_k, sp_kv = Spare(ht_v, NT), Spare(k_v, NT), Spare(kv_v, 2)
    sp_mx, sp_mh, sp_yx, sp_yh = Spare(mx_v, 2), Spare(mh_v, 2), Spare(yx_v, NT, 0), Spare(yh_v, NT, 0)
    sp_oa, sp_kt, sp_kg = [Spare(r, 1) for r in oa_v], [Spare(r, NT) for r in kt_v], Spare(kg_v, NG)
    sp_u, sp_wt = [Spare(u, 0, M1) for u in u_v], Spare(wt_v, NT, 0)

    heads = [(r, Spare(r, NT)) for r in (on0_v, on1_v, on2_v, on3_v)]

    def block(cost, src, dst, fn, *args):
        return (cost, functools.partial(fn, *args), src.release if src else None, dst.word)

    def transpose_filter(ct, t0, n):
        def one(t):
            ht_v[ct, _ds((t0 + t) * 64, 64), :] = _pk(_upk(h_v[ct, :, _ds((t0 + t) * 128, 128, 128)]).T)

        return [block(20, None, sp_ht, one, t) for t in range(n)]

    def transpose_weight(half, w_v):
        def one(ft, kt):
            wt_v[ft, kt, 64 * half:64 * half + 64, :] = _pk(_upk(w_v[ft, 64 * kt:64 * kt + 64, :]).T)

        return [block(20, None, sp_wt, one, ft, kt) for ft in range(NT) for kt in range(NT)]

    def align_keys(r0, r1):
        def one(r):
            rows = pl.ds(r, 16)
            lane = lax.broadcasted_iota(i32, (16, 128), 1)
            for g in range(NG):
                t, off = divmod(80 * g, 128)
                x = kt_v[r // 256][t, pl.ds(r % 256, 16), :]
                if off > 48:
                    x = jnp.where(lane >= off, x, kt_v[r // 256][t + 1, pl.ds(r % 256, 16), :])
                kg_v[g, rows, :] = pltpu.roll(x, 128 - off, 1) if off else x

        return [block(20, sp_kt[r // 256], sp_kg, one, r) for r in range(r0, r1, 16)]

    def merge(xs, ys):
        keyed = [((i + 0.5) / len(bs), n, b) for n, bs in enumerate((xs, ys)) for i, b in enumerate(bs)]
        return [b for _, _, b in sorted(keyed, key=lambda e: e[:2])]

    def forward_unit(ct, bb):
        r0 = pl.multiple_of(bb * 8, 8)

        def short_conv(n1):
            w = [par_v[ct, j] for j in range(4)]
            base = r0 + 32 * n1
            p0, p1, p2 = (k_v[ct, pl.ds(base + 8 - j, 8), :] for j in range(3))
            e0, o0, e1, o1, o2 = _even(p0), _odd(p0), _even(p1), _odd(p1), _odd(p2)
            vv = v_v[ct, _ds(base, 8), :]
            return ((w[0] * e0 + w[1] * o1 + w[2] * e1 + w[3] * o2) * _even(vv),
                    (w[0] * o0 + w[1] * e0 + w[2] * o1 + w[3] * e1) * _odd(vv))

        def park(mid, par, vals):
            for s, (re, im) in vals.items():
                mid[par, pl.ds(16 * s, 8), :] = re[1]
                mid[par, pl.ds(16 * s + 8, 8), :] = im[1]

        def conv(n1s):
            for n1 in n1s:
                for par, y in enumerate(short_conv(n1)):
                    kv_v[par, pl.ds(8 * n1, 8), :] = y

        def first_x(j, par):
            xs = [kv_v[par, _ds(8 * (j + 4 * m) + zero_s[2], 8), :] for m in range(8)]
            park(mx_v, par, _fwd_first(j, xs))

        def first_h(j, par):
            xs = [(_odd if par else _even)(ht_v[ct, _ds(r0 + 32 * (j + 4 * m), 8), :]) for m in range(8)]
            if par == 0 and j == 0:
                xs[0] = xs[0] + jnp.where(bb == 0, par_v[ct, 4], 0.0)
            park(mh_v, par, _fwd_first(j, xs))

        def second(mid, dst, par, subs):
            for s0, n, k0, dk in subs:
                zs = [((_FWD_MID_SIGNS[s][0], mid[par, _ds(16 * s + zero_s[2], 8), :]),
                       (_FWD_MID_SIGNS[s][1], mid[par, _ds(16 * s + 8 + zero_s[2], 8), :]))
                      for s in range(s0, s0 + n)]
                for i, (re, im) in enumerate(_fft(zs)):
                    y = jnp.concatenate([re[1], im[1]], axis=0).astype(bf16)
                    dst[ct, k0 + dk * i, _ds(bb * 32 + 16 * par, 16, 16), :] = y

        def seconds(mid, dst, sp_src, sp_dst):
            return [block(64 if len(subs) == 1 else 40, sp_src, sp_dst, second, mid, dst, par, subs)
                    for par in range(2) for subs in (_SUBS[0:1], _SUBS[1:2], _SUBS[2:3], _SUBS[3:5])]

        def firsts(fn, sp_src, sp_dst):
            return [block(105, sp_src, sp_dst, fn, j, par) for par in range(2) for j in range(4)]

        convs = [block(92, sp_k, sp_kv, conv, range(n, n + 4)) for n in range(0, M1, 4)]
        return (firsts(first_h, sp_ht, sp_mh) + convs + seconds(mh_v, yh_b, sp_mh, sp_yh)
                + firsts(first_x, sp_kv, sp_mx) + seconds(mx_v, yx_b, sp_mx, sp_yx))

    def pacer(blocks, slots, lead=0, free=0, lag=0):
        return _Pacer(sub8 < zero_s[2], blocks, slots, lead, free, lag)

    def phase0():
        def pieces(s, fts):
            return [functools.partial(project_k, 4 * s + j, ft) for ft in fts for j in range(4)]

        def run(blocks, todo, lead=0, free=0):
            pacer(blocks, len(todo) * 8 // PACE0, lead, free, LAG0).run(todo)

        wait(c_wk[0] + c_wk[1] + c_x[0])
        run([], pieces(0, range(2)))
        wait(c_wk[2] + c_wk[3] + c_wk[4])
        run([], pieces(0, range(2, NT)))
        wait(c_x[1])
        run(align_keys(0, 256), pieces(1, range(NT)))
        wait(c_x[2])
        run(align_keys(256, 384), pieces(2, range(2)), 1)
        wait(c_wq + c_x[3])
        run(merge(transpose_weight(0, wq_v), align_keys(384, 512)),
            pieces(2, range(2, NT)) + pieces(3, range(2)), 2)
        wait(c_wv + c_h[0])
        run(transpose_weight(1, wv_v) + transpose_filter(0, 0, 16), pieces(3, range(2, NT)), 2, 100)

    def phase1(i, c):
        ct = i // 2
        for t in range(NT - 1):
            wait_when(i == 2 * t, c_kv[t] + c_h[t + 1])
        blocks = transpose_filter(ct + 1, 8 * (i % 2), TR1)
        for u in range(2):
            blocks += forward_unit(ct, 2 * (i % 2) + u)
        blocks += transpose_filter(ct + 1, 8 * (i % 2) + TR1, 8 - TR1)
        pieces = [functools.partial(project_qv, 2 * i + j, ft, halves)
                  for j in range(2) for ft in range(NT) for halves in HALVES]
        pacer(blocks, 20 * 8 // PACE1, LEAD1, FREE1, LAG1).run(pieces)
        return c


    def spectral(ct, u_out, z):
        zs = {}

        def fwd(k1, pace):
            g = _upk(pace.pace(gf_v[k1], PACE2))
            x = _dot(g, _upk(yx_v[ct, k1]))
            h = _dot(g, _upk(yh_v[ct, k1]))
            rows = []
            for a in range(8):
                xr, xi = x[16 * a:16 * a + 8], x[16 * a + 8:16 * a + 16]
                hr, hi = h[16 * a:16 * a + 8], h[16 * a + 8:16 * a + 16]
                rows += [xr * hr - xi * hi, xr * hi + xi * hr]
            pace.note(x)
            zs[k1] = jnp.concatenate(rows, axis=0).astype(bf16)

        def inv(k1, pace):
            u_out[z, k1] = _dot(_upk(pace.pace(gi_v[k1], PACE2)), zs.pop(k1))

        pieces = []
        for k1 in range(M1 + LOOK2):
            if k1 < M1:
                pieces.append(functools.partial(fwd, k1))
            if k1 >= LOOK2:
                pieces.append(functools.partial(inv, k1 - LOOK2))
        return pieces

    def inverse(ct, z):
        u_in = u_v[ct]

        def first(mid, a, subs):
            for s0, n, k0, dk in subs:
                zs = [((1, u_in[z, k, 16 * a:16 * a + 8, :]), (1, u_in[z, k, 16 * a + 8:16 * a + 16, :]))
                      for k in range(k0, M1, dk)]
                for i, (re, im) in enumerate(_ifft(zs)):
                    mid[a % 2, pl.ds(16 * (s0 + i), 8), :] = re[1]
                    mid[a % 2, pl.ds(16 * (s0 + i) + 8, 8), :] = im[1]

        def last(mid, bb, j, par):
            w = {s: ((_INV_MID_SIGNS[s][0], mid[par, _ds(16 * s + zero_s[2], 8), :]),
                     (_INV_MID_SIGNS[s][1], mid[par, _ds(16 * s + 8 + zero_s[2], 8), :]))
                 for s in _slots(j)}
            for m, (sign, y) in enumerate(_inv_last(j, w)):
                n1 = j + 4 * m
                if par == 0:
                    kv_v[0, pl.ds(8 * n1, 8), :] = y
                    continue
                gate_q = _upk(q_v[ct, pl.ds(32 * n1 + 8 * bb, 8), :]).astype(f32)
                y = jnp.concatenate([kv_v[0, _ds(8 * n1 + zero_s[2], 8), :], y], axis=0) * gate_q
                oa_b[ct][0, pl.ds(64 * n1 + 16 * bb, 16), :] = (y if sign > 0 else -y).astype(bf16)

        blocks = []
        for bb in range(4):
            mid, sp_mid = (mh_v, sp_mh) if bb % 2 else (mx_v, sp_mx)
            blocks += [block(56 if len(subs) == 1 else 32, sp_u[ct], sp_mid, first, mid, a, subs)
                       for a in (2 * bb, 2 * bb + 1)
                       for subs in (_SUBS[0:1], _SUBS[1:2], _SUBS[2:3], _SUBS[3:5])]
            blocks += [block(125 if par else 85, sp_mid, sp_oa[ct] if par else sp_kv, last, mid, bb, j, par)
                       for par in range(2) for j in range(4)]
        return blocks

    def stream(cts, z):
        return [piece for ct in cts for piece in spectral(ct, u_v[ct], z)]

    def phase2():
        wait(c_kv[NT - 1] + c_g + c_q)
        z0, z1 = zero_s[0], zero_s[1]
        slots = 64 * 8 // PACE2
        blocks = [b for bb in range(4) for b in forward_unit(NT - 1, bb)]
        pacer(blocks, NF2 * slots, LEAD2, 0, LAG2F).run(stream(range(NF2), z0))
        blocks = [b for ct in range(NI2) for b in inverse(ct, z1)]
        blocks = merge(blocks, align_keys(512, 1024))
        pacer(blocks, (NT - NF2) * slots, 0, FREE2, LAG2).run(stream(range(NF2, NT), z0))
        start([c for ct in range(NI2) for c in c_oa[ct]])

    prow = lax.broadcasted_iota(i32, (16, 128), 0)
    base = {3: 0, 2: 4, 1: 7, 0: 9}
    steps = [(j, t) for j in (3, 2, 1, 0) for t in range(j + 1)]

    def attend(uq, s_out, m_out, zo, up, s_in, m_in, zi, memory, pace=None):
        ri = lax.broadcasted_iota(i32, (128, 128), 0)
        ci = lax.broadcasted_iota(i32, (128, 128), 1)
        bias = jnp.where(ri <= ci, 0.0, -1e9 * LOG2E).astype(f32)
        if uq is not None:
            sq, gq = uq // NG, uq % NG
        if up is not None:
            sp, gp = up // NG, up % NG
            gates = [gate_v[4 * gp + i] for i in range(4)]
        weights, run_max, acc = {}, {}, {}

        def q_weights(j):
            if j not in weights:
                ws = []
                for i in range(4):
                    own = (prow >= 2 * i) & (prow < 2 * i + 10)
                    qw = jnp.where(own, qt_v[4 * sq + j, _ds(40 * gq + 8 * i, 16), :], jnp.uint32(0))
                    parts = [jnp.zeros((8 * i, 128), u32)] if i else []
                    ws.append(jnp.concatenate(parts + [qw, jnp.zeros((48 - 8 * i, 128), u32)], axis=0))
                weights[j] = _upk(jnp.concatenate(ws, axis=1))
            return weights[j]

        def v_rows(i, t):
            free = prow >= 12 if i < 2 else prow < 4
            return _upk(jnp.where(free, jnp.uint32(0x3F803F80), vt_v[4 * sp + t, _ds(40 * gp + 8 * i, 16), :]))

        if memory:
            prev = 4 * (sp - 1)
            upd = None
            for t in range(4):
                pk_t = _phi(_upk(kg_v[gp, _ds((prev + t) * 64, 64), :]).astype(f32)).astype(bf16)
                lhs = jnp.concatenate([vt_v[prev + t, _ds(40 * gp, 40), :],
                                       jnp.full((8, 128), 0x3F803F80, u32)], axis=0)
                d = _dot(_upk(lhs), pk_t)
                upd = d if upd is None else upd + d
            m = mem_v[gp] + upd[:88]
            mem_v[gp] = m
            own = [(lane8 >= DH * i) & (lane8 < DH * i + DH) for i in range(4)]
            rows = []
            for r in range(10):
                lo, hi = (8 * r) // DH, (8 * r + 7) // DH
                blk = m[8 * r:8 * r + 8]
                a = jnp.where(own[lo], blk * gates[lo], 0.0)
                if hi != lo:
                    a = jnp.where(sub8 < 4, a, jnp.where(own[hi], blk * gates[hi], 0.0))
                rows.append(a)
            rows += [jnp.where(own[i], m[80:88], 0.0) for i in range(4)]
            mem_lhs = jnp.concatenate(rows, axis=0).astype(bf16)

        def memory_read(j):
            w = jnp.concatenate([pqt_v[4 * sp + j, _ds(40 * gp, 40), :], jnp.zeros((24, 128), u32)], axis=0)
            r = _dot(mem_lhs, _upk(w))
            inv = [_recip(r[80 + 8 * i:88 + 8 * i] + 1e-6) for i in range(4)]
            rows = []
            for b in range(10):
                lo, hi = (8 * b) // DH, (8 * b + 7) // DH
                rows.append(r[8 * b:8 * b + 8] * (inv[lo] if lo == hi else jnp.where(sub8 < 4, inv[lo], inv[hi])))
            return rows

        def finish(j):
            a = []
            for i in range(4):
                o = acc[(j, i)]
                r = _recip(o[24:32] if i < 2 else o[0:8]) * (1.0 - gates[i])
                a.append([o[8 * b:8 * b + 8] * r for b in range(4)])
            low = sub8 < 4
            rows = [a[0][0], a[0][1], jnp.where(low, a[0][2], a[1][0]), a[1][1], a[1][2],
                    a[2][1], a[2][2], jnp.where(low, a[2][3], a[3][1]), a[3][2], a[3][3]]
            if memory:
                rows = [x + y for x, y in zip(rows, memory_read(j))]
            ot_b[4 * sp + j, _ds(80 * gp, 80, 16), :] = jnp.concatenate(rows, axis=0).astype(bf16)

        for j, t in steps:
            if uq is not None:
                keys = kg_v[gq, _ds(256 * sq + 64 * t, 64), :]
                keys = _upk(pace.pace(keys, 2) if pace else keys)
                logits = _dot(keys, q_weights(j))
                if pace:
                    pace.note(logits[:, :128])
            if up is not None:
                ps = [jnp.exp2(s_in[zi, i, base[j] + t].reshape(16, 8, 128) - m_in[zi, j, i][None])
                      .reshape(128, 128).astype(bf16) for i in range(4)]
            if uq is not None:
                for i in range(4):
                    st = logits[:, 128 * i:128 * i + 128]
                    if t == j:
                        st = st + bias
                    s_out[zo, i, base[j] + t] = st
                    mx = jnp.max(st.reshape(16, 8, 128), axis=0)
                    run_max[(j, i)] = mx if t == 0 else jnp.maximum(run_max[(j, i)], mx)
                    if t == j:
                        m_out[zo, j, i] = jnp.broadcast_to(
                            jnp.max(run_max[(j, i)], axis=0, keepdims=True), (8, 128))
            if up is not None:
                for i in range(4):
                    d = _dot(v_rows(i, t), ps[i])
                    acc[(j, i)] = d if t == 0 else acc[(j, i)] + d
                if t == j:
                    finish(j)

    def phase3_first():
        mem_v[...] = jnp.zeros(mem_v.shape, f32)
        z0, z1 = zero_s[0], zero_s[1]
        pacer(inverse(NI2, z1), 40, 0, 0, 2).run(
            [lambda p: attend(0, sa_v, ma_v, z0, None, None, None, None, False, p)])
        start(c_oa[NI2])

    def attend_pair(memory, last=False):
        def body(i, c):
            z0, z1 = zero_s[0], zero_s[1]
            attend(2 * i + 1, sb_v, mb_v, z0, 2 * i, sa_v, ma_v, z1, memory)
            attend(None if last else 2 * i + 2, sa_v, ma_v, z0, 2 * i + 1, sb_v, mb_v, z1, memory)
            return c
        return body

    def transpose_heads(tile):
        on_v, sp_on = heads[tile // 4]

        def one(ft):
            rows = pl.ds(64 * (tile % 4), 64)
            on_v[ft, rows, :] = _pk(_upk(ot_v[tile, 64 * ft:64 * ft + 64, :]).T)

        return [block(20, None, sp_on, one, ft) for ft in range(NT)]

    def out_project(tile, nt, pace):
        on_v = heads[tile // 4][0]
        parts = [on_v[ft, _ds(64 * (tile % 4) + zero_s[0], 64), :] for ft in range(NT)]
        parts[0] = pace.pace(parts[0], PACE4)
        y = _dot(_upk(jnp.concatenate(parts, axis=1)), _upk(wo_v[nt]))
        pace.note(y)
        ob_b[nt, pl.ds(128 * tile, 128), :] = y.astype(bf16)

    def phase4():
        wait(c_wo)
        cts = list(range(NI2 + 1, NT))
        for tile in range(4):
            for b in transpose_heads(tile):
                b[1]()
        for n, (t0, t1) in enumerate(OUT_CHUNKS):
            nxt = OUT_CHUNKS[n + 1] if n + 1 < len(OUT_CHUNKS) else (0, 0)
            blocks = [b for t in range(max(nxt[0], 4), nxt[1]) for b in transpose_heads(t)]
            mine = cts[len(cts) * n // NS4:len(cts) * (n + 1) // NS4] if n < NS4 else []
            blocks = merge(blocks, [b for ct in mine for b in inverse(ct, zero_s[1])])
            pacer(blocks, (t1 - t0) * NT * 8 // PACE4, 0, FREE4, LAG4).run(
                [functools.partial(out_project, t, nt) for t in range(t0, t1) for nt in range(NT)])
            start([c for ct in mine for c in c_oa[ct]] + c_ob[n])

    phase0()
    lax.fori_loop(0, 2 * (NT - 1), phase1, 0)
    phase2()
    phase3_first()
    lax.fori_loop(0, 4, attend_pair(False), 0)
    lax.fori_loop(4, 15, attend_pair(True), 0)
    attend_pair(True, last=True)(15, 0)
    phase4()
    for cs in c_oa + c_ob:
        wait(cs)


@jax.jit
def pallas_concat_heads__ssm_conv_h3__memory_aug_infini_attn__prompt_kernel(
    A_q: jax.Array,
    A_k: jax.Array,
    A_v: jax.Array,
    A_shift_k: jax.Array,
    A_ssm_k: jax.Array,
    A_ssm_D: jax.Array,
    B_x: jax.Array,
    B_wq: jax.Array,
    B_wk: jax.Array,
    B_wv: jax.Array,
    B_wo: jax.Array,
    B_beta: jax.Array,
):
    hbm = pl.BlockSpec(memory_space=pl.ANY)
    vmem = pl.BlockSpec(memory_space=pltpu.VMEM)
    V = pltpu.VMEM
    scratch = [
        V((NT, S, 128), bf16),
        V((NT, D, 128), bf16), V((NT, D, 128), bf16),
        V((NT, D, 128), bf16), V((NT, D, 128), bf16),
        V((NT + 1, S + 16, 128), bf16), V((NT, S, 128), bf16),
        V((NT, 128, S), bf16), V((NT, S, 128), bf16),
        V((M1, 64, 128), u32), V((M1, 64, 128), u32),
        *[V((2, S, 128), bf16)] * NT, V((NT, S, 128), bf16),
        V((NT + 1, NT, 128, 128), u32),
        V((NT + 1, S // 2, 128), u32),
        V((3, 16 * M1, 128), f32), V((3, 16 * M1, 128), f32),
        V((3, 8 * M1, 128), f32),
        V((NT, 5, 8, 128), f32),
        V((NT + 1, M1, 128, 128), bf16), V((NT + 1, M1, 128, 128), bf16),
        *[V((1, M1 + 1, 128, 128), f32)] * NT,
        *[V((NT + 1, SEG, 128), bf16)] * 4,
        V((NG + 1, S // 2, 128), u32),
        V((16, D, 128), bf16), V((16, D, 128), bf16),
        V((16, D, 128), bf16), V((16, D, 128), bf16),
        *[V((NT + 1, SEG // 2, 128), u32)] * 4,
        V((1, 4, 10, 128, 128), f32), V((1, 4, 4, 8, 128), f32),
        V((1, 4, 10, 128, 128), f32), V((1, 4, 4, 8, 128), f32),
        V((NG, 88, 128), f32),
        V((4 * NG, 8, 128), f32),
        pltpu.SMEM((3,), i32),
        pltpu.SemaphoreType.DMA((40,)),
    ]
    out = pl.pallas_call(
        _kernel,
        out_shape=jax.ShapeDtypeStruct((S, 2 * D), bf16),
        in_specs=[hbm, hbm, hbm, vmem, hbm, vmem, hbm, hbm, hbm, hbm, hbm, vmem, hbm, hbm],
        out_specs=hbm,
        scratch_shapes=scratch,
        compiler_params=pltpu.CompilerParams(vmem_limit_bytes=110 * 2**20),
    )(
        A_q.reshape(S, D), A_k.reshape(S, D), A_v.reshape(S, D), A_shift_k.T, A_ssm_k, A_ssm_D,
        B_x.reshape(S, D), B_wq, B_wk, B_wv, B_wo, B_beta, _G_FWD, _G_INV,
    )
    return out.reshape(1, S, 2 * D)
```

```python
import functools
import itertools
import math

import jax
import jax.numpy as jnp
import ml_dtypes
import numpy as np
from jax import lax
from jax.experimental import pallas as pl
from jax.experimental.pallas import tpu as pltpu

S = 2048
D = 640
NT = D // 128
DH = 20
NG = 8
SEG = 512
M1, M2 = 32, 64

bf16 = jnp.bfloat16
f32 = jnp.float32
u32 = jnp.uint32
i32 = jnp.int32

LOG2E = math.log2(math.e)
Q_SCALE = DH ** -0.5 * LOG2E
PACE0 = 4
X_CHUNKS = ((0, 2), (2, 6), (6, 10), (10, 12), (12, 16))
K_FIRST = (0, 2, 6, 10)
UNROLL1 = 1
PACE1 = 1
LEAD1 = 6
FREE1 = 300
LAG1 = 2
HALVES = ((0,), (1,))
PACE2 = 4
LEAD2 = 4
FREE2 = 0
LOOK2 = 5
LAG2 = 4
LAG2F = 4
NF2 = 3
NI2 = 1
NS4 = 3
UNROLL3 = 2
PACE4 = 4
FREE4 = 0
LEAD4 = 0
FILL4 = 10
OUT_CHUNKS = ((0, 4), (4, 8), (8, 12), (12, 15), (15, 16))
LAG4 = 0


def _neg(a):
    return None if a is None else (-a[0], a[1])


def _add(a, b):
    if a is None:
        return b
    if b is None:
        return a
    if a[0] == b[0]:
        return (a[0], a[1] + b[1])
    if a[0] > 0:
        return (1, a[1] - b[1])
    return (1, b[1] - a[1])


def _sub(a, b):
    return _add(a, _neg(b))


def _scale(a, c):
    if a is None or abs(c) < 1e-12:
        return None
    if abs(abs(c) - 1.0) < 1e-12:
        return a if c > 0 else _neg(a)
    return (a[0], a[1] * float(c))


def _cmul(z, ang):
    c, s = math.cos(ang), math.sin(ang)
    x, y = z
    if x is not None and y is not None and abs(abs(c) - abs(s)) < 1e-12:
        r = 1.0 if c * s > 0 else -1.0
        if r > 0:
            return (_scale(_sub(x, y), c), _scale(_add(y, x), c))
        return (_scale(_add(x, y), c), _scale(_sub(y, x), c))
    return (_sub(_scale(x, c), _scale(y, s)), _add(_scale(y, c), _scale(x, s)))


def _cadd(a, b):
    return (_add(a[0], b[0]), _add(a[1], b[1]))


def _csub(a, b):
    return (_sub(a[0], b[0]), _sub(a[1], b[1]))


def _dif_step(a, b, c, d, j, n):
    t1, t2 = _csub(a, c), _csub(b, d)
    mi_t2 = (t2[1], _neg(t2[0]))
    return (_cadd(a, c), _cadd(b, d),
            _cmul(_cadd(t1, mi_t2), -2 * math.pi * j / n),
            _cmul(_csub(t1, mi_t2), -6 * math.pi * j / n))


def _dit_step(e0, e1, o1, o3, j, n):
    a, b = _cmul(o1, 2 * math.pi * j / n), _cmul(o3, 6 * math.pi * j / n)
    s, d = _cadd(a, b), _csub(a, b)
    i_d = (_neg(d[1]), d[0])
    return _cadd(e0, s), _cadd(e1, i_d), _csub(e0, s), _csub(e1, i_d)


def _fft(z):
    n = len(z)
    if n == 1:
        return list(z)
    if n == 2:
        return [_cadd(z[0], z[1]), _csub(z[0], z[1])]
    q = n // 4
    steps = [_dif_step(*z[j::q], j, n) for j in range(q)]
    out = [None] * n
    out[0::2] = _fft([s[0] for s in steps] + [s[1] for s in steps])
    out[1::4] = _fft([s[2] for s in steps])
    out[3::4] = _fft([s[3] for s in steps])
    return out


def _ifft(z):
    n = len(z)
    if n == 1:
        return list(z)
    if n == 2:
        return [_cadd(z[0], z[1]), _csub(z[0], z[1])]
    q = n // 4
    e, o1, o3 = _ifft(z[0::2]), _ifft(z[1::4]), _ifft(z[3::4])
    out = [None] * n
    for j in range(q):
        out[j::q] = _dit_step(e[j], e[j + q], o1[j], o3[j], j, n)
    return out


_SUBS = ((0, 8, 0, 4), (8, 8, 1, 4), (16, 8, 3, 4), (24, 4, 2, 8), (28, 4, 6, 8))


def _fwd_first(j, xs):
    z = [_cmul(((1, x), None), -2 * math.pi * (j + 4 * m) / (4 * M1)) for m, x in enumerate(xs)]
    lo, hi = _dif_step(*z[0::2], j, 32), _dif_step(*z[1::2], j + 4, 32)
    mid = _dif_step(lo[0], hi[0], lo[1], hi[1], j, 16)
    return {j: mid[0], j + 4: mid[1], 8 + j: lo[2], 12 + j: hi[2],
            16 + j: lo[3], 20 + j: hi[3], 24 + j: mid[2], 28 + j: mid[3]}


def _inv_last(j, w):
    mid = _dit_step(w[j], w[j + 4], w[24 + j], w[28 + j], j, 16)
    lo = _dit_step(mid[0], mid[2], w[8 + j], w[16 + j], j, 32)
    hi = _dit_step(mid[1], mid[3], w[12 + j], w[20 + j], j + 4, 32)
    z = [None] * 8
    z[0::2], z[1::2] = lo, hi
    return [_cmul(v, 2 * math.pi * (j + 4 * m) / (4 * M1))[0] for m, v in enumerate(z)]


def _slots(j):
    return (j, j + 4, 8 + j, 12 + j, 16 + j, 20 + j, 24 + j, 28 + j)


def _codelet_signs():
    one = (1, 1.0)
    mid = {}
    for j in range(4):
        mid.update(_fwd_first(j, [1.0] * 8))
    mid = {s: (v[0][0], v[1][0]) for s, v in mid.items()}
    out = {}
    for s0, n, k0, dk in _SUBS:
        ys = _fft([((mid[s0 + i][0], 1.0), (mid[s0 + i][1], 1.0)) for i in range(n)])
        out.update({k0 + dk * i: (y[0][0], y[1][0]) for i, y in enumerate(ys)})
    imid = {}
    for s0, n, _, _ in _SUBS:
        imid.update({s0 + i: (w[0][0], w[1][0]) for i, w in enumerate(_ifft([(one, one)] * n))})
    return mid, out, imid


_FWD_MID_SIGNS, _FWD_SIGNS, _INV_MID_SIGNS = _codelet_signs()


class _Pacer:
    def __init__(self, never, blocks, slots, lead=0, free=0, lag=2):
        self.never, self.blocks, self.slots, self.lag = never, list(blocks), slots - lead, lag
        self.total = sum(b[0] for b in self.blocks) - free
        self.slot, self.spent, self.results = -lead, 0, []

    def note(self, result):
        self.results.append(result[:8])

    def _run_block(self):
        cost, fn, release, word = self.blocks.pop(0)
        self.spent += cost
        if release is not None and len(self.results) >= self.lag > 0:
            release(self.results[-self.lag])
        fn()
        return word

    def pace(self, x, every):
        parts = [x[8 * r:8 * r + 8] for r in range(x.shape[0] // 8)]
        for r in range(0, len(parts), every):
            self.slot += 1
            words = []
            while self.blocks and ((self.spent + self.blocks[0][0] / 2) * self.slots
                                   <= self.total * min(self.slot, self.slots)):
                word = self._run_block()
                if word not in words:
                    words.append(word)
            for word in words:
                parts[r] = jnp.where(self.never, word(), parts[r])
        return jnp.concatenate(parts, axis=0)

    def run(self, pieces):
        for piece in pieces:
            piece(self)
        while self.blocks:
            self._run_block()


def _pack_rows(m):
    b = np.asarray(m, np.float32).astype(ml_dtypes.bfloat16).view(np.uint16).astype(np.uint32)
    return np.ascontiguousarray(b[..., 0::2, :] | (b[..., 1::2, :] << 16))


def _dft_tables():
    r = np.arange(128)
    part = (r // 8) % 2
    nat = 8 * (r // 16) + r % 8
    eo = 16 * (r // 32) + 2 * (r % 8) + (r // 16) % 2
    fwd = np.zeros((M1, 128, 128))
    inv = np.zeros((M1, 128, 128))
    for k1 in range(M1):
        freq = k1 + M1 * nat + 0.25
        ph = 2 * np.pi * freq[:, None] * eo[None, :] / S
        same = part[:, None] == part[None, :]
        cross = np.where(part[:, None] == 0, 1.0, -1.0)
        sg = np.where(part == 0, _FWD_SIGNS[k1][0], _FWD_SIGNS[k1][1])
        fwd[k1] = np.where(same, np.cos(ph), cross * np.sin(ph)) * sg[None, :]
        ph = 2 * np.pi * nat[:, None] * freq[None, :] / S
        inv[k1] = np.where(same, np.cos(ph), -cross * np.sin(ph)) / S
    return _pack_rows(fwd), _pack_rows(inv)


_G_FWD, _G_INV = _dft_tables()


def _pk(x):
    return pltpu.bitcast(x, u32)


def _upk(x):
    return pltpu.bitcast(x, bf16)


_pk_mm = _pk


def _even(x):
    return pltpu.bitcast(x << 16, f32)


def _odd(x):
    return pltpu.bitcast(x & jnp.uint32(0xFFFF0000), f32)


def _dot(a, b):
    return lax.dot_general(a, b, (((1,), (0,)), ((), ())), preferred_element_type=f32)


def _dot_t(a, b):
    return lax.dot_general(a, b, (((1,), (1,)), ((), ())), preferred_element_type=f32)


def _phi(t):
    return jnp.where(t > 0, t + 1.0, jnp.exp2(t * LOG2E))


def _recip(x):
    r = pltpu.reciprocal(x, approx=True)
    return r * (2.0 - x * r)


def _ds(start, size, align=8):
    return pl.ds(pl.multiple_of(start, align), size)


def _kernel(
    q_hbm, k_hbm, v_hbm, shift_hbm, h_hbm, d_hbm,
    x_hbm, wq_hbm, wk_hbm, wv_hbm, wo_hbm, beta_hbm, gf_hbm, gi_hbm,
    out_hbm,
    x_b, wq_b, wk_b, wv_b, wo_b, k_b, v_b, h_b, q_b, gf_v, gi_v,
    oa0_b, oa1_b, oa2_b, oa3_b, oa4_b, ob_b,
    wt_v, ht_v, mx_v, mh_v, kv_v, par_v, yx_b, yh_b, u0_v, u1_v, u2_v, u3_v, u4_v,
    k0_b, k1_b, k2_b, k3_b, kg_v, qt_b, pqt_b, vt_v, ot_b, on0_v, on1_v, on2_v, on3_v,
    sa0_v, sa1_v, sa2_v, sa3_v, sb0_v, sb1_v, sb2_v, sb3_v, mem_v, gate_v, mask_v, shift_ref, d_ref, beta_ref, zero_s, sems,
):
    u_v = (u0_v, u1_v, u2_v, u3_v, u4_v)
    kt_b = (k0_b, k1_b, k2_b, k3_b)
    s_v = ((sa0_v, sa1_v, sa2_v, sa3_v), (sb0_v, sb1_v, sb2_v, sb3_v))
    oa_b = (oa0_b, oa1_b, oa2_b, oa3_b, oa4_b)
    x_v, wq_v, wk_v, wv_v, wo_v = (r.bitcast(u32) for r in (x_b, wq_b, wk_b, wv_b, wo_b))
    k_v, v_v, h_v, q_v = (r.bitcast(u32) for r in (k_b, v_b, h_b, q_b))
    yx_v, yh_v = (r.bitcast(u32) for r in (yx_b, yh_b))
    oa_v = [r.bitcast(u32) for r in oa_b]
    kt_v = [r.bitcast(u32) for r in kt_b]
    qt_v, pqt_v, ot_v = (r.bitcast(u32) for r in (qt_b, pqt_b, ot_b))

    n_sem = [0]

    def group(pairs):
        sem = sems.at[n_sem[0]]
        n_sem[0] += 1
        return [pltpu.make_async_copy(src, dst, sem) for src, dst in pairs]

    def cols(t):
        return pl.ds(128 * t, 128)

    def weight(hbm, buf):
        return group([(hbm.at[:, cols(t)], buf.at[t]) for t in range(NT)])

    def xrows(r0, n):
        return group([(x_hbm.at[pl.ds(r0, n), cols(t)], x_b.at[t, pl.ds(r0, n)]) for t in range(NT)])

    c_wk = [group([(wk_hbm.at[:, cols(t)], wk_b.at[t])]) for t in range(NT)]
    c_wq, c_wv, c_wo = (weight(a, b) for a, b in ((wq_hbm, wq_b), (wv_hbm, wv_b), (wo_hbm, wo_b)))
    c_x = [xrows(128 * t0, 128 * (t1 - t0)) for t0, t1 in X_CHUNKS]
    c_h = [group([(h_hbm.at[cols(t)], h_b.at[t])]) for t in range(NT)]
    c_kv = [group([(k_hbm.at[:, cols(t)], k_b.at[t, pl.ds(16, S)]),
                   (v_hbm.at[:, cols(t)], v_b.at[t])]) for t in range(NT)]
    c_g = group([(gf_hbm, gf_v), (gi_hbm, gi_v)])
    c_q = group([(q_hbm.at[:, cols(t)], q_b.at[t]) for t in range(NT)])
    c_oa = [group([(oa_b[t].at[0], out_hbm.at[:, cols(t)])]) for t in range(NT)]
    c_ob = [group([(ob_b.at[t, pl.ds(128 * t0, 128 * (t1 - t0))],
                    out_hbm.at[pl.ds(128 * t0, 128 * (t1 - t0)), cols(NT + t)]) for t in range(NT)])
            for t0, t1 in OUT_CHUNKS]

    def start(cs):
        for c in cs:
            c.start()

    def wait(cs):
        for c in cs:
            c.wait()

    def wait_when(cond, cs):
        pl.when(cond)(lambda: wait(cs))

    c_par = group([(shift_hbm, shift_ref), (d_hbm, d_ref), (beta_hbm, beta_ref)])
    start(c_x[0] + c_wk[0] + c_wk[1])

    sub8 = lax.broadcasted_iota(i32, (8, 128), 0)
    lane8 = lax.broadcasted_iota(i32, (8, 128), 1)

    zero_s[0] = 0
    zero_s[1] = 0
    zero_s[2] = 0

    def unpack_parameters():
        taps = shift_ref[...].astype(f32)
        skip = d_ref[...].astype(f32).reshape(1, D)
        for t in range(NT):
            for j in range(4):
                par_v[t, j] = jnp.broadcast_to(taps[j:j + 1, 128 * t:128 * t + 128], (8, 128))
            par_v[t, 4] = jnp.where(sub8 == 0, skip[:, 128 * t:128 * t + 128], 0.0)
            k_v[t, 0:8, :] = jnp.zeros((8, 128), u32)
        beta = beta_ref[...].astype(f32).reshape(1, 4 * NG)
        gate = 1.0 / (1.0 + jnp.exp(-beta))
        for h in range(4 * NG):
            gate_v[h] = jnp.broadcast_to(gate[:, h:h + 1], (8, 128))


    def key_buffer(tile):
        n = max(i for i, first in enumerate(K_FIRST) if first <= tile)
        return n, K_FIRST[n]

    def project_k(tile, ft, pace):
        parts = [x_v[kt, pl.ds(64 * tile, 64), :] for kt in range(NT)]
        parts[0] = pace.pace(parts[0], PACE0)
        k = _dot(_upk(jnp.concatenate(parts, axis=1)), _upk(wk_v[ft]))
        pace.note(k)
        n, first = key_buffer(tile)
        kt_b[n][ft, pl.ds(128 * (tile - first), 128), :] = k.astype(bf16)

    def project_qv(tile, ft, halves, pace):
        xt = _upk(jnp.concatenate([x_v[kt, _ds(tile * 64, 64), :] for kt in range(NT)], axis=1))
        lo, hi = 64 * halves[0], 64 * halves[-1] + 64
        parts = [wt_v[ft, kt, lo:hi, :] for kt in range(NT)]
        parts[0] = pace.pace(parts[0], PACE1)
        r = _dot_t(_upk(jnp.concatenate(parts, axis=1)), xt)
        pace.note(r)
        rows = pl.ds(128 * ft, 128)
        for i, half in enumerate(halves):
            y = r[128 * i:128 * i + 128]
            if half == 0:
                qt_b[tile, rows, :] = (y * Q_SCALE).astype(bf16)
                pqt_b[tile, rows, :] = _phi(y).astype(bf16)
            else:
                vt_v[tile, rows, :] = y

    class Spare:
        def __init__(self, view, *idx):
            self.view, self.idx = view, idx
            view[(*idx, slice(0, 8), slice(None))] = jnp.zeros((8, 128), view.dtype)

        def word(self):
            return pltpu.bitcast(self.view[(*self.idx, _ds(zero_s[2], 8), slice(None))], u32)

        def release(self, value):
            self.view[(*self.idx, _ds(zero_s[2] + 8, 8), slice(None))] = pltpu.bitcast(value, self.view.dtype)

    sp_ht, sp_k, sp_kv = Spare(ht_v, NT), Spare(k_v, NT), Spare(kv_v, 2)
    sp_mx, sp_mh, sp_yx, sp_yh = Spare(mx_v, 2), Spare(mh_v, 2), Spare(yx_v, NT, 0), Spare(yh_v, NT, 0)
    sp_oa, sp_kt, sp_kg = [Spare(r, 1) for r in oa_v], [Spare(r, NT) for r in kt_v], Spare(kg_v, NG)
    sp_u, sp_wt = [Spare(u, 0, M1) for u in u_v], Spare(wt_v, NT, 0)

    heads = [(r, Spare(r, NT)) for r in (on0_v, on1_v, on2_v, on3_v)]

    def block(cost, src, dst, fn, *args):
        return (cost, functools.partial(fn, *args), src.release if src else None, dst.word)

    def transpose_filter(ct, t0, n):
        def one(t):
            ht_v[ct, _ds((t0 + t) * 64, 64), :] = _pk(_upk(h_v[ct, :, _ds((t0 + t) * 128, 128, 128)]).T)

        return [block(20, None, sp_ht, one, t) for t in range(n)]

    def transpose_weight(half, w_v):
        def one(ft, kt):
            wt_v[ft, kt, 64 * half:64 * half + 64, :] = _pk(_upk(w_v[ft, 64 * kt:64 * kt + 64, :]).T)

        return [block(20, None, sp_wt, one, ft, kt) for ft in range(NT) for kt in range(NT)]

    def align_keys(tile0, tile1):
        def one(r):
            n, first = key_buffer(r // 64)
            rows = pl.ds(r - 64 * first, 16)
            lane = lax.broadcasted_iota(i32, (16, 128), 1)
            for g in range(NG):
                t, off = divmod(80 * g, 128)
                x = kt_v[n][t, rows, :]
                if off > 48:
                    x = jnp.where(lane >= off, x, kt_v[n][t + 1, rows, :])
                kg_v[g, pl.ds(r, 16), :] = pltpu.roll(x, 128 - off, 1) if off else x

        return [block(20, sp_kt[key_buffer(r // 64)[0]], sp_kg, one, r) for r in range(64 * tile0, 64 * tile1, 16)]

    def merge(xs, ys):
        keyed = [((i + 0.5) / len(bs), n, b) for n, bs in enumerate((xs, ys)) for i, b in enumerate(bs)]
        return [b for _, _, b in sorted(keyed, key=lambda e: e[:2])]

    def forward_unit(ct, bb):
        r0 = pl.multiple_of(bb * 8, 8)

        def short_conv(n1):
            w = [par_v[ct, j] for j in range(4)]
            base = r0 + 32 * n1
            p0, p1, p2 = (k_v[ct, pl.ds(base + 8 - j, 8), :] for j in range(3))
            e0, o0, e1, o1, o2 = _even(p0), _odd(p0), _even(p1), _odd(p1), _odd(p2)
            vv = v_v[ct, _ds(base, 8), :]
            return ((w[0] * e0 + w[1] * o1 + w[2] * e1 + w[3] * o2) * _even(vv),
                    (w[0] * o0 + w[1] * e0 + w[2] * o1 + w[3] * e1) * _odd(vv))

        def park(mid, par, vals):
            for s, (re, im) in vals.items():
                mid[par, pl.ds(16 * s, 8), :] = re[1]
                mid[par, pl.ds(16 * s + 8, 8), :] = im[1]

        def conv(n1s):
            for n1 in n1s:
                for par, y in enumerate(short_conv(n1)):
                    kv_v[par, pl.ds(8 * n1, 8), :] = y

        def first_x(j, par):
            xs = [kv_v[par, _ds(8 * (j + 4 * m) + zero_s[2], 8), :] for m in range(8)]
            park(mx_v, par, _fwd_first(j, xs))

        def first_h(j, par):
            xs = [(_odd if par else _even)(ht_v[ct, _ds(r0 + 32 * (j + 4 * m), 8), :]) for m in range(8)]
            if par == 0 and j == 0:
                xs[0] = xs[0] + jnp.where(bb == 0, par_v[ct, 4], 0.0)
            park(mh_v, par, _fwd_first(j, xs))

        def second(mid, dst, par, subs):
            for s0, n, k0, dk in subs:
                zs = [((_FWD_MID_SIGNS[s][0], mid[par, _ds(16 * s + zero_s[2], 8), :]),
                       (_FWD_MID_SIGNS[s][1], mid[par, _ds(16 * s + 8 + zero_s[2], 8), :]))
                      for s in range(s0, s0 + n)]
                for i, (re, im) in enumerate(_fft(zs)):
                    y = jnp.concatenate([re[1], im[1]], axis=0).astype(bf16)
                    dst[ct, k0 + dk * i, _ds(bb * 32 + 16 * par, 16, 16), :] = y

        def seconds(mid, dst, sp_src, sp_dst):
            return [block(64 if len(subs) == 1 else 40, sp_src, sp_dst, second, mid, dst, par, subs)
                    for par in range(2) for subs in (_SUBS[0:1], _SUBS[1:2], _SUBS[2:3], _SUBS[3:5])]

        def firsts(fn, sp_src, sp_dst):
            return [block(105, sp_src, sp_dst, fn, j, par) for par in range(2) for j in range(4)]

        convs = [block(92, sp_k, sp_kv, conv, range(n, n + 4)) for n in range(0, M1, 4)]
        return (firsts(first_h, sp_ht, sp_mh) + convs + seconds(mh_v, yh_b, sp_mh, sp_yh)
                + firsts(first_x, sp_kv, sp_mx) + seconds(mx_v, yx_b, sp_mx, sp_yx))

    def pacer(blocks, slots, lead=0, free=0, lag=0):
        return _Pacer(sub8 < zero_s[2], blocks, slots, lead, free, lag)

    def phase0():
        def run(blocks, chunk, fts, lead=0, free=0):
            todo = [functools.partial(project_k, tile, ft) for ft in fts for tile in range(*X_CHUNKS[chunk])]
            pacer(blocks, len(todo) * 8 // PACE0, lead, free, 0).run(todo)

        for cs in (*c_wk[2:], c_par):
            start(cs)
        wait(c_x[0] + c_wk[0] + c_wk[1])
        for cs in (c_x[1], c_x[2], c_wq):
            start(cs)
        run([], 0, range(2))
        wait(c_wk[2] + c_wk[3] + c_wk[4] + c_par)
        for cs in (c_x[3], c_wv, c_x[4], c_h[0], c_kv[0], c_h[1]):
            start(cs)
        unpack_parameters()
        run([], 0, range(2, NT))
        wait(c_x[1])
        for cs in (c_kv[1], c_h[2], c_kv[2], c_h[3], c_kv[3], c_h[4], c_kv[4], c_g, c_q, c_wo):
            start(cs)
        run(align_keys(0, 2), 1, range(NT))
        wait(c_x[2] + c_wq)
        run(merge(transpose_weight(0, wq_v), align_keys(2, 6)), 2, range(NT), 2)
        wait(c_x[3] + c_wv)
        run(merge(transpose_weight(1, wv_v), align_keys(6, 7)), 3, range(NT), 2)
        wait(c_x[4] + c_h[0])
        run(merge(transpose_filter(0, 0, 16), align_keys(7, 10)), 4, range(NT), 2)

    def phase1(i, c):
        n = UNROLL1
        for t in range(NT - 1):
            wait_when(i == 2 * t // n, c_kv[t] + c_h[t + 1])
        blocks, pieces = [], []
        for r in range(n):
            half = n * i + r
            ct, odd = half >> 1, half & 1
            ffts = [b for u in range(2) for b in forward_unit(ct, 2 * odd + u)]
            blocks += ffts + transpose_filter(ct + 1, 8 * odd, 8)
            pieces += [functools.partial(project_qv, 2 * half + j, ft, halves)
                       for j in range(2) for ft in range(NT) for halves in HALVES]
        pacer(blocks, n * 20 * 8 // PACE1, LEAD1, FREE1, LAG1).run(pieces)
        return c

    def spectral(ct, u_out, z):
        zs = {}

        def fwd(k1, pace):
            g = _upk(pace.pace(gf_v[k1], PACE2))
            x = _dot(g, _upk(yx_v[ct, k1]))
            h = _dot(g, _upk(yh_v[ct, k1]))
            rows = []
            for a in range(8):
                xr, xi = x[16 * a:16 * a + 8], x[16 * a + 8:16 * a + 16]
                hr, hi = h[16 * a:16 * a + 8], h[16 * a + 8:16 * a + 16]
                rows += [xr * hr - xi * hi, xr * hi + xi * hr]
            pace.note(x)
            zs[k1] = jnp.concatenate(rows, axis=0).astype(bf16)

        def inv(k1, pace):
            u_out[z, k1] = _dot(_upk(pace.pace(gi_v[k1], PACE2)), zs.pop(k1))

        pieces = []
        for k1 in range(M1 + LOOK2):
            if k1 < M1:
                pieces.append(functools.partial(fwd, k1))
            if k1 >= LOOK2:
                pieces.append(functools.partial(inv, k1 - LOOK2))
        return pieces

    def inverse(ct, z):
        u_in = u_v[ct]

        def first(mid, a, subs):
            for s0, n, k0, dk in subs:
                zs = [((1, u_in[z, k, 16 * a:16 * a + 8, :]), (1, u_in[z, k, 16 * a + 8:16 * a + 16, :]))
                      for k in range(k0, M1, dk)]
                for i, (re, im) in enumerate(_ifft(zs)):
                    mid[a % 2, pl.ds(16 * (s0 + i), 8), :] = re[1]
                    mid[a % 2, pl.ds(16 * (s0 + i) + 8, 8), :] = im[1]

        def last(mid, bb, j, par):
            w = {s: ((_INV_MID_SIGNS[s][0], mid[par, _ds(16 * s + zero_s[2], 8), :]),
                     (_INV_MID_SIGNS[s][1], mid[par, _ds(16 * s + 8 + zero_s[2], 8), :]))
                 for s in _slots(j)}
            for m, (sign, y) in enumerate(_inv_last(j, w)):
                n1 = j + 4 * m
                if par == 0:
                    kv_v[0, pl.ds(8 * n1, 8), :] = y
                    continue
                gate_q = _upk(q_v[ct, pl.ds(32 * n1 + 8 * bb, 8), :]).astype(f32)
                y = jnp.concatenate([kv_v[0, _ds(8 * n1 + zero_s[2], 8), :], y], axis=0) * gate_q
                oa_b[ct][0, pl.ds(64 * n1 + 16 * bb, 16), :] = (y if sign > 0 else -y).astype(bf16)

        blocks = []
        for bb in range(4):
            mid, sp_mid = (mh_v, sp_mh) if bb % 2 else (mx_v, sp_mx)
            blocks += [block(56 if len(subs) == 1 else 32, sp_u[ct], sp_mid, first, mid, a, subs)
                       for a in (2 * bb, 2 * bb + 1)
                       for subs in (_SUBS[0:1], _SUBS[1:2], _SUBS[2:3], _SUBS[3:5])]
            blocks += [block(125 if par else 85, sp_mid, sp_oa[ct] if par else sp_kv, last, mid, bb, j, par)
                       for par in range(2) for j in range(4)]
        return blocks

    def stream(cts, z):
        return [piece for ct in cts for piece in spectral(ct, u_v[ct], z)]

    def phase2():
        wait(c_kv[NT - 1] + c_g + c_q + c_wo)
        z0, z1 = zero_s[0], zero_s[1]
        slots = 64 * 8 // PACE2
        blocks = [b for bb in range(4) for b in forward_unit(NT - 1, bb)]
        pacer(blocks, NF2 * slots, LEAD2, 0, LAG2F).run(stream(range(NF2), z0))
        blocks = [b for ct in range(NI2) for b in inverse(ct, z1)]
        blocks = merge(blocks, align_keys(10, 16))
        pacer(blocks, (NT - NF2) * slots, 0, FREE2, LAG2).run(stream(range(NF2, NT), z0))
        start([c for ct in range(NI2) for c in c_oa[ct]])

    prow = lax.broadcasted_iota(i32, (16, 128), 0)
    steps = [(j, t) for j in (3, 2, 1, 0) for t in range(j + 1)]

    def fill_masks():
        key = lax.broadcasted_iota(i32, (64, 128), 0)
        lane = lax.broadcasted_iota(i32, (64, 128), 1)
        for n, query in enumerate((lane, (lane + 64) & 127, lane & 63)):
            mask_v[n] = jnp.where(key <= query, 0.0, -1e9 * LOG2E).astype(f32)

    def attend(uq, s_out, zo, up, s_in, zi, memory, pace=None, final=False, filler=None):
        low, left = sub8 < 4, lane8 < 64
        if uq is not None:
            sq, gq = uq >> 3, uq & 7
        if up is not None:
            sp, gp = up >> 3, up & 7
            gates = [gate_v[4 * gp + i] for i in range(4)]
        weights, run_max, acc = {}, {}, {}

        def stack(*parts):
            rows = sum(x.shape[0] for x in parts)
            return jnp.concatenate([x for x in parts if x.shape[0]] + [jnp.zeros((64 - rows, 128), u32)], axis=0)

        def q_weights(j):
            if j not in weights:
                qw = []
                for i in range(4):
                    own = (prow >= 2 * i) & (prow < 2 * i + 10)
                    w = qt_v[4 * sq + j, _ds(40 * gq + 8 * i, 16), :]
                    qw.append(jnp.where(own, pltpu.roll(w, 64, 1) if i % 2 else w, jnp.uint32(0)))
                single = [stack(jnp.zeros((8 * i, 128), u32), qw[i]) for i in range(4)]
                shared = []
                for i in (0, 2):
                    a, b = qw[i], qw[i + 1]
                    shared.append(stack(jnp.zeros((8 * i, 128), u32), jnp.where(left, 0, a[:8]),
                                        jnp.where(left, b[:8], a[8:]), jnp.where(left, b[8:], 0)))
                weights[j] = (_upk(jnp.concatenate(single, axis=1)), [_upk(w) for w in shared])
            return weights[j]

        def keys(t, r0, n):
            x = kg_v[gq, _ds(256 * sq + 64 * t + r0 // 2, n // 2), :]
            return _upk(pace.pace(x, 2) if pace else x)

        def column_max(x):
            return jnp.max(x.reshape(x.shape[0] // 8, 8, 128), axis=0)

        def score(j, t):
            single, shared = q_weights(j)
            if t < j:
                return _dot(keys(t, 0, 128), single), None
            main = _dot(keys(t, 0, 64), single)
            tail = [jnp.concatenate([_dot(keys(t, r, 32), w) for r in (64, 96)], axis=0) for w in shared]
            return main, tail

        def keep(j, t, main, tail):
            if pace:
                pace.note(main[:, :128])
            if tail is not None:
                tail = [x + mask_v[2] for x in tail]
                for n, x in enumerate(tail):
                    s_out[j][zo, 2 * n, pl.ds(128 * j + 64, 64)] = x
                tail = [column_max(x) for x in tail]
            for i in range(4):
                st = main[:, 128 * i:128 * i + 128]
                if t == j:
                    st = st + mask_v[i % 2]
                    s_out[j][zo, i, pl.ds(128 * j, 64)] = st
                else:
                    s_out[j][zo, i, pl.ds(128 * t, 128)] = st
                mx = column_max(st)
                run_max[j, i] = mx if t == 0 else jnp.maximum(run_max[j, i], mx)
                if t == j:
                    mine = left if i % 2 else ~left
                    mx = jnp.where(mine, jnp.maximum(run_max[j, i], tail[i // 2]), run_max[j, i])
                    s_out[j][zo, i, pl.ds(128 * j + 128, 8)] = jnp.broadcast_to(
                        jnp.max(mx, axis=0, keepdims=True), (8, 128))

        def expo(x, m):
            return jnp.exp2(x.reshape(x.shape[0] // 8, 8, 128) - m[None]).reshape(x.shape).astype(bf16)

        def probs(j, t):
            m = [s_in[j][zi, i, pl.ds(128 * j + 128, 8)] for i in range(4)]
            if t < j:
                return [expo(s_in[j][zi, i, pl.ds(128 * t, 128)], m[i]) for i in range(4)]
            ps = []
            half = lax.broadcasted_iota(i32, (32, 128), 1) < 64
            for i in (0, 2):
                tail = _pk_mm(expo(s_in[j][zi, i, pl.ds(128 * j + 64, 64)], jnp.where(left, m[i + 1], m[i])))
                for n, part in enumerate((jnp.where(half, 0, tail), jnp.where(half, tail, 0))):
                    main = expo(s_in[j][zi, i + n, pl.ds(128 * j, 64)], m[i + n])
                    ps.append(jnp.concatenate([main, _upk(part)], axis=0))
            return ps

        def v_rows(i, t):
            r0 = (0, 16, 40, 56)[i]
            v = [vt_v[4 * sp + t, _ds(80 * gp + r0 + 8 * b, 8), :] for b in range(3)]
            if i % 2:
                v[0] = jnp.where(low, 1.0, v[0])
            else:
                v[2] = jnp.where(low, v[2], 1.0)
            return jnp.concatenate(v, axis=0)

        if memory:
            prev = 4 * (sp - 1)
            upd = None
            for t in range(4):
                pk_t = _phi(_upk(kg_v[gp, _ds((prev + t) * 64, 64), :]).astype(f32)).astype(bf16)
                lhs = jnp.concatenate([vt_v[prev + t, _ds(80 * gp, 80), :], jnp.ones((8, 128), f32)], axis=0)
                d = _dot(lhs, pk_t)
                upd = d if upd is None else upd + d
            m = mem_v[gp] + upd
            mem_v[gp] = m
            own = [(lane8 >= DH * i) & (lane8 < DH * i + DH) for i in range(4)]
            rows = []
            for r in range(10):
                lo, hi = (8 * r) // DH, (8 * r + 7) // DH
                blk = m[8 * r:8 * r + 8]
                a = jnp.where(own[lo], blk * gates[lo], 0.0)
                if hi != lo:
                    a = jnp.where(low, a, jnp.where(own[hi], blk * gates[hi], 0.0))
                rows.append(a)
            rows += [jnp.where((low & own[i]) | (~low & own[i + 1]), m[80:88], 0.0) for i in (0, 2)]
            mem_lhs = jnp.concatenate(rows, axis=0).astype(bf16)

        def memory_read(j):
            w = jnp.concatenate([pqt_v[4 * sp + j, _ds(40 * gp, 40), :], jnp.zeros((24, 128), u32)], axis=0)
            r = _dot(mem_lhs, _upk(w))
            rows = []
            for n in range(2):
                inv = _recip(r[80 + 8 * n:88 + 8 * n] + 1e-6)
                swap = pltpu.roll(inv, 4, 0)
                scales = [jnp.where(low, inv, swap)] * 2 + [inv] + [jnp.where(low, swap, inv)] * 2
                rows += [r[40 * n + 8 * b:40 * n + 8 * b + 8] * scales[b] for b in range(5)]
            return rows

        def finish(j):
            rows = []
            for i in (0, 2):
                a, b = acc[j, i], pltpu.roll(acc[j, i + 1], 64, 1)
                inv = _recip(jnp.where(low, b[0:8], a[16:24])) * (1.0 - jnp.where(low, gates[i + 1], gates[i]))
                swap = pltpu.roll(inv, 4, 0)
                first, second = jnp.where(low, swap, inv), jnp.where(low, inv, swap)
                rows += [a[0:8] * first, a[8:16] * first, jnp.where(low, a[16:24], b[0:8]) * swap,
                         b[8:16] * second, b[16:24] * second]
            if memory:
                rows = [x + y for x, y in zip(rows, memory_read(j))]
            ot_b[4 * sp + j, _ds(80 * gp, 80, 16), :] = jnp.concatenate(rows, axis=0).astype(bf16)

        def weigh(j, t, ps):
            for i in range(4):
                d = _dot(v_rows(i, t), ps[i])
                acc[j, i] = d if t == 0 else acc[j, i] + d
            if t == j:
                finish(j)

        for n, (j, t) in enumerate(steps):
            if up is None:
                keep(j, t, *score(j, t))
            elif uq is None:
                filler()
                weigh(j, t, probs(j, t))
            elif final and not memory and n == len(steps) - 1:
                weigh(j, t, probs(j, t))
                keep(j, t, *score(j, t))
            else:
                scores = score(j, t)
                ps = probs(j, t)
                keep(j, t, *scores)
                weigh(j, t, ps)

    def phase3_first():
        mem_v[...] = jnp.zeros(mem_v.shape, f32)
        z0, z1 = zero_s[0], zero_s[1]
        pacer(inverse(NI2, z1), 36, 0, 0, 2).run(
            [lambda p: attend(0, s_v[0], z0, None, None, None, False, p)])
        start(c_oa[NI2])

    def attend_units(memory, filler=None):
        def body(i, c):
            for n in range(UNROLL3):
                unit, final = UNROLL3 * i + n, n == UNROLL3 - 1
                attend(None if filler and final else unit + 1, s_v[1 - n % 2], zero_s[0],
                       unit, s_v[n % 2], zero_s[1], memory, final=final, filler=filler)
            return c
        return body

    def transpose_heads(tile):
        on_v, sp_on = heads[tile // 4]

        def one(ft):
            rows = pl.ds(64 * (tile % 4), 64)
            on_v[ft, rows, :] = _pk(_upk(ot_v[tile, 64 * ft:64 * ft + 64, :]).T)

        return [block(20, None, sp_on, one, ft) for ft in range(NT)]

    def out_project(tile, nt, pace):
        on_v = heads[tile // 4][0]
        parts = [on_v[ft, _ds(64 * (tile % 4) + zero_s[0], 64), :] for ft in range(NT)]
        parts[0] = pace.pace(parts[0], PACE4)
        y = _dot(_upk(jnp.concatenate(parts, axis=1)), _upk(wo_v[nt]))
        pace.note(y)
        ob_b[nt, pl.ds(128 * tile, 128), :] = y.astype(bf16)

    def phase4():
        cts = list(range(NI2 + 1, NT))
        for n, (t0, t1) in enumerate(OUT_CHUNKS):
            nxt = OUT_CHUNKS[n + 1] if n + 1 < len(OUT_CHUNKS) else (0, 0)
            blocks = [b for t in range(*nxt) for b in transpose_heads(t)]
            mine = cts[len(cts) * n // NS4:len(cts) * (n + 1) // NS4] if n < NS4 else []
            blocks = merge(blocks, [b for ct in mine for b in inverse(ct, zero_s[1])])
            pace = pacer(blocks, (t1 - t0) * NT * 8 // PACE4, LEAD4 if n == 0 else 0, FREE4, LAG4)
            pieces = [functools.partial(out_project, t, nt) for t in range(t0, t1) for nt in range(NT)]
            if n == 0:
                count = itertools.count()
                attend_units(True, lambda: pieces.pop(0)(pace) if next(count) < FILL4 else None)(
                    4 * NG // UNROLL3 - 1, 0)
            pace.run(pieces)
            start([c for ct in mine for c in c_oa[ct]] + c_ob[n])

    fill_masks()
    phase0()
    lax.fori_loop(0, 2 * (NT - 1) // UNROLL1, phase1, 0)
    phase2()
    phase3_first()
    lax.fori_loop(0, NG // UNROLL3, attend_units(False), 0)
    lax.fori_loop(NG // UNROLL3, 4 * NG // UNROLL3 - 1, attend_units(True), 0)
    for tile in range(*OUT_CHUNKS[0]):
        for b in transpose_heads(tile):
            b[1]()
    phase4()
    for cs in c_oa + c_ob:
        wait(cs)


@jax.jit
def pallas_concat_heads__ssm_conv_h3__memory_aug_infini_attn__prompt_kernel(
    A_q: jax.Array,
    A_k: jax.Array,
    A_v: jax.Array,
    A_shift_k: jax.Array,
    A_ssm_k: jax.Array,
    A_ssm_D: jax.Array,
    B_x: jax.Array,
    B_wq: jax.Array,
    B_wk: jax.Array,
    B_wv: jax.Array,
    B_wo: jax.Array,
    B_beta: jax.Array,
):
    hbm = pl.BlockSpec(memory_space=pl.ANY)
    V = pltpu.VMEM
    scratch = [
        V((NT, S, 128), bf16),
        V((NT, D, 128), bf16), V((NT, D, 128), bf16),
        V((NT, D, 128), bf16), V((NT, D, 128), bf16),
        V((NT + 1, S + 16, 128), bf16), V((NT, S, 128), bf16),
        V((NT, 128, S), bf16), V((NT, S, 128), bf16),
        V((M1, 64, 128), u32), V((M1, 64, 128), u32),
        *[V((2, S, 128), bf16)] * NT, V((NT, S, 128), bf16),
        V((NT + 1, NT, 128, 128), u32),
        V((NT + 1, S // 2, 128), u32),
        V((3, 16 * M1, 128), f32), V((3, 16 * M1, 128), f32),
        V((3, 8 * M1, 128), f32),
        V((NT, 5, 8, 128), f32),
        V((NT + 1, M1, 128, 128), bf16), V((NT + 1, M1, 128, 128), bf16),
        *[V((1, M1 + 1, 128, 128), f32)] * NT,
        *[V((NT + 1, 128 * n, 128), bf16) for n in (2, 4, 4, 6)],
        V((NG + 1, S // 2, 128), u32),
        V((16, D, 128), bf16), V((16, D, 128), bf16),
        V((16, D, 128), f32), V((16, D, 128), bf16),
        *[V((NT + 1, SEG // 2, 128), u32)] * 4,
        *[V((1, 4, 128 * j + 136, 128), f32) for j in range(4)] * 2,
        V((NG, 88, 128), f32),
        V((4 * NG, 8, 128), f32),
        V((3, 64, 128), f32),
        V((4, D), bf16), V((D,), bf16), V((4 * NG,), bf16),
        pltpu.SMEM((3,), i32),
        pltpu.SemaphoreType.DMA((48,)),
    ]
    out = pl.pallas_call(
        _kernel,
        out_shape=jax.ShapeDtypeStruct((S, 2 * D), bf16),
        in_specs=[hbm] * 14,
        out_specs=hbm,
        scratch_shapes=scratch,
        compiler_params=pltpu.CompilerParams(vmem_limit_bytes=110 * 2**20),
    )(
        A_q.reshape(S, D), A_k.reshape(S, D), A_v.reshape(S, D), A_shift_k.T, A_ssm_k, A_ssm_D,
        B_x.reshape(S, D), B_wq, B_wk, B_wv, B_wo, B_beta, _G_FWD, _G_INV,
    )
    return out.reshape(1, S, 2 * D)
```

```python
import functools
import itertools
import math

import jax
import jax.numpy as jnp
import ml_dtypes
import numpy as np
from jax import lax
from jax.experimental import pallas as pl
from jax.experimental.pallas import tpu as pltpu

S = 2048
D = 640
NT = D // 128
DH = 20
NG = 8
SEG = 512
M1, M2 = 32, 64

bf16 = jnp.bfloat16
f32 = jnp.float32
u32 = jnp.uint32
i32 = jnp.int32

LOG2E = math.log2(math.e)
Q_SCALE = DH ** -0.5 * LOG2E
PACE0 = 4
X_CHUNKS = ((0, 2), (2, 6), (6, 10), (10, 12), (12, 16))
K_FIRST = (0, 2, 6, 10)
UNROLL1 = 1
PACE1 = 1
LEAD1 = 6
FREE1 = 300
LAG1 = 2
HALVES = ((0,), (1,))
PACE2 = 4
LEAD2 = 4
FREE2 = 400
LOOK2 = 5
LAG2 = 4
LAG2F = 4
NF2 = 3
NI2 = 2
NK2 = 0
HOST4 = (0, 1, 2, 3, 3, 3)
UNROLL3 = 2
UPDATE3 = (0, 1, 1, 2)
PACE4 = 4
FREE4 = 0
LEAD4 = 0
FILL4 = 10
OUT_CHUNKS = ((0, 4), (4, 8), (8, 12), (12, 15), (15, 16))
LAG4 = 0


def _neg(a):
    return None if a is None else (-a[0], a[1])


def _add(a, b):
    if a is None:
        return b
    if b is None:
        return a
    if a[0] == b[0]:
        return (a[0], a[1] + b[1])
    if a[0] > 0:
        return (1, a[1] - b[1])
    return (1, b[1] - a[1])


def _sub(a, b):
    return _add(a, _neg(b))


def _scale(a, c):
    if a is None or abs(c) < 1e-12:
        return None
    if abs(abs(c) - 1.0) < 1e-12:
        return a if c > 0 else _neg(a)
    return (a[0], a[1] * float(c))


def _cmul(z, ang):
    c, s = math.cos(ang), math.sin(ang)
    x, y = z
    if x is not None and y is not None and abs(abs(c) - abs(s)) < 1e-12:
        r = 1.0 if c * s > 0 else -1.0
        if r > 0:
            return (_scale(_sub(x, y), c), _scale(_add(y, x), c))
        return (_scale(_add(x, y), c), _scale(_sub(y, x), c))
    return (_sub(_scale(x, c), _scale(y, s)), _add(_scale(y, c), _scale(x, s)))


def _cadd(a, b):
    return (_add(a[0], b[0]), _add(a[1], b[1]))


def _csub(a, b):
    return (_sub(a[0], b[0]), _sub(a[1], b[1]))


def _dif_step(a, b, c, d, j, n):
    t1, t2 = _csub(a, c), _csub(b, d)
    mi_t2 = (t2[1], _neg(t2[0]))
    return (_cadd(a, c), _cadd(b, d),
            _cmul(_cadd(t1, mi_t2), -2 * math.pi * j / n),
            _cmul(_csub(t1, mi_t2), -6 * math.pi * j / n))


def _dit_step(e0, e1, o1, o3, j, n):
    a, b = _cmul(o1, 2 * math.pi * j / n), _cmul(o3, 6 * math.pi * j / n)
    s, d = _cadd(a, b), _csub(a, b)
    i_d = (_neg(d[1]), d[0])
    return _cadd(e0, s), _cadd(e1, i_d), _csub(e0, s), _csub(e1, i_d)


def _fft(z):
    n = len(z)
    if n == 1:
        return list(z)
    if n == 2:
        return [_cadd(z[0], z[1]), _csub(z[0], z[1])]
    q = n // 4
    steps = [_dif_step(*z[j::q], j, n) for j in range(q)]
    out = [None] * n
    out[0::2] = _fft([s[0] for s in steps] + [s[1] for s in steps])
    out[1::4] = _fft([s[2] for s in steps])
    out[3::4] = _fft([s[3] for s in steps])
    return out


def _ifft(z):
    n = len(z)
    if n == 1:
        return list(z)
    if n == 2:
        return [_cadd(z[0], z[1]), _csub(z[0], z[1])]
    q = n // 4
    e, o1, o3 = _ifft(z[0::2]), _ifft(z[1::4]), _ifft(z[3::4])
    out = [None] * n
    for j in range(q):
        out[j::q] = _dit_step(e[j], e[j + q], o1[j], o3[j], j, n)
    return out


_SUBS = ((0, 8, 0, 4), (8, 8, 1, 4), (16, 8, 3, 4), (24, 4, 2, 8), (28, 4, 6, 8))


def _fwd_first(j, xs):
    z = [_cmul(((1, x), None), -2 * math.pi * (j + 4 * m) / (4 * M1)) for m, x in enumerate(xs)]
    lo, hi = _dif_step(*z[0::2], j, 32), _dif_step(*z[1::2], j + 4, 32)
    mid = _dif_step(lo[0], hi[0], lo[1], hi[1], j, 16)
    return {j: mid[0], j + 4: mid[1], 8 + j: lo[2], 12 + j: hi[2],
            16 + j: lo[3], 20 + j: hi[3], 24 + j: mid[2], 28 + j: mid[3]}


def _inv_last(j, w):
    mid = _dit_step(w[j], w[j + 4], w[24 + j], w[28 + j], j, 16)
    lo = _dit_step(mid[0], mid[2], w[8 + j], w[16 + j], j, 32)
    hi = _dit_step(mid[1], mid[3], w[12 + j], w[20 + j], j + 4, 32)
    z = [None] * 8
    z[0::2], z[1::2] = lo, hi
    return [_cmul(v, 2 * math.pi * (j + 4 * m) / (4 * M1))[0] for m, v in enumerate(z)]


def _slots(j):
    return (j, j + 4, 8 + j, 12 + j, 16 + j, 20 + j, 24 + j, 28 + j)


def _codelet_signs():
    one = (1, 1.0)
    mid = {}
    for j in range(4):
        mid.update(_fwd_first(j, [1.0] * 8))
    mid = {s: (v[0][0], v[1][0]) for s, v in mid.items()}
    out = {}
    for s0, n, k0, dk in _SUBS:
        ys = _fft([((mid[s0 + i][0], 1.0), (mid[s0 + i][1], 1.0)) for i in range(n)])
        out.update({k0 + dk * i: (y[0][0], y[1][0]) for i, y in enumerate(ys)})
    imid = {}
    for s0, n, _, _ in _SUBS:
        imid.update({s0 + i: (w[0][0], w[1][0]) for i, w in enumerate(_ifft([(one, one)] * n))})
    return mid, out, imid


_FWD_MID_SIGNS, _FWD_SIGNS, _INV_MID_SIGNS = _codelet_signs()


class _Pacer:
    def __init__(self, never, blocks, slots, lead=0, free=0, lag=2):
        self.never, self.blocks, self.slots, self.lag = never, list(blocks), slots - lead, lag
        self.total = sum(b[0] for b in self.blocks) - free
        self.slot, self.spent, self.results = -lead, 0, []

    def note(self, result):
        self.results.append(result[:8])

    def _run_block(self):
        cost, fn, release, word = self.blocks.pop(0)
        self.spent += cost
        if release is not None and len(self.results) >= self.lag > 0:
            release(self.results[-self.lag])
        fn()
        return word

    def pace(self, x, every):
        parts = [x[8 * r:8 * r + 8] for r in range(x.shape[0] // 8)]
        for r in range(0, len(parts), every):
            self.slot += 1
            words = []
            while self.blocks and ((self.spent + self.blocks[0][0] / 2) * self.slots
                                   <= self.total * min(self.slot, self.slots)):
                word = self._run_block()
                if word not in words:
                    words.append(word)
            for word in words:
                parts[r] = jnp.where(self.never, word(), parts[r])
        return jnp.concatenate(parts, axis=0)

    def run(self, pieces):
        for piece in pieces:
            piece(self)
        while self.blocks:
            self._run_block()


def _pack_rows(m):
    b = np.asarray(m, np.float32).astype(ml_dtypes.bfloat16).view(np.uint16).astype(np.uint32)
    return np.ascontiguousarray(b[..., 0::2, :] | (b[..., 1::2, :] << 16))


def _dft_tables():
    r = np.arange(128)
    part = (r // 8) % 2
    nat = 8 * (r // 16) + r % 8
    eo = 16 * (r // 32) + 2 * (r % 8) + (r // 16) % 2
    fwd = np.zeros((M1, 128, 128))
    inv = np.zeros((M1, 128, 128))
    for k1 in range(M1):
        freq = k1 + M1 * nat + 0.25
        ph = 2 * np.pi * freq[:, None] * eo[None, :] / S
        same = part[:, None] == part[None, :]
        cross = np.where(part[:, None] == 0, 1.0, -1.0)
        sg = np.where(part == 0, _FWD_SIGNS[k1][0], _FWD_SIGNS[k1][1])
        fwd[k1] = np.where(same, np.cos(ph), cross * np.sin(ph)) * sg[None, :]
        ph = 2 * np.pi * nat[:, None] * freq[None, :] / S
        inv[k1] = np.where(same, np.cos(ph), -cross * np.sin(ph)) / S
    return _pack_rows(fwd), _pack_rows(inv)


_G_FWD, _G_INV = _dft_tables()


def _pk(x):
    return pltpu.bitcast(x, u32)


def _upk(x):
    return pltpu.bitcast(x, bf16)


_pk_mm = _pk


def _even(x):
    return pltpu.bitcast(x << 16, f32)


def _odd(x):
    return pltpu.bitcast(x & jnp.uint32(0xFFFF0000), f32)


def _dot(a, b):
    return lax.dot_general(a, b, (((1,), (0,)), ((), ())), preferred_element_type=f32)


def _dot_t(a, b):
    return lax.dot_general(a, b, (((1,), (1,)), ((), ())), preferred_element_type=f32)


def _phi(t):
    return jnp.where(t > 0, t + 1.0, jnp.exp2(t * LOG2E))


def _recip(x):
    r = pltpu.reciprocal(x, approx=True)
    return r * (2.0 - x * r)


def _ds(start, size, align=8):
    return pl.ds(pl.multiple_of(start, align), size)


def _kernel(
    q_hbm, k_hbm, v_hbm, shift_hbm, h_hbm, d_hbm,
    x_hbm, wq_hbm, wk_hbm, wv_hbm, wo_hbm, beta_hbm, gf_hbm, gi_hbm,
    out_hbm,
    x_b, wq_b, wk_b, wv_b, wo_b, k_b, v_b, h_b, q_b, gf_v, gi_v,
    oa0_b, oa1_b, oa2_b, oa3_b, oa4_b, ob_b,
    wt_v, ht_v, mx_v, mh_v, kv_v, par_v, yx_b, yh_b, u0_v, u1_v, u2_v, u3_v, u4_v,
    k0_b, k1_b, k2_b, k3_b, kg_v, qt_b, pqt_b, vt_v, ot_b, on0_v, on1_v, on2_v, on3_v,
    sa0_v, sa1_v, sa2_v, sa3_v, sb0_v, sb1_v, sb2_v, sb3_v, mem_v, gate_v, mask_v, shift_ref, d_ref, beta_ref, zero_s, sems,
):
    u_v = (u0_v, u1_v, u2_v, u3_v, u4_v)
    kt_b = (k0_b, k1_b, k2_b, k3_b)
    s_v = ((sa0_v, sa1_v, sa2_v, sa3_v), (sb0_v, sb1_v, sb2_v, sb3_v))
    oa_b = (oa0_b, oa1_b, oa2_b, oa3_b, oa4_b)
    x_v, wq_v, wk_v, wv_v, wo_v = (r.bitcast(u32) for r in (x_b, wq_b, wk_b, wv_b, wo_b))
    k_v, v_v, h_v, q_v = (r.bitcast(u32) for r in (k_b, v_b, h_b, q_b))
    yx_v, yh_v = (r.bitcast(u32) for r in (yx_b, yh_b))
    oa_v = [r.bitcast(u32) for r in oa_b]
    kt_v = [r.bitcast(u32) for r in kt_b]
    qt_v, pqt_v, ot_v = (r.bitcast(u32) for r in (qt_b, pqt_b, ot_b))

    n_sem = [0]

    def group(pairs):
        sem = sems.at[n_sem[0]]
        n_sem[0] += 1
        return [pltpu.make_async_copy(src, dst, sem) for src, dst in pairs]

    def cols(t):
        return pl.ds(128 * t, 128)

    def weight(hbm, buf):
        return group([(hbm.at[:, cols(t)], buf.at[t]) for t in range(NT)])

    def xrows(r0, n):
        return group([(x_hbm.at[pl.ds(r0, n), cols(t)], x_b.at[t, pl.ds(r0, n)]) for t in range(NT)])

    c_wk = [group([(wk_hbm.at[:, cols(t)], wk_b.at[t])]) for t in range(NT)]
    c_wq, c_wv, c_wo = (weight(a, b) for a, b in ((wq_hbm, wq_b), (wv_hbm, wv_b), (wo_hbm, wo_b)))
    c_x = [xrows(128 * t0, 128 * (t1 - t0)) for t0, t1 in X_CHUNKS]
    c_h = [group([(h_hbm.at[cols(t)], h_b.at[t])]) for t in range(NT)]
    c_kv = [group([(k_hbm.at[:, cols(t)], k_b.at[t, pl.ds(16, S)]),
                   (v_hbm.at[:, cols(t)], v_b.at[t])]) for t in range(NT)]
    c_g = group([(gf_hbm, gf_v), (gi_hbm, gi_v)])
    c_q = group([(q_hbm.at[:, cols(t)], q_b.at[t]) for t in range(NT)])
    c_oa = [group([(oa_b[t].at[0], out_hbm.at[:, cols(t)])]) for t in range(NT)]
    c_ob = [group([(ob_b.at[t, pl.ds(128 * t0, 128 * (t1 - t0))],
                    out_hbm.at[pl.ds(128 * t0, 128 * (t1 - t0)), cols(NT + t)]) for t in range(NT)])
            for t0, t1 in OUT_CHUNKS]

    def start(cs):
        for c in cs:
            c.start()

    def wait(cs):
        for c in cs:
            c.wait()

    def wait_when(cond, cs):
        pl.when(cond)(lambda: wait(cs))

    c_par = group([(shift_hbm, shift_ref), (d_hbm, d_ref), (beta_hbm, beta_ref)])
    start(c_x[0] + c_wk[0] + c_wk[1])

    sub8 = lax.broadcasted_iota(i32, (8, 128), 0)
    lane8 = lax.broadcasted_iota(i32, (8, 128), 1)

    zero_s[0] = 0
    zero_s[1] = 0
    zero_s[2] = 0

    def unpack_parameters():
        taps = shift_ref[...].astype(f32)
        skip = d_ref[...].astype(f32).reshape(1, D)
        for t in range(NT):
            for j in range(4):
                par_v[t, j] = jnp.broadcast_to(taps[j:j + 1, 128 * t:128 * t + 128], (8, 128))
            par_v[t, 4] = jnp.where(sub8 == 0, skip[:, 128 * t:128 * t + 128], 0.0)
            k_v[t, 0:8, :] = jnp.zeros((8, 128), u32)
        beta = beta_ref[...].astype(f32).reshape(1, 4 * NG)
        gate = 1.0 / (1.0 + jnp.exp(-beta))
        for h in range(4 * NG):
            gate_v[h] = jnp.broadcast_to(gate[:, h:h + 1], (8, 128))


    def key_buffer(tile):
        n = max(i for i, first in enumerate(K_FIRST) if first <= tile)
        return n, K_FIRST[n]

    def project_k(tile, ft, pace):
        parts = [x_v[kt, pl.ds(64 * tile, 64), :] for kt in range(NT)]
        parts[0] = pace.pace(parts[0], PACE0)
        k = _dot(_upk(jnp.concatenate(parts, axis=1)), _upk(wk_v[ft]))
        pace.note(k)
        n, first = key_buffer(tile)
        kt_b[n][ft, pl.ds(128 * (tile - first), 128), :] = k.astype(bf16)

    def project_qv(tile, ft, halves, pace):
        xt = _upk(jnp.concatenate([x_v[kt, _ds(tile * 64, 64), :] for kt in range(NT)], axis=1))
        lo, hi = 64 * halves[0], 64 * halves[-1] + 64
        parts = [wt_v[ft, kt, lo:hi, :] for kt in range(NT)]
        parts[0] = pace.pace(parts[0], PACE1)
        r = _dot_t(_upk(jnp.concatenate(parts, axis=1)), xt)
        pace.note(r)
        rows = pl.ds(128 * ft, 128)
        for i, half in enumerate(halves):
            y = r[128 * i:128 * i + 128]
            if half == 0:
                qt_b[tile, rows, :] = (y * Q_SCALE).astype(bf16)
                pqt_b[tile, rows, :] = _phi(y).astype(bf16)
            else:
                vt_v[tile, rows, :] = y

    class Spare:
        def __init__(self, view, *idx):
            self.view, self.idx = view, idx
            view[(*idx, slice(0, 8), slice(None))] = jnp.zeros((8, 128), view.dtype)

        def word(self):
            return pltpu.bitcast(self.view[(*self.idx, _ds(zero_s[2], 8), slice(None))], u32)

        def release(self, value):
            self.view[(*self.idx, _ds(zero_s[2] + 8, 8), slice(None))] = pltpu.bitcast(value, self.view.dtype)

    sp_ht, sp_k, sp_kv = Spare(ht_v, NT), Spare(k_v, NT), Spare(kv_v, 2)
    sp_mx, sp_mh, sp_yx, sp_yh = Spare(mx_v, 2), Spare(mh_v, 2), Spare(yx_v, NT, 0), Spare(yh_v, NT, 0)
    sp_oa, sp_kt, sp_kg = [Spare(r, 1) for r in oa_v], [Spare(r, NT) for r in kt_v], Spare(kg_v, NG)
    sp_u, sp_wt = [Spare(u, 0, M1) for u in u_v], Spare(wt_v, NT, 0)

    heads = [(r, Spare(r, NT)) for r in (on0_v, on1_v, on2_v, on3_v)]

    def block(cost, src, dst, fn, *args):
        return (cost, functools.partial(fn, *args), src.release if src else None, dst.word)

    def transpose_filter(ct, t0, n):
        def one(t):
            ht_v[ct, _ds((t0 + t) * 64, 64), :] = _pk(_upk(h_v[ct, :, _ds((t0 + t) * 128, 128, 128)]).T)

        return [block(20, None, sp_ht, one, t) for t in range(n)]

    def transpose_weight(half, w_v):
        def one(ft, kt):
            wt_v[ft, kt, 64 * half:64 * half + 64, :] = _pk(_upk(w_v[ft, 64 * kt:64 * kt + 64, :]).T)

        return [block(20, None, sp_wt, one, ft, kt) for ft in range(NT) for kt in range(NT)]

    def align_keys(tile0, tile1):
        def one(r):
            n, first = key_buffer(r // 64)
            rows = pl.ds(r - 64 * first, 16)
            lane = lax.broadcasted_iota(i32, (16, 128), 1)
            for g in range(NG):
                t, off = divmod(80 * g, 128)
                x = kt_v[n][t, rows, :]
                if off > 48:
                    x = jnp.where(lane >= off, x, kt_v[n][t + 1, rows, :])
                kg_v[g, pl.ds(r, 16), :] = pltpu.roll(x, 128 - off, 1) if off else x

        return [block(20, sp_kt[key_buffer(r // 64)[0]], sp_kg, one, r) for r in range(64 * tile0, 64 * tile1, 16)]

    def merge(xs, ys):
        keyed = [((i + 0.5) / len(bs), n, b) for n, bs in enumerate((xs, ys)) for i, b in enumerate(bs)]
        return [b for _, _, b in sorted(keyed, key=lambda e: e[:2])]

    def forward_unit(ct, bb):
        r0 = pl.multiple_of(bb * 8, 8)

        def short_conv(n1):
            w = [par_v[ct, j] for j in range(4)]
            base = r0 + 32 * n1
            p0, p1, p2 = (k_v[ct, pl.ds(base + 8 - j, 8), :] for j in range(3))
            e0, o0, e1, o1, o2 = _even(p0), _odd(p0), _even(p1), _odd(p1), _odd(p2)
            vv = v_v[ct, _ds(base, 8), :]
            return ((w[0] * e0 + w[1] * o1 + w[2] * e1 + w[3] * o2) * _even(vv),
                    (w[0] * o0 + w[1] * e0 + w[2] * o1 + w[3] * e1) * _odd(vv))

        def park(mid, par, vals):
            for s, (re, im) in vals.items():
                mid[par, pl.ds(16 * s, 8), :] = re[1]
                mid[par, pl.ds(16 * s + 8, 8), :] = im[1]

        def conv(n1s):
            for n1 in n1s:
                for par, y in enumerate(short_conv(n1)):
                    kv_v[par, pl.ds(8 * n1, 8), :] = y

        def first_x(j, par):
            xs = [kv_v[par, _ds(8 * (j + 4 * m) + zero_s[2], 8), :] for m in range(8)]
            park(mx_v, par, _fwd_first(j, xs))

        def first_h(j, par):
            xs = [(_odd if par else _even)(ht_v[ct, _ds(r0 + 32 * (j + 4 * m), 8), :]) for m in range(8)]
            if par == 0 and j == 0:
                xs[0] = xs[0] + jnp.where(bb == 0, par_v[ct, 4], 0.0)
            park(mh_v, par, _fwd_first(j, xs))

        def second(mid, dst, par, subs):
            for s0, n, k0, dk in subs:
                zs = [((_FWD_MID_SIGNS[s][0], mid[par, _ds(16 * s + zero_s[2], 8), :]),
                       (_FWD_MID_SIGNS[s][1], mid[par, _ds(16 * s + 8 + zero_s[2], 8), :]))
                      for s in range(s0, s0 + n)]
                for i, (re, im) in enumerate(_fft(zs)):
                    y = jnp.concatenate([re[1], im[1]], axis=0).astype(bf16)
                    dst[ct, k0 + dk * i, _ds(bb * 32 + 16 * par, 16, 16), :] = y

        def seconds(mid, dst, sp_src, sp_dst):
            return [block(64 if len(subs) == 1 else 40, sp_src, sp_dst, second, mid, dst, par, subs)
                    for par in range(2) for subs in (_SUBS[0:1], _SUBS[1:2], _SUBS[2:3], _SUBS[3:5])]

        def firsts(fn, sp_src, sp_dst):
            return [block(105, sp_src, sp_dst, fn, j, par) for par in range(2) for j in range(4)]

        convs = [block(92, sp_k, sp_kv, conv, range(n, n + 4)) for n in range(0, M1, 4)]
        return (firsts(first_h, sp_ht, sp_mh) + convs + seconds(mh_v, yh_b, sp_mh, sp_yh)
                + firsts(first_x, sp_kv, sp_mx) + seconds(mx_v, yx_b, sp_mx, sp_yx))

    def pacer(blocks, slots, lead=0, free=0, lag=0):
        return _Pacer(sub8 < zero_s[2], blocks, slots, lead, free, lag)

    def phase0():
        def run(blocks, chunk, fts, lead=0, free=0):
            todo = [functools.partial(project_k, tile, ft) for ft in fts for tile in range(*X_CHUNKS[chunk])]
            pacer(blocks, len(todo) * 8 // PACE0, lead, free, 0).run(todo)

        for cs in (*c_wk[2:], c_par):
            start(cs)
        wait(c_x[0] + c_wk[0] + c_wk[1])
        for cs in (c_x[1], c_x[2], c_wq):
            start(cs)
        run([], 0, range(2))
        wait(c_wk[2] + c_wk[3] + c_wk[4] + c_par)
        for cs in (c_x[3], c_wv, c_x[4], c_h[0], c_kv[0], c_h[1]):
            start(cs)
        unpack_parameters()
        run([], 0, range(2, NT))
        wait(c_x[1])
        for cs in (c_kv[1], c_h[2], c_kv[2], c_h[3], c_kv[3], c_h[4], c_kv[4], c_g, c_q, c_wo):
            start(cs)
        run(align_keys(0, 2), 1, range(NT))
        wait(c_x[2] + c_wq)
        run(merge(transpose_weight(0, wq_v), align_keys(2, 6)), 2, range(NT), 2)
        wait(c_x[3] + c_wv)
        run(merge(transpose_weight(1, wv_v), align_keys(6, 7)), 3, range(NT), 2)
        wait(c_x[4] + c_h[0])
        run(merge(transpose_filter(0, 0, 16), align_keys(7, 10)), 4, range(NT), 2)

    def phase1(i, c):
        n = UNROLL1
        for t in range(NT - 1):
            wait_when(i == 2 * t // n, c_kv[t] + c_h[t + 1])
        blocks, pieces = [], []
        for r in range(n):
            half = n * i + r
            ct, odd = half >> 1, half & 1
            ffts = [b for u in range(2) for b in forward_unit(ct, 2 * odd + u)]
            blocks += ffts + transpose_filter(ct + 1, 8 * odd, 8)
            pieces += [functools.partial(project_qv, 2 * half + j, ft, halves)
                       for j in range(2) for ft in range(NT) for halves in HALVES]
        pacer(blocks, n * 20 * 8 // PACE1, LEAD1, FREE1, LAG1).run(pieces)
        return c

    def spectral(ct, u_out, z):
        zs = {}

        def fwd(k1, pace):
            g = _upk(pace.pace(gf_v[k1], PACE2))
            x = _dot(g, _upk(yx_v[ct, k1]))
            h = _dot(g, _upk(yh_v[ct, k1]))
            rows = []
            for a in range(8):
                xr, xi = x[16 * a:16 * a + 8], x[16 * a + 8:16 * a + 16]
                hr, hi = h[16 * a:16 * a + 8], h[16 * a + 8:16 * a + 16]
                rows += [xr * hr - xi * hi, xr * hi + xi * hr]
            pace.note(x)
            zs[k1] = jnp.concatenate(rows, axis=0).astype(bf16)

        def inv(k1, pace):
            u_out[z, k1] = _dot(_upk(pace.pace(gi_v[k1], PACE2)), zs.pop(k1))

        pieces = []
        for k1 in range(M1 + LOOK2):
            if k1 < M1:
                pieces.append(functools.partial(fwd, k1))
            if k1 >= LOOK2:
                pieces.append(functools.partial(inv, k1 - LOOK2))
        return pieces

    def inverse(ct, z):
        u_in = u_v[ct]

        def first(mid, a, subs):
            for s0, n, k0, dk in subs:
                zs = [((1, u_in[z, k, 16 * a:16 * a + 8, :]), (1, u_in[z, k, 16 * a + 8:16 * a + 16, :]))
                      for k in range(k0, M1, dk)]
                for i, (re, im) in enumerate(_ifft(zs)):
                    mid[a % 2, pl.ds(16 * (s0 + i), 8), :] = re[1]
                    mid[a % 2, pl.ds(16 * (s0 + i) + 8, 8), :] = im[1]

        def last(mid, bb, j, par):
            w = {s: ((_INV_MID_SIGNS[s][0], mid[par, _ds(16 * s + zero_s[2], 8), :]),
                     (_INV_MID_SIGNS[s][1], mid[par, _ds(16 * s + 8 + zero_s[2], 8), :]))
                 for s in _slots(j)}
            for m, (sign, y) in enumerate(_inv_last(j, w)):
                n1 = j + 4 * m
                if par == 0:
                    kv_v[0, pl.ds(8 * n1, 8), :] = y
                    continue
                gate_q = _upk(q_v[ct, pl.ds(32 * n1 + 8 * bb, 8), :]).astype(f32)
                y = jnp.concatenate([kv_v[0, _ds(8 * n1 + zero_s[2], 8), :], y], axis=0) * gate_q
                oa_b[ct][0, pl.ds(64 * n1 + 16 * bb, 16), :] = (y if sign > 0 else -y).astype(bf16)

        blocks = []
        for bb in range(4):
            mid, sp_mid = (mh_v, sp_mh) if bb % 2 else (mx_v, sp_mx)
            blocks += [block(56 if len(subs) == 1 else 32, sp_u[ct], sp_mid, first, mid, a, subs)
                       for a in (2 * bb, 2 * bb + 1)
                       for subs in (_SUBS[0:1], _SUBS[1:2], _SUBS[2:3], _SUBS[3:5])]
            blocks += [block(125 if par else 85, sp_mid, sp_oa[ct] if par else sp_kv, last, mid, bb, j, par)
                       for par in range(2) for j in range(4)]
        return blocks

    def stream(cts, z):
        return [piece for ct in cts for piece in spectral(ct, u_v[ct], z)]

    prow = lax.broadcasted_iota(i32, (16, 128), 0)
    steps = [(j, t) for j in (3, 2, 1, 0) for t in range(j + 1)]

    def fill_masks():
        key = lax.broadcasted_iota(i32, (64, 128), 0)
        lane = lax.broadcasted_iota(i32, (64, 128), 1)
        for n, query in enumerate((lane, (lane + 64) & 127, lane & 63)):
            mask_v[n] = jnp.where(key <= query, 0.0, -1e9 * LOG2E).astype(f32)

    def attend(uq, s_out, zo, up, s_in, zi, memory, pace=None, final=False, filler=None):
        low, left = sub8 < 4, lane8 < 64
        if uq is not None:
            sq, gq = uq >> 3, uq & 7
        if up is not None:
            sp, gp = up >> 3, up & 7
            gates = [gate_v[4 * gp + i] for i in range(4)]
        weights, run_max, acc = {}, {}, {}

        def stack(*parts):
            rows = sum(x.shape[0] for x in parts)
            return jnp.concatenate([x for x in parts if x.shape[0]] + [jnp.zeros((64 - rows, 128), u32)], axis=0)

        def q_weights(j):
            if j not in weights:
                qw = []
                for i in range(4):
                    own = (prow >= 2 * i) & (prow < 2 * i + 10)
                    w = qt_v[4 * sq + j, _ds(40 * gq + 8 * i, 16), :]
                    qw.append(jnp.where(own, pltpu.roll(w, 64, 1) if i % 2 else w, jnp.uint32(0)))
                single = [stack(jnp.zeros((8 * i, 128), u32), qw[i]) for i in range(4)]
                shared = []
                for i in (0, 2):
                    a, b = qw[i], qw[i + 1]
                    shared.append(stack(jnp.zeros((8 * i, 128), u32), jnp.where(left, 0, a[:8]),
                                        jnp.where(left, b[:8], a[8:]), jnp.where(left, b[8:], 0)))
                weights[j] = (_upk(jnp.concatenate(single, axis=1)), [_upk(w) for w in shared])
            return weights[j]

        def keys(t, r0, n):
            x = kg_v[gq, _ds(256 * sq + 64 * t + r0 // 2, n // 2), :]
            return _upk(pace.pace(x, 2) if pace else x)

        def column_max(x):
            return jnp.max(x.reshape(x.shape[0] // 8, 8, 128), axis=0)

        def score(j, t):
            single, shared = q_weights(j)
            if t < j:
                return _dot(keys(t, 0, 128), single), None
            main = _dot(keys(t, 0, 64), single)
            tail = [jnp.concatenate([_dot(keys(t, r, 32), w) for r in (64, 96)], axis=0) for w in shared]
            return main, tail

        def keep(j, t, main, tail):
            if pace:
                pace.note(main[:, :128])
            if tail is not None:
                tail = [x + mask_v[2] for x in tail]
                for n, x in enumerate(tail):
                    s_out[j][zo, 2 * n, pl.ds(128 * j + 64, 64)] = x
                tail = [column_max(x) for x in tail]
            for i in range(4):
                st = main[:, 128 * i:128 * i + 128]
                if t == j:
                    st = st + mask_v[i % 2]
                    s_out[j][zo, i, pl.ds(128 * j, 64)] = st
                else:
                    s_out[j][zo, i, pl.ds(128 * t, 128)] = st
                mx = column_max(st)
                run_max[j, i] = mx if t == 0 else jnp.maximum(run_max[j, i], mx)
                if t == j:
                    mine = left if i % 2 else ~left
                    mx = jnp.where(mine, jnp.maximum(run_max[j, i], tail[i // 2]), run_max[j, i])
                    s_out[j][zo, i, pl.ds(128 * j + 128, 8)] = jnp.broadcast_to(
                        jnp.max(mx, axis=0, keepdims=True), (8, 128))

        def expo(x, m):
            return jnp.exp2(x.reshape(x.shape[0] // 8, 8, 128) - m[None]).reshape(x.shape).astype(bf16)

        def probs(j, t):
            m = [s_in[j][zi, i, pl.ds(128 * j + 128, 8)] for i in range(4)]
            if t < j:
                return [expo(s_in[j][zi, i, pl.ds(128 * t, 128)], m[i]) for i in range(4)]
            ps = []
            half = lax.broadcasted_iota(i32, (32, 128), 1) < 64
            for i in (0, 2):
                tail = _pk_mm(expo(s_in[j][zi, i, pl.ds(128 * j + 64, 64)], jnp.where(left, m[i + 1], m[i])))
                for n, part in enumerate((jnp.where(half, 0, tail), jnp.where(half, tail, 0))):
                    main = expo(s_in[j][zi, i + n, pl.ds(128 * j, 64)], m[i + n])
                    ps.append(jnp.concatenate([main, _upk(part)], axis=0))
            return ps

        def v_rows(i, t):
            r0 = (0, 16, 40, 56)[i]
            v = [vt_v[4 * sp + t, _ds(80 * gp + r0 + 8 * b, 8), :] for b in range(3)]
            if i % 2:
                v[0] = jnp.where(low, 1.0, v[0])
            else:
                v[2] = jnp.where(low, v[2], 1.0)
            return jnp.concatenate(v, axis=0)

        mem = {}

        def memory_update(t):
            tile = 4 * (sp - 1) + t
            pk_t = _phi(_upk(kg_v[gp, _ds(tile * 64, 64), :]).astype(f32)).astype(bf16)
            lhs = jnp.concatenate([vt_v[tile, _ds(80 * gp, 80), :], jnp.ones((8, 128), f32)], axis=0)
            d = _dot(lhs, pk_t)
            mem["sum"] = d if t == 0 else mem["sum"] + d
            if t < 3:
                return
            m = mem_v[gp] + mem["sum"]
            mem_v[gp] = m
            own = [(lane8 >= DH * i) & (lane8 < DH * i + DH) for i in range(4)]
            rows = []
            for r in range(10):
                lo, hi = (8 * r) // DH, (8 * r + 7) // DH
                blk = m[8 * r:8 * r + 8]
                a = jnp.where(own[lo], blk * gates[lo], 0.0)
                if hi != lo:
                    a = jnp.where(low, a, jnp.where(own[hi], blk * gates[hi], 0.0))
                rows.append(a)
            rows += [jnp.where((low & own[i]) | (~low & own[i + 1]), m[80:88], 0.0) for i in (0, 2)]
            mem["lhs"] = jnp.concatenate(rows, axis=0).astype(bf16)

        def memory_read(j):
            w = jnp.concatenate([pqt_v[4 * sp + j, _ds(40 * gp, 40), :], jnp.zeros((24, 128), u32)], axis=0)
            r = _dot(mem["lhs"], _upk(w))
            rows = []
            for n in range(2):
                inv = _recip(r[80 + 8 * n:88 + 8 * n] + 1e-6)
                swap = pltpu.roll(inv, 4, 0)
                scales = [jnp.where(low, inv, swap)] * 2 + [inv] + [jnp.where(low, swap, inv)] * 2
                rows += [r[40 * n + 8 * b:40 * n + 8 * b + 8] * scales[b] for b in range(5)]
            return rows

        def finish(j):
            rows = []
            for i in (0, 2):
                a, b = acc[j, i], pltpu.roll(acc[j, i + 1], 64, 1)
                inv = _recip(jnp.where(low, b[0:8], a[16:24])) * (1.0 - jnp.where(low, gates[i + 1], gates[i]))
                swap = pltpu.roll(inv, 4, 0)
                first, second = jnp.where(low, swap, inv), jnp.where(low, inv, swap)
                rows += [a[0:8] * first, a[8:16] * first, jnp.where(low, a[16:24], b[0:8]) * swap,
                         b[8:16] * second, b[16:24] * second]
            if memory:
                rows = [x + y for x, y in zip(rows, memory_read(j))]
            ot_b[4 * sp + j, _ds(80 * gp, 80, 16), :] = jnp.concatenate(rows, axis=0).astype(bf16)

        def weigh(j, t, ps):
            for i in range(4):
                d = _dot(v_rows(i, t), ps[i])
                acc[j, i] = d if t == 0 else acc[j, i] + d
            if t == j:
                finish(j)

        def update(n):
            for t in range(4):
                if memory and UPDATE3[t] == n:
                    memory_update(t)

        for n, (j, t) in enumerate(steps):
            if up is None:
                keep(j, t, *score(j, t))
            elif uq is None:
                filler()
                update(n)
                weigh(j, t, probs(j, t))
            elif final and not memory and n == len(steps) - 1:
                weigh(j, t, probs(j, t))
                keep(j, t, *score(j, t))
            else:
                scores = score(j, t)
                update(n)
                ps = probs(j, t)
                keep(j, t, *scores)
                weigh(j, t, ps)

    def phase2():
        wait(c_kv[NT - 1] + c_g + c_q + c_wo)
        mem_v[...] = jnp.zeros(mem_v.shape, f32)
        z0, z1 = zero_s[0], zero_s[1]
        slots = 64 * 8 // PACE2
        blocks = [b for bb in range(4) for b in forward_unit(NT - 1, bb)]
        pacer(merge(blocks, align_keys(10, 10 + NK2)), NF2 * slots, LEAD2, 0, LAG2F).run(stream(range(NF2), z0))
        blocks = merge([b for ct in range(NI2) for b in inverse(ct, z1)], align_keys(10 + NK2, 16))
        pacer(blocks, (NT - NF2) * slots + 36, 0, FREE2, LAG2).run(
            stream(range(NF2, NT), z0) + [lambda p: attend(0, s_v[0], z0, None, None, None, False, p)])
        start([c for ct in range(NI2) for c in c_oa[ct]])

    def attend_units(memory, filler=None):
        def body(i, c):
            for n in range(UNROLL3):
                unit, final = UNROLL3 * i + n, n == UNROLL3 - 1
                attend(None if filler and final else unit + 1, s_v[1 - n % 2], zero_s[0],
                       unit, s_v[n % 2], zero_s[1], memory, final=final, filler=filler)
            return c
        return body

    def transpose_heads(tile):
        on_v, sp_on = heads[tile // 4]

        def one(ft):
            rows = pl.ds(64 * (tile % 4), 64)
            on_v[ft, rows, :] = _pk(_upk(ot_v[tile, 64 * ft:64 * ft + 64, :]).T)

        return [block(20, None, sp_on, one, ft) for ft in range(NT)]

    def out_project(tile, nt, pace):
        on_v = heads[tile // 4][0]
        parts = [on_v[ft, _ds(64 * (tile % 4) + zero_s[0], 64), :] for ft in range(NT)]
        parts[0] = pace.pace(parts[0], PACE4)
        y = _dot(_upk(jnp.concatenate(parts, axis=1)), _upk(wo_v[nt]))
        pace.note(y)
        ob_b[nt, pl.ds(128 * tile, 128), :] = y.astype(bf16)

    def phase4():
        cts = list(range(NI2, NT))
        for n, (t0, t1) in enumerate(OUT_CHUNKS):
            nxt = OUT_CHUNKS[n + 1] if n + 1 < len(OUT_CHUNKS) else (0, 0)
            blocks = [b for t in range(*nxt) for b in transpose_heads(t)]
            mine = cts[HOST4[n]:HOST4[n + 1]]
            blocks = merge(blocks, [b for ct in mine for b in inverse(ct, zero_s[1])])
            pace = pacer(blocks, (t1 - t0) * NT * 8 // PACE4, LEAD4 if n == 0 else 0, FREE4, LAG4)
            pieces = [functools.partial(out_project, t, nt) for t in range(t0, t1) for nt in range(NT)]
            if n == 0:
                count = itertools.count()
                attend_units(True, lambda: pieces.pop(0)(pace) if next(count) < FILL4 else None)(
                    4 * NG // UNROLL3 - 1, 0)
            pace.run(pieces)
            start([c for ct in mine for c in c_oa[ct]] + c_ob[n])

    fill_masks()
    phase0()
    lax.fori_loop(0, 2 * (NT - 1) // UNROLL1, phase1, 0)
    phase2()
    lax.fori_loop(0, NG // UNROLL3, attend_units(False), 0)
    lax.fori_loop(NG // UNROLL3, 4 * NG // UNROLL3 - 1, attend_units(True), 0)
    for tile in range(*OUT_CHUNKS[0]):
        for b in transpose_heads(tile):
            b[1]()
    phase4()
    for cs in c_oa + c_ob:
        wait(cs)


@jax.jit
def pallas_concat_heads__ssm_conv_h3__memory_aug_infini_attn__prompt_kernel(
    A_q: jax.Array,
    A_k: jax.Array,
    A_v: jax.Array,
    A_shift_k: jax.Array,
    A_ssm_k: jax.Array,
    A_ssm_D: jax.Array,
    B_x: jax.Array,
    B_wq: jax.Array,
    B_wk: jax.Array,
    B_wv: jax.Array,
    B_wo: jax.Array,
    B_beta: jax.Array,
):
    hbm = pl.BlockSpec(memory_space=pl.ANY)
    V = pltpu.VMEM
    scratch = [
        V((NT, S, 128), bf16),
        V((NT, D, 128), bf16), V((NT, D, 128), bf16),
        V((NT, D, 128), bf16), V((NT, D, 128), bf16),
        V((NT + 1, S + 16, 128), bf16), V((NT, S, 128), bf16),
        V((NT, 128, S), bf16), V((NT, S, 128), bf16),
        V((M1, 64, 128), u32), V((M1, 64, 128), u32),
        *[V((2, S, 128), bf16)] * NT, V((NT, S, 128), bf16),
        V((NT + 1, NT, 128, 128), u32),
        V((NT + 1, S // 2, 128), u32),
        V((3, 16 * M1, 128), f32), V((3, 16 * M1, 128), f32),
        V((3, 8 * M1, 128), f32),
        V((NT, 5, 8, 128), f32),
        V((NT + 1, M1, 128, 128), bf16), V((NT + 1, M1, 128, 128), bf16),
        *[V((1, M1 + 1, 128, 128), f32)] * NT,
        *[V((NT + 1, 128 * n, 128), bf16) for n in (2, 4, 4, 6)],
        V((NG + 1, S // 2, 128), u32),
        V((16, D, 128), bf16), V((16, D, 128), bf16),
        V((16, D, 128), f32), V((16, D, 128), bf16),
        *[V((NT + 1, SEG // 2, 128), u32)] * 4,
        *[V((1, 4, 128 * j + 136, 128), f32) for j in range(4)] * 2,
        V((NG, 88, 128), f32),
        V((4 * NG, 8, 128), f32),
        V((3, 64, 128), f32),
        V((4, D), bf16), V((D,), bf16), V((4 * NG,), bf16),
        pltpu.SMEM((3,), i32),
        pltpu.SemaphoreType.DMA((48,)),
    ]
    out = pl.pallas_call(
        _kernel,
        out_shape=jax.ShapeDtypeStruct((S, 2 * D), bf16),
        in_specs=[hbm] * 14,
        out_specs=hbm,
        scratch_shapes=scratch,
        compiler_params=pltpu.CompilerParams(vmem_limit_bytes=110 * 2**20),
    )(
        A_q.reshape(S, D), A_k.reshape(S, D), A_v.reshape(S, D), A_shift_k.T, A_ssm_k, A_ssm_D,
        B_x.reshape(S, D), B_wq, B_wk, B_wv, B_wo, B_beta, _G_FWD, _G_INV,
    )
    return out.reshape(1, S, 2 * D)
```

```python
import functools
import itertools
import math

import jax
import jax.numpy as jnp
import ml_dtypes
import numpy as np
from jax import lax
from jax.experimental import pallas as pl
from jax.experimental.pallas import tpu as pltpu

S = 2048
D = 640
NT = D // 128
DH = 20
NG = 8
SEG = 512
M1, M2 = 32, 64

bf16 = jnp.bfloat16
f32 = jnp.float32
u32 = jnp.uint32
i32 = jnp.int32

LOG2E = math.log2(math.e)
Q_SCALE = DH ** -0.5 * LOG2E
PACE0 = 4
X_CHUNKS = ((0, 2), (2, 6), (6, 10), (10, 12), (12, 16))
K_FIRST = (0, 2, 6, 10)
UNROLL1 = 2
PACE1 = 1
LEAD1 = 6
FREE1 = 300
LAG1 = 2
HALVES = ((0,), (1,))
PACE2 = 4
LEAD2 = 4
FREE2 = 400
LOOK2 = 5
LAG2 = 4
LAG2F = 4
NF2 = 3
NI2 = 2
NK2 = 0
HOST4 = (0, 1, 2, 3, 3, 3)
UNROLL3 = 2
UPDATE3 = (0, 1, 1, 2)
PACE4 = 4
FREE4 = 0
LEAD4 = 0
FILL4 = 10
OUT_CHUNKS = ((0, 4), (4, 8), (8, 12), (12, 15), (15, 16))
LAG4 = 0


def _neg(a):
    return None if a is None else (-a[0], a[1])


def _add(a, b):
    if a is None:
        return b
    if b is None:
        return a
    if a[0] == b[0]:
        return (a[0], a[1] + b[1])
    if a[0] > 0:
        return (1, a[1] - b[1])
    return (1, b[1] - a[1])


def _sub(a, b):
    return _add(a, _neg(b))


def _scale(a, c):
    if a is None or abs(c) < 1e-12:
        return None
    if abs(abs(c) - 1.0) < 1e-12:
        return a if c > 0 else _neg(a)
    return (a[0], a[1] * float(c))


def _cmul(z, ang):
    c, s = math.cos(ang), math.sin(ang)
    x, y = z
    if x is not None and y is not None and abs(abs(c) - abs(s)) < 1e-12:
        r = 1.0 if c * s > 0 else -1.0
        if r > 0:
            return (_scale(_sub(x, y), c), _scale(_add(y, x), c))
        return (_scale(_add(x, y), c), _scale(_sub(y, x), c))
    return (_sub(_scale(x, c), _scale(y, s)), _add(_scale(y, c), _scale(x, s)))


def _cadd(a, b):
    return (_add(a[0], b[0]), _add(a[1], b[1]))


def _csub(a, b):
    return (_sub(a[0], b[0]), _sub(a[1], b[1]))


def _dif_step(a, b, c, d, j, n):
    t1, t2 = _csub(a, c), _csub(b, d)
    mi_t2 = (t2[1], _neg(t2[0]))
    return (_cadd(a, c), _cadd(b, d),
            _cmul(_cadd(t1, mi_t2), -2 * math.pi * j / n),
            _cmul(_csub(t1, mi_t2), -6 * math.pi * j / n))


def _dit_step(e0, e1, o1, o3, j, n):
    a, b = _cmul(o1, 2 * math.pi * j / n), _cmul(o3, 6 * math.pi * j / n)
    s, d = _cadd(a, b), _csub(a, b)
    i_d = (_neg(d[1]), d[0])
    return _cadd(e0, s), _cadd(e1, i_d), _csub(e0, s), _csub(e1, i_d)


def _fft(z):
    n = len(z)
    if n == 1:
        return list(z)
    if n == 2:
        return [_cadd(z[0], z[1]), _csub(z[0], z[1])]
    q = n // 4
    steps = [_dif_step(*z[j::q], j, n) for j in range(q)]
    out = [None] * n
    out[0::2] = _fft([s[0] for s in steps] + [s[1] for s in steps])
    out[1::4] = _fft([s[2] for s in steps])
    out[3::4] = _fft([s[3] for s in steps])
    return out


def _ifft(z):
    n = len(z)
    if n == 1:
        return list(z)
    if n == 2:
        return [_cadd(z[0], z[1]), _csub(z[0], z[1])]
    q = n // 4
    e, o1, o3 = _ifft(z[0::2]), _ifft(z[1::4]), _ifft(z[3::4])
    out = [None] * n
    for j in range(q):
        out[j::q] = _dit_step(e[j], e[j + q], o1[j], o3[j], j, n)
    return out


_SUBS = ((0, 8, 0, 4), (8, 8, 1, 4), (16, 8, 3, 4), (24, 4, 2, 8), (28, 4, 6, 8))


def _fwd_first(j, xs):
    z = [_cmul(((1, x), None), -2 * math.pi * (j + 4 * m) / (4 * M1)) for m, x in enumerate(xs)]
    lo, hi = _dif_step(*z[0::2], j, 32), _dif_step(*z[1::2], j + 4, 32)
    mid = _dif_step(lo[0], hi[0], lo[1], hi[1], j, 16)
    return {j: mid[0], j + 4: mid[1], 8 + j: lo[2], 12 + j: hi[2],
            16 + j: lo[3], 20 + j: hi[3], 24 + j: mid[2], 28 + j: mid[3]}


def _inv_last(j, w):
    mid = _dit_step(w[j], w[j + 4], w[24 + j], w[28 + j], j, 16)
    lo = _dit_step(mid[0], mid[2], w[8 + j], w[16 + j], j, 32)
    hi = _dit_step(mid[1], mid[3], w[12 + j], w[20 + j], j + 4, 32)
    z = [None] * 8
    z[0::2], z[1::2] = lo, hi
    return [_cmul(v, 2 * math.pi * (j + 4 * m) / (4 * M1))[0] for m, v in enumerate(z)]


def _slots(j):
    return (j, j + 4, 8 + j, 12 + j, 16 + j, 20 + j, 24 + j, 28 + j)


def _codelet_signs():
    one = (1, 1.0)
    mid = {}
    for j in range(4):
        mid.update(_fwd_first(j, [1.0] * 8))
    mid = {s: (v[0][0], v[1][0]) for s, v in mid.items()}
    out = {}
    for s0, n, k0, dk in _SUBS:
        ys = _fft([((mid[s0 + i][0], 1.0), (mid[s0 + i][1], 1.0)) for i in range(n)])
        out.update({k0 + dk * i: (y[0][0], y[1][0]) for i, y in enumerate(ys)})
    imid = {}
    for s0, n, _, _ in _SUBS:
        imid.update({s0 + i: (w[0][0], w[1][0]) for i, w in enumerate(_ifft([(one, one)] * n))})
    return mid, out, imid


_FWD_MID_SIGNS, _FWD_SIGNS, _INV_MID_SIGNS = _codelet_signs()


class _Pacer:
    def __init__(self, never, blocks, slots, lead=0, free=0, lag=2):
        self.never, self.blocks, self.slots, self.lag = never, list(blocks), slots - lead, lag
        self.total = sum(b[0] for b in self.blocks) - free
        self.slot, self.spent, self.results = -lead, 0, []

    def note(self, result):
        self.results.append(result[:8])

    def _run_block(self):
        cost, fn, release, word = self.blocks.pop(0)
        self.spent += cost
        if release is not None and len(self.results) >= self.lag > 0:
            release(self.results[-self.lag])
        fn()
        return word

    def pace(self, x, every):
        parts = [x[8 * r:8 * r + 8] for r in range(x.shape[0] // 8)]
        for r in range(0, len(parts), every):
            self.slot += 1
            words = []
            while self.blocks and ((self.spent + self.blocks[0][0] / 2) * self.slots
                                   <= self.total * min(self.slot, self.slots)):
                word = self._run_block()
                if word not in words:
                    words.append(word)
            for word in words:
                parts[r] = jnp.where(self.never, word(), parts[r])
        return jnp.concatenate(parts, axis=0)

    def run(self, pieces):
        for piece in pieces:
            piece(self)
        while self.blocks:
            self._run_block()


def _pack_rows(m):
    b = np.asarray(m, np.float32).astype(ml_dtypes.bfloat16).view(np.uint16).astype(np.uint32)
    return np.ascontiguousarray(b[..., 0::2, :] | (b[..., 1::2, :] << 16))


def _dft_tables():
    r = np.arange(128)
    part = (r // 8) % 2
    nat = 8 * (r // 16) + r % 8
    eo = 16 * (r // 32) + 2 * (r % 8) + (r // 16) % 2
    fwd = np.zeros((M1, 128, 128))
    inv = np.zeros((M1, 128, 128))
    for k1 in range(M1):
        freq = k1 + M1 * nat + 0.25
        ph = 2 * np.pi * freq[:, None] * eo[None, :] / S
        same = part[:, None] == part[None, :]
        cross = np.where(part[:, None] == 0, 1.0, -1.0)
        sg = np.where(part == 0, _FWD_SIGNS[k1][0], _FWD_SIGNS[k1][1])
        fwd[k1] = np.where(same, np.cos(ph), cross * np.sin(ph)) * sg[None, :]
        ph = 2 * np.pi * nat[:, None] * freq[None, :] / S
        inv[k1] = np.where(same, np.cos(ph), -cross * np.sin(ph)) / S
    return _pack_rows(fwd), _pack_rows(inv)


_G_FWD, _G_INV = _dft_tables()


def _pk(x):
    return pltpu.bitcast(x, u32)


def _upk(x):
    return pltpu.bitcast(x, bf16)


_pk_mm = _pk


def _even(x):
    return pltpu.bitcast(x << 16, f32)


def _odd(x):
    return pltpu.bitcast(x & jnp.uint32(0xFFFF0000), f32)


def _dot(a, b):
    return lax.dot_general(a, b, (((1,), (0,)), ((), ())), preferred_element_type=f32)


def _dot_t(a, b):
    return lax.dot_general(a, b, (((1,), (1,)), ((), ())), preferred_element_type=f32)


def _phi(t):
    return jnp.where(t > 0, t + 1.0, jnp.exp2(t * LOG2E))


def _recip(x):
    r = pltpu.reciprocal(x, approx=True)
    return r * (2.0 - x * r)


def _ds(start, size, align=8):
    return pl.ds(pl.multiple_of(start, align), size)


def _kernel(
    q_hbm, k_hbm, v_hbm, shift_hbm, h_hbm, d_hbm,
    x_hbm, wq_hbm, wk_hbm, wv_hbm, wo_hbm, beta_hbm, gf_hbm, gi_hbm,
    out_hbm,
    x_b, wq_b, wk_b, wv_b, wo_b, k_b, v_b, h_b, q_b, gf_v, gi_v,
    oa0_b, oa1_b, oa2_b, oa3_b, oa4_b, ob_b,
    wt_v, ht_v, mx_v, mh_v, kv_v, par_v, yx_b, yh_b, u0_v, u1_v, u2_v, u3_v, u4_v,
    k0_b, k1_b, k2_b, k3_b, kg_v, qt_b, pqt_b, vt_v, ot_b, on0_v, on1_v, on2_v, on3_v,
    sa0_v, sa1_v, sa2_v, sa3_v, sb0_v, sb1_v, sb2_v, sb3_v, mem_v, gate_v, mask_v, first_q, late_v, shift_ref, d_ref, beta_ref, zero_s, sems,
):
    u_v = (u0_v, u1_v, u2_v, u3_v, u4_v)
    kt_b = (k0_b, k1_b, k2_b, k3_b)
    s_v = ((sa0_v, sa1_v, sa2_v, sa3_v), (sb0_v, sb1_v, sb2_v, sb3_v))
    oa_b = (oa0_b, oa1_b, oa2_b, oa3_b, oa4_b)
    x_v, wq_v, wk_v, wv_v, wo_v = (r.bitcast(u32) for r in (x_b, wq_b, wk_b, wv_b, wo_b))
    k_v, v_v, h_v, q_v = (r.bitcast(u32) for r in (k_b, v_b, h_b, q_b))
    yx_v, yh_v = (r.bitcast(u32) for r in (yx_b, yh_b))
    oa_v = [r.bitcast(u32) for r in oa_b]
    kt_v = [r.bitcast(u32) for r in kt_b]
    qt_v, pqt_v, ot_v = (r.bitcast(u32) for r in (qt_b, pqt_b, ot_b))

    n_sem = [0]

    def group(pairs):
        sem = sems.at[n_sem[0]]
        n_sem[0] += 1
        return [pltpu.make_async_copy(src, dst, sem) for src, dst in pairs]

    def cols(t):
        return pl.ds(128 * t, 128)

    def weight(hbm, buf):
        return group([(hbm.at[:, cols(t)], buf.at[t]) for t in range(NT)])

    def xrows(r0, n):
        return group([(x_hbm.at[pl.ds(r0, n), cols(t)], x_b.at[t, pl.ds(r0, n)]) for t in range(NT)])

    c_wk = [group([(wk_hbm.at[:, cols(t)], wk_b.at[t])]) for t in range(NT)]
    c_wq, c_wv, c_wo = (weight(a, b) for a, b in ((wq_hbm, wq_b), (wv_hbm, wv_b), (wo_hbm, wo_b)))
    c_x = [xrows(128 * t0, 128 * (t1 - t0)) for t0, t1 in X_CHUNKS]
    c_h = [group([(h_hbm.at[cols(t)], h_b.at[t])]) for t in range(NT)]
    c_kv = [group([(k_hbm.at[:, cols(t)], k_b.at[t, pl.ds(16, S)]),
                   (v_hbm.at[:, cols(t)], v_b.at[t])]) for t in range(NT)]
    c_g = group([(gf_hbm, gf_v), (gi_hbm, gi_v)])
    c_q = group([(q_hbm.at[:, cols(t)], q_b.at[t]) for t in range(NT)])
    c_oa = [group([(oa_b[t].at[0], out_hbm.at[:, cols(t)])]) for t in range(NT)]
    c_ob = [group([(ob_b.at[t, pl.ds(128 * t0, 128 * (t1 - t0))],
                    out_hbm.at[pl.ds(128 * t0, 128 * (t1 - t0)), cols(NT + t)]) for t in range(NT)])
            for t0, t1 in OUT_CHUNKS]

    def start(cs):
        for c in cs:
            c.start()

    def wait(cs):
        for c in cs:
            c.wait()

    def wait_when(cond, cs):
        pl.when(cond)(lambda: wait(cs))

    c_par = group([(shift_hbm, shift_ref), (d_hbm, d_ref), (beta_hbm, beta_ref)])
    start(c_x[0] + c_wk[0] + c_wk[1])

    sub8 = lax.broadcasted_iota(i32, (8, 128), 0)
    lane8 = lax.broadcasted_iota(i32, (8, 128), 1)

    zero_s[0] = 0
    zero_s[1] = 0
    zero_s[2] = 0

    def unpack_parameters():
        taps = shift_ref[...].astype(f32)
        skip = d_ref[...].astype(f32).reshape(1, D)
        for t in range(NT):
            for j in range(4):
                par_v[t, j] = jnp.broadcast_to(taps[j:j + 1, 128 * t:128 * t + 128], (8, 128))
            par_v[t, 4] = jnp.where(sub8 == 0, skip[:, 128 * t:128 * t + 128], 0.0)
            k_v[t, 0:8, :] = jnp.zeros((8, 128), u32)
        beta = beta_ref[...].astype(f32).reshape(1, 4 * NG)
        gate = 1.0 / (1.0 + jnp.exp(-beta))
        for h in range(4 * NG):
            gate_v[h] = jnp.broadcast_to(gate[:, h:h + 1], (8, 128))


    def key_buffer(tile):
        n = max(i for i, first in enumerate(K_FIRST) if first <= tile)
        return n, K_FIRST[n]

    def project_k(tile, ft, pace):
        parts = [x_v[kt, pl.ds(64 * tile, 64), :] for kt in range(NT)]
        parts[0] = pace.pace(parts[0], PACE0)
        k = _dot(_upk(jnp.concatenate(parts, axis=1)), _upk(wk_v[ft]))
        pace.note(k)
        n, first = key_buffer(tile)
        kt_b[n][ft, pl.ds(128 * (tile - first), 128), :] = k.astype(bf16)

    def project_qv(tile, ft, halves, pace):
        xt = _upk(jnp.concatenate([x_v[kt, _ds(tile * 64, 64), :] for kt in range(NT)], axis=1))
        lo, hi = 64 * halves[0], 64 * halves[-1] + 64
        parts = [wt_v[ft, kt, lo:hi, :] for kt in range(NT)]
        parts[0] = pace.pace(parts[0], PACE1)
        r = _dot_t(_upk(jnp.concatenate(parts, axis=1)), xt)
        pace.note(r)
        rows = pl.ds(128 * ft, 128)
        for i, half in enumerate(halves):
            y = r[128 * i:128 * i + 128]
            if half == 0:
                qt_b[tile, rows, :] = (y * Q_SCALE).astype(bf16)
                pqt_b[tile, rows, :] = _phi(y).astype(bf16)
            else:
                vt_v[tile, rows, :] = y

    class Spare:
        def __init__(self, view, *idx):
            self.view, self.idx = view, idx
            view[(*idx, slice(0, 8), slice(None))] = jnp.zeros((8, 128), view.dtype)

        def word(self):
            return pltpu.bitcast(self.view[(*self.idx, _ds(zero_s[2], 8), slice(None))], u32)

        def release(self, value):
            self.view[(*self.idx, _ds(zero_s[2] + 8, 8), slice(None))] = pltpu.bitcast(value, self.view.dtype)

    sp_ht, sp_k, sp_kv = Spare(ht_v, NT), Spare(k_v, NT), Spare(kv_v, 2)
    sp_mx, sp_mh, sp_yx, sp_yh = Spare(mx_v, 2), Spare(mh_v, 2), Spare(yx_v, NT, 0), Spare(yh_v, NT, 0)
    sp_oa, sp_kt, sp_kg = [Spare(r, 1) for r in oa_v], [Spare(r, NT) for r in kt_v], Spare(kg_v, NG)
    sp_u, sp_wt = [Spare(u, 0, M1) for u in u_v], Spare(wt_v, NT, 0)

    heads = [(r, Spare(r, NT)) for r in (on0_v, on1_v, on2_v, on3_v)]

    def block(cost, src, dst, fn, *args):
        return (cost, functools.partial(fn, *args), src.release if src else None, dst.word)

    def transpose_filter(ct, t0, n):
        def one(t):
            ht_v[ct, _ds((t0 + t) * 64, 64), :] = _pk(_upk(h_v[ct, :, _ds((t0 + t) * 128, 128, 128)]).T)

        return [block(20, None, sp_ht, one, t) for t in range(n)]

    def transpose_weight(half, w_v):
        def one(ft, kt):
            wt_v[ft, kt, 64 * half:64 * half + 64, :] = _pk(_upk(w_v[ft, 64 * kt:64 * kt + 64, :]).T)

        return [block(20, None, sp_wt, one, ft, kt) for ft in range(NT) for kt in range(NT)]

    def align_keys(tile0, tile1):
        def one(r):
            n, first = key_buffer(r // 64)
            rows = pl.ds(r - 64 * first, 16)
            lane = lax.broadcasted_iota(i32, (16, 128), 1)
            for g in range(NG):
                t, off = divmod(80 * g, 128)
                x = kt_v[n][t, rows, :]
                if off > 48:
                    x = jnp.where(lane >= off, x, kt_v[n][t + 1, rows, :])
                kg_v[g, pl.ds(r, 16), :] = pltpu.roll(x, 128 - off, 1) if off else x

        return [block(20, sp_kt[key_buffer(r // 64)[0]], sp_kg, one, r) for r in range(64 * tile0, 64 * tile1, 16)]

    def merge(xs, ys):
        keyed = [((i + 0.5) / len(bs), n, b) for n, bs in enumerate((xs, ys)) for i, b in enumerate(bs)]
        return [b for _, _, b in sorted(keyed, key=lambda e: e[:2])]

    def forward_unit(ct, bb):
        r0 = pl.multiple_of(bb * 8, 8)

        def short_conv(n1):
            w = [par_v[ct, j] for j in range(4)]
            base = r0 + 32 * n1
            p0, p1, p2 = (k_v[ct, pl.ds(base + 8 - j, 8), :] for j in range(3))
            e0, o0, e1, o1, o2 = _even(p0), _odd(p0), _even(p1), _odd(p1), _odd(p2)
            vv = v_v[ct, _ds(base, 8), :]
            return ((w[0] * e0 + w[1] * o1 + w[2] * e1 + w[3] * o2) * _even(vv),
                    (w[0] * o0 + w[1] * e0 + w[2] * o1 + w[3] * e1) * _odd(vv))

        def park(mid, par, vals):
            for s, (re, im) in vals.items():
                mid[par, pl.ds(16 * s, 8), :] = re[1]
                mid[par, pl.ds(16 * s + 8, 8), :] = im[1]

        def conv(n1s):
            for n1 in n1s:
                for par, y in enumerate(short_conv(n1)):
                    kv_v[par, pl.ds(8 * n1, 8), :] = y

        def first_x(j, par):
            xs = [kv_v[par, _ds(8 * (j + 4 * m) + zero_s[2], 8), :] for m in range(8)]
            park(mx_v, par, _fwd_first(j, xs))

        def first_h(j, par):
            xs = [(_odd if par else _even)(ht_v[ct, _ds(r0 + 32 * (j + 4 * m), 8), :]) for m in range(8)]
            if par == 0 and j == 0:
                xs[0] = xs[0] + jnp.where(bb == 0, par_v[ct, 4], 0.0)
            park(mh_v, par, _fwd_first(j, xs))

        def second(mid, dst, par, subs):
            for s0, n, k0, dk in subs:
                zs = [((_FWD_MID_SIGNS[s][0], mid[par, _ds(16 * s + zero_s[2], 8), :]),
                       (_FWD_MID_SIGNS[s][1], mid[par, _ds(16 * s + 8 + zero_s[2], 8), :]))
                      for s in range(s0, s0 + n)]
                for i, (re, im) in enumerate(_fft(zs)):
                    y = jnp.concatenate([re[1], im[1]], axis=0).astype(bf16)
                    dst[ct, k0 + dk * i, _ds(bb * 32 + 16 * par, 16, 16), :] = y

        def seconds(mid, dst, sp_src, sp_dst):
            return [block(64 if len(subs) == 1 else 40, sp_src, sp_dst, second, mid, dst, par, subs)
                    for par in range(2) for subs in (_SUBS[0:1], _SUBS[1:2], _SUBS[2:3], _SUBS[3:5])]

        def firsts(fn, sp_src, sp_dst):
            return [block(105, sp_src, sp_dst, fn, j, par) for par in range(2) for j in range(4)]

        convs = [block(92, sp_k, sp_kv, conv, range(n, n + 4)) for n in range(0, M1, 4)]
        return (firsts(first_h, sp_ht, sp_mh) + convs + seconds(mh_v, yh_b, sp_mh, sp_yh)
                + firsts(first_x, sp_kv, sp_mx) + seconds(mx_v, yx_b, sp_mx, sp_yx))

    def pacer(blocks, slots, lead=0, free=0, lag=0):
        return _Pacer(sub8 < zero_s[2], blocks, slots, lead, free, lag)

    def phase0():
        def run(blocks, chunk, fts, lead=0, free=0):
            todo = [functools.partial(project_k, tile, ft) for ft in fts for tile in range(*X_CHUNKS[chunk])]
            pacer(blocks, len(todo) * 8 // PACE0, lead, free, 0).run(todo)

        for cs in (*c_wk[2:], c_par):
            start(cs)
        wait(c_x[0] + c_wk[0] + c_wk[1])
        for cs in (c_x[1], c_x[2], c_wq):
            start(cs)
        run([], 0, range(2))
        wait(c_wk[2] + c_wk[3] + c_wk[4] + c_par)
        for cs in (c_x[3], c_wv, c_x[4], c_h[0], c_kv[0], c_h[1]):
            start(cs)
        unpack_parameters()
        run([], 0, range(2, NT))
        wait(c_x[1])
        for cs in (c_kv[1], c_h[2], c_kv[2], c_h[3], c_kv[3], c_h[4], c_kv[4], c_g, c_q, c_wo):
            start(cs)
        run(align_keys(0, 2), 1, range(NT))
        wait(c_x[2] + c_wq)
        run(merge(transpose_weight(0, wq_v), align_keys(2, 6)), 2, range(NT), 2)
        wait(c_x[3] + c_wv)
        run(merge(transpose_weight(1, wv_v), align_keys(6, 7)), 3, range(NT), 2)
        wait(c_x[4] + c_h[0])
        run(merge(transpose_filter(0, 0, 16), align_keys(7, 10)), 4, range(NT), 2)

    def phase1(i, c):
        n = UNROLL1
        for t in range(NT - 1):
            wait_when(i == 2 * t // n, c_kv[t] + c_h[t + 1])
        blocks, pieces = [], []
        for r in range(n):
            half = n * i + r
            ct, odd = half >> 1, half & 1
            ffts = [b for u in range(2) for b in forward_unit(ct, 2 * odd + u)]
            blocks += ffts + transpose_filter(ct + 1, 8 * odd, 8)
            pieces += [functools.partial(project_qv, 2 * half + j, ft, halves)
                       for j in range(2) for ft in range(NT) for halves in HALVES]
        pacer(blocks, n * 20 * 8 // PACE1, LEAD1, FREE1, LAG1).run(pieces)
        return c

    def spectral(ct, u_out, z):
        zs = {}

        def fwd(k1, pace):
            g = _upk(pace.pace(gf_v[k1], PACE2))
            x = _dot(g, _upk(yx_v[ct, k1]))
            h = _dot(g, _upk(yh_v[ct, k1]))
            rows = []
            for a in range(8):
                xr, xi = x[16 * a:16 * a + 8], x[16 * a + 8:16 * a + 16]
                hr, hi = h[16 * a:16 * a + 8], h[16 * a + 8:16 * a + 16]
                rows += [xr * hr - xi * hi, xr * hi + xi * hr]
            pace.note(x)
            zs[k1] = jnp.concatenate(rows, axis=0).astype(bf16)

        def inv(k1, pace):
            u_out[z, k1] = _dot(_upk(pace.pace(gi_v[k1], PACE2)), zs.pop(k1))

        pieces = []
        for k1 in range(M1 + LOOK2):
            if k1 < M1:
                pieces.append(functools.partial(fwd, k1))
            if k1 >= LOOK2:
                pieces.append(functools.partial(inv, k1 - LOOK2))
        return pieces

    def inverse(ct, z):
        u_in = u_v[ct]

        def first(mid, a, subs):
            for s0, n, k0, dk in subs:
                zs = [((1, u_in[z, k, 16 * a:16 * a + 8, :]), (1, u_in[z, k, 16 * a + 8:16 * a + 16, :]))
                      for k in range(k0, M1, dk)]
                for i, (re, im) in enumerate(_ifft(zs)):
                    mid[a % 2, pl.ds(16 * (s0 + i), 8), :] = re[1]
                    mid[a % 2, pl.ds(16 * (s0 + i) + 8, 8), :] = im[1]

        def last(mid, bb, j, par):
            w = {s: ((_INV_MID_SIGNS[s][0], mid[par, _ds(16 * s + zero_s[2], 8), :]),
                     (_INV_MID_SIGNS[s][1], mid[par, _ds(16 * s + 8 + zero_s[2], 8), :]))
                 for s in _slots(j)}
            for m, (sign, y) in enumerate(_inv_last(j, w)):
                n1 = j + 4 * m
                if par == 0:
                    kv_v[0, pl.ds(8 * n1, 8), :] = y
                    continue
                gate_q = _upk(q_v[ct, pl.ds(32 * n1 + 8 * bb, 8), :]).astype(f32)
                y = jnp.concatenate([kv_v[0, _ds(8 * n1 + zero_s[2], 8), :], y], axis=0) * gate_q
                oa_b[ct][0, pl.ds(64 * n1 + 16 * bb, 16), :] = (y if sign > 0 else -y).astype(bf16)

        blocks = []
        for bb in range(4):
            mid, sp_mid = (mh_v, sp_mh) if bb % 2 else (mx_v, sp_mx)
            blocks += [block(56 if len(subs) == 1 else 32, sp_u[ct], sp_mid, first, mid, a, subs)
                       for a in (2 * bb, 2 * bb + 1)
                       for subs in (_SUBS[0:1], _SUBS[1:2], _SUBS[2:3], _SUBS[3:5])]
            blocks += [block(125 if par else 85, sp_mid, sp_oa[ct] if par else sp_kv, last, mid, bb, j, par)
                       for par in range(2) for j in range(4)]
        return blocks

    def stream(cts, z):
        return [piece for ct in cts for piece in spectral(ct, u_v[ct], z)]

    prow = lax.broadcasted_iota(i32, (16, 128), 0)
    steps = [(j, t) for j in (3, 2, 1, 0) for t in range(j + 1)]

    def fill_masks():
        key = lax.broadcasted_iota(i32, (64, 128), 0)
        lane = lax.broadcasted_iota(i32, (64, 128), 1)
        for n, query in enumerate((lane, (lane + 64) & 127, lane & 63)):
            mask_v[n] = jnp.where(key <= query, 0.0, -1e9 * LOG2E).astype(f32)

    def head_queries(unit, j):
        out = []
        for i in range(4):
            own = (prow >= 2 * i) & (prow < 2 * i + 10)
            w = qt_v[4 * (unit >> 3) + j, _ds(40 * (unit & 7) + 8 * i, 16), :]
            out.append(jnp.where(own, pltpu.roll(w, 64, 1) if i % 2 else w, jnp.uint32(0)))
        return out

    def prepare_queries(unit):
        for i, w in enumerate(head_queries(unit, 3)):
            first_q[i] = w

    def write_heads(unit, j, local, stored):
        low = sub8 < 4
        gates = [gate_v[4 * (unit & 7) + i] for i in range(4)]
        rows = []
        for i in (0, 2):
            a, b = local[24 * i:24 * i + 24], pltpu.roll(local[24 * i + 24:24 * i + 48], 64, 1)
            inv = _recip(jnp.where(low, b[0:8], a[16:24])) * (1.0 - jnp.where(low, gates[i + 1], gates[i]))
            swap = pltpu.roll(inv, 4, 0)
            first, second = jnp.where(low, swap, inv), jnp.where(low, inv, swap)
            rows += [a[0:8] * first, a[8:16] * first, jnp.where(low, a[16:24], b[0:8]) * swap,
                     b[8:16] * second, b[16:24] * second]
        if stored is not None:
            for n in range(2):
                inv = _recip(stored[80 + 8 * n:88 + 8 * n] + 1e-6)
                swap = pltpu.roll(inv, 4, 0)
                scales = [jnp.where(low, inv, swap)] * 2 + [inv] + [jnp.where(low, swap, inv)] * 2
                for b in range(5):
                    rows[5 * n + b] = rows[5 * n + b] + stored[40 * n + 8 * b:40 * n + 8 * b + 8] * scales[b]
        ot_b[4 * (unit >> 3) + j, _ds(80 * (unit & 7), 80, 16), :] = jnp.concatenate(rows, axis=0).astype(bf16)

    def attend(uq, s_out, zo, up, s_in, zi, memory, pace=None, first=False, final=False, filler=None,
               late=None):
        low, left = sub8 < 4, lane8 < 64
        if uq is not None:
            sq, gq = uq >> 3, uq & 7
        if up is not None:
            sp, gp = up >> 3, up & 7
            gates = [gate_v[4 * gp + i] for i in range(4)]
        weights, run_max, acc = {}, {}, {}

        def stack(*parts):
            rows = sum(x.shape[0] for x in parts)
            return jnp.concatenate([x for x in parts if x.shape[0]] + [jnp.zeros((64 - rows, 128), u32)], axis=0)

        def q_weights(j):
            if j not in weights:
                if first and j == 3:
                    qw = [first_q[i] for i in range(4)]
                else:
                    qw = head_queries(uq, j)
                single = [stack(jnp.zeros((8 * i, 128), u32), qw[i]) for i in range(4)]
                shared = []
                for i in (0, 2):
                    a, b = qw[i], qw[i + 1]
                    shared.append(stack(jnp.zeros((8 * i, 128), u32), jnp.where(left, 0, a[:8]),
                                        jnp.where(left, b[:8], a[8:]), jnp.where(left, b[8:], 0)))
                weights[j] = (_upk(jnp.concatenate(single, axis=1)), [_upk(w) for w in shared])
            return weights[j]

        def keys(t, r0, n):
            x = kg_v[gq, _ds(256 * sq + 64 * t + r0 // 2, n // 2), :]
            return _upk(pace.pace(x, 2) if pace else x)

        def column_max(x):
            return jnp.max(x.reshape(x.shape[0] // 8, 8, 128), axis=0)

        def reduce_max(x):
            return jnp.broadcast_to(jnp.max(x, axis=0, keepdims=True), (8, 128))

        def score(j, t):
            single, shared = q_weights(j)
            if t < j:
                return _dot(keys(t, 0, 128), single), None
            main = _dot(keys(t, 0, 64), single)
            tail = [jnp.concatenate([_dot(keys(t, r, 32), w) for r in (64, 96)], axis=0) for w in shared]
            return main, tail

        def keep(j, t, main, tail):
            if pace:
                pace.note(main[:, :128])
            if tail is not None:
                tail = [x + mask_v[2] for x in tail]
                for n, x in enumerate(tail):
                    s_out[j][zo, 2 * n, pl.ds(128 * j + 64, 64)] = x
                tail = [column_max(x) for x in tail]
            for i in range(4):
                st = main[:, 128 * i:128 * i + 128]
                if t == j:
                    st = st + mask_v[i % 2]
                    s_out[j][zo, i, pl.ds(128 * j, 64)] = st
                else:
                    s_out[j][zo, i, pl.ds(128 * t, 128)] = st
                mx = column_max(st)
                run_max[j, i] = mx if t == 0 else jnp.maximum(run_max[j, i], mx)
                if t == j:
                    mine = left if i % 2 else ~left
                    mx = jnp.where(mine, jnp.maximum(run_max[j, i], tail[i // 2]), run_max[j, i])
                    s_out[j][zo, i, pl.ds(128 * j + 128, 8)] = reduce_max(mx) if j else mx

        def expo(x, m):
            return jnp.exp2(x.reshape(x.shape[0] // 8, 8, 128) - m[None]).reshape(x.shape).astype(bf16)

        def probs(j, t):
            m = [s_in[j][zi, i, pl.ds(128 * j + 128, 8)] for i in range(4)]
            if j == 0:
                m = [reduce_max(x) for x in m]
            if t < j:
                return [expo(s_in[j][zi, i, pl.ds(128 * t, 128)], m[i]) for i in range(4)]
            ps = []
            half = lax.broadcasted_iota(i32, (32, 128), 1) < 64
            for i in (0, 2):
                tail = _pk_mm(expo(s_in[j][zi, i, pl.ds(128 * j + 64, 64)], jnp.where(left, m[i + 1], m[i])))
                for n, part in enumerate((jnp.where(half, 0, tail), jnp.where(half, tail, 0))):
                    main = expo(s_in[j][zi, i + n, pl.ds(128 * j, 64)], m[i + n])
                    ps.append(jnp.concatenate([main, _upk(part)], axis=0))
            return ps

        def v_rows(i, t):
            r0 = (0, 16, 40, 56)[i]
            v = [vt_v[4 * sp + t, _ds(80 * gp + r0 + 8 * b, 8), :] for b in range(3)]
            if i % 2:
                v[0] = jnp.where(low, 1.0, v[0])
            else:
                v[2] = jnp.where(low, v[2], 1.0)
            return jnp.concatenate(v, axis=0)

        mem = {}

        def memory_update(t):
            tile = 4 * (sp - 1) + t
            pk_t = _phi(_upk(kg_v[gp, _ds(tile * 64, 64), :]).astype(f32)).astype(bf16)
            lhs = jnp.concatenate([vt_v[tile, _ds(80 * gp, 80), :], jnp.ones((8, 128), f32)], axis=0)
            d = _dot(lhs, pk_t)
            mem["sum"] = d if t == 0 else mem["sum"] + d
            if t < 3:
                return
            m = mem_v[gp] + mem["sum"]
            mem_v[gp] = m
            own = [(lane8 >= DH * i) & (lane8 < DH * i + DH) for i in range(4)]
            rows = []
            for r in range(10):
                lo, hi = (8 * r) // DH, (8 * r + 7) // DH
                blk = m[8 * r:8 * r + 8]
                a = jnp.where(own[lo], blk * gates[lo], 0.0)
                if hi != lo:
                    a = jnp.where(low, a, jnp.where(own[hi], blk * gates[hi], 0.0))
                rows.append(a)
            rows += [jnp.where((low & own[i]) | (~low & own[i + 1]), m[80:88], 0.0) for i in (0, 2)]
            mem["lhs"] = jnp.concatenate(rows, axis=0).astype(bf16)

        def memory_read(j):
            w = jnp.concatenate([pqt_v[4 * sp + j, _ds(40 * gp, 40), :], jnp.zeros((24, 128), u32)], axis=0)
            return _dot(mem["lhs"], _upk(w))

        def finish(j):
            local = jnp.concatenate([acc[j, i] for i in range(4)], axis=0)
            stored = memory_read(j) if memory else None
            if final and j == 0 and filler is None:
                late_v[0:96] = local
                late_v[96:192] = stored if memory else jnp.zeros((96, 128), f32)
            else:
                write_heads(up, j, local, stored)

        def weigh(j, t, ps):
            for i in range(4):
                d = _dot(v_rows(i, t), ps[i])
                acc[j, i] = d if t == 0 else acc[j, i] + d
            if t == j:
                finish(j)

        def update(n):
            if late is not None and n == 0:
                late()
            for t in range(4):
                if memory and UPDATE3[t] == n:
                    memory_update(t)

        for n, (j, t) in enumerate(steps):
            if up is None:
                keep(j, t, *score(j, t))
            elif uq is None:
                filler()
                update(n)
                weigh(j, t, probs(j, t))
            else:
                scores = score(j, t)
                update(n)
                ps = probs(j, t)
                keep(j, t, *scores)
                weigh(j, t, ps)

    def phase2():
        wait(c_kv[NT - 1] + c_g + c_q + c_wo)
        mem_v[...] = jnp.zeros(mem_v.shape, f32)
        z0, z1 = zero_s[0], zero_s[1]
        slots = 64 * 8 // PACE2
        blocks = [b for bb in range(4) for b in forward_unit(NT - 1, bb)]
        pacer(merge(blocks, align_keys(10, 10 + NK2)), NF2 * slots, LEAD2, 0, LAG2F).run(stream(range(NF2), z0))
        blocks = merge([b for ct in range(NI2) for b in inverse(ct, z1)], align_keys(10 + NK2, 16))
        pacer(blocks, (NT - NF2) * slots + 36, 0, FREE2, LAG2).run(
            stream(range(NF2, NT), z0) + [lambda p: attend(0, s_v[0], z0, None, None, None, False, p)])
        prepare_queries(1)
        late_v[...] = jnp.ones(late_v.shape, f32)
        start([c for ct in range(NI2) for c in c_oa[ct]])

    def attend_units(memory, filler=None):
        def body(i, c):
            prev = jnp.where(i > 0, UNROLL3 * i - 1, 4 * NG)
            late = functools.partial(write_heads, prev, 0, late_v[0:96], late_v[96:192] if memory else None)
            for n in range(UNROLL3):
                unit, final = UNROLL3 * i + n, n == UNROLL3 - 1
                attend(None if filler and final else unit + 1, s_v[1 - n % 2], zero_s[0],
                       unit, s_v[n % 2], zero_s[1], memory, first=n == 0, final=final, filler=filler,
                       late=late if n == 0 else None)
            if filler is None:
                prepare_queries(UNROLL3 * (i + 1) + 1)
            return c
        return body

    def transpose_heads(tile):
        on_v, sp_on = heads[tile // 4]

        def one(ft):
            rows = pl.ds(64 * (tile % 4), 64)
            on_v[ft, rows, :] = _pk(_upk(ot_v[tile, 64 * ft:64 * ft + 64, :]).T)

        return [block(20, None, sp_on, one, ft) for ft in range(NT)]

    def out_project(tile, nt, pace):
        on_v = heads[tile // 4][0]
        parts = [on_v[ft, _ds(64 * (tile % 4) + zero_s[0], 64), :] for ft in range(NT)]
        parts[0] = pace.pace(parts[0], PACE4)
        y = _dot(_upk(jnp.concatenate(parts, axis=1)), _upk(wo_v[nt]))
        pace.note(y)
        ob_b[nt, pl.ds(128 * tile, 128), :] = y.astype(bf16)

    def phase4():
        cts = list(range(NI2, NT))
        for n, (t0, t1) in enumerate(OUT_CHUNKS):
            nxt = OUT_CHUNKS[n + 1] if n + 1 < len(OUT_CHUNKS) else (0, 0)
            blocks = [b for t in range(*nxt) for b in transpose_heads(t)]
            mine = cts[HOST4[n]:HOST4[n + 1]]
            blocks = merge(blocks, [b for ct in mine for b in inverse(ct, zero_s[1])])
            pace = pacer(blocks, (t1 - t0) * NT * 8 // PACE4, LEAD4 if n == 0 else 0, FREE4, LAG4)
            pieces = [functools.partial(out_project, t, nt) for t in range(t0, t1) for nt in range(NT)]
            if n == 0:
                count = itertools.count()
                attend_units(True, lambda: pieces.pop(0)(pace) if next(count) < FILL4 else None)(
                    4 * NG // UNROLL3 - 1, 0)
            pace.run(pieces)
            start([c for ct in mine for c in c_oa[ct]] + c_ob[n])

    fill_masks()
    phase0()
    lax.fori_loop(0, 2 * (NT - 1) // UNROLL1, phase1, 0)
    phase2()
    lax.fori_loop(0, NG // UNROLL3, attend_units(False), 0)
    lax.fori_loop(NG // UNROLL3, 4 * NG // UNROLL3 - 1, attend_units(True), 0)
    for tile in range(*OUT_CHUNKS[0]):
        for b in transpose_heads(tile):
            b[1]()
    phase4()
    for cs in c_oa + c_ob:
        wait(cs)


@jax.jit
def pallas_concat_heads__ssm_conv_h3__memory_aug_infini_attn__prompt_kernel(
    A_q: jax.Array,
    A_k: jax.Array,
    A_v: jax.Array,
    A_shift_k: jax.Array,
    A_ssm_k: jax.Array,
    A_ssm_D: jax.Array,
    B_x: jax.Array,
    B_wq: jax.Array,
    B_wk: jax.Array,
    B_wv: jax.Array,
    B_wo: jax.Array,
    B_beta: jax.Array,
):
    hbm = pl.BlockSpec(memory_space=pl.ANY)
    V = pltpu.VMEM
    scratch = [
        V((NT, S, 128), bf16),
        V((NT, D, 128), bf16), V((NT, D, 128), bf16),
        V((NT, D, 128), bf16), V((NT, D, 128), bf16),
        V((NT + 1, S + 16, 128), bf16), V((NT, S, 128), bf16),
        V((NT, 128, S), bf16), V((NT, S, 128), bf16),
        V((M1, 64, 128), u32), V((M1, 64, 128), u32),
        *[V((2, S, 128), bf16)] * NT, V((NT, S, 128), bf16),
        V((NT + 1, NT, 128, 128), u32),
        V((NT + 1, S // 2, 128), u32),
        V((3, 16 * M1, 128), f32), V((3, 16 * M1, 128), f32),
        V((3, 8 * M1, 128), f32),
        V((NT, 5, 8, 128), f32),
        V((NT + 1, M1, 128, 128), bf16), V((NT + 1, M1, 128, 128), bf16),
        *[V((1, M1 + 1, 128, 128), f32)] * NT,
        *[V((NT + 1, 128 * n, 128), bf16) for n in (2, 4, 4, 6)],
        V((NG + 1, S // 2, 128), u32),
        V((16, D, 128), bf16), V((16, D, 128), bf16),
        V((16, D, 128), f32), V((17, D, 128), bf16),
        *[V((NT + 1, SEG // 2, 128), u32)] * 4,
        *[V((1, 4, 128 * j + 136, 128), f32) for j in range(4)] * 2,
        V((NG, 88, 128), f32),
        V((4 * NG, 8, 128), f32),
        V((3, 64, 128), f32),
        V((4, 16, 128), u32),
        V((192, 128), f32),
        V((4, D), bf16), V((D,), bf16), V((4 * NG,), bf16),
        pltpu.SMEM((3,), i32),
        pltpu.SemaphoreType.DMA((48,)),
    ]
    out = pl.pallas_call(
        _kernel,
        out_shape=jax.ShapeDtypeStruct((S, 2 * D), bf16),
        in_specs=[hbm] * 14,
        out_specs=hbm,
        scratch_shapes=scratch,
        compiler_params=pltpu.CompilerParams(vmem_limit_bytes=110 * 2**20),
    )(
        A_q.reshape(S, D), A_k.reshape(S, D), A_v.reshape(S, D), A_shift_k.T, A_ssm_k, A_ssm_D,
        B_x.reshape(S, D), B_wq, B_wk, B_wv, B_wo, B_beta, _G_FWD, _G_INV,
    )
    return out.reshape(1, S, 2 * D)
```

```python
import functools
import itertools
import math

import jax
import jax.numpy as jnp
import ml_dtypes
import numpy as np
from jax import lax
from jax.experimental import pallas as pl
from jax.experimental.pallas import tpu as pltpu

S = 2048
D = 640
NT = D // 128
DH = 20
NG = 8
SEG = 512
M1, M2 = 32, 64

bf16 = jnp.bfloat16
f32 = jnp.float32
u32 = jnp.uint32
i32 = jnp.int32

LOG2E = math.log2(math.e)
Q_SCALE = DH ** -0.5 * LOG2E

X_CHUNKS = ((0, 2), (2, 6), (6, 12), (12, 16))
K_FIRST = (0, 2, 6, 12)
PACE0 = 4
PACE1, LEAD1, FREE1, LAG1 = 1, 6, 150, 2
PACE2, LEAD2, FREE2, LAG2 = 4, 4, 400, 4
LOOK2 = 5
NF2, NI2 = 3, 2
UPDATE3 = (0, 1, 1, 2)
PACE4 = 4
FILL4 = 10
OUT_CHUNKS = ((0, 4), (4, 8), (8, 12), (12, 15), (15, 16))
HOST4 = (0, 1, 2, 3, 3, 3)


def _neg(a):
    return None if a is None else (-a[0], a[1])


def _add(a, b):
    if a is None:
        return b
    if b is None:
        return a
    if a[0] == b[0]:
        return (a[0], a[1] + b[1])
    if a[0] > 0:
        return (1, a[1] - b[1])
    return (1, b[1] - a[1])


def _sub(a, b):
    return _add(a, _neg(b))


def _scale(a, c):
    if a is None or abs(c) < 1e-12:
        return None
    if abs(abs(c) - 1.0) < 1e-12:
        return a if c > 0 else _neg(a)
    return (a[0], a[1] * float(c))


def _cmul(z, ang):
    c, s = math.cos(ang), math.sin(ang)
    x, y = z
    if x is not None and y is not None and abs(abs(c) - abs(s)) < 1e-12:
        r = 1.0 if c * s > 0 else -1.0
        if r > 0:
            return (_scale(_sub(x, y), c), _scale(_add(y, x), c))
        return (_scale(_add(x, y), c), _scale(_sub(y, x), c))
    return (_sub(_scale(x, c), _scale(y, s)), _add(_scale(y, c), _scale(x, s)))


def _cadd(a, b):
    return (_add(a[0], b[0]), _add(a[1], b[1]))


def _csub(a, b):
    return (_sub(a[0], b[0]), _sub(a[1], b[1]))


def _dif_step(a, b, c, d, j, n):
    t1, t2 = _csub(a, c), _csub(b, d)
    mi_t2 = (t2[1], _neg(t2[0]))
    return (_cadd(a, c), _cadd(b, d),
            _cmul(_cadd(t1, mi_t2), -2 * math.pi * j / n),
            _cmul(_csub(t1, mi_t2), -6 * math.pi * j / n))


def _dit_step(e0, e1, o1, o3, j, n):
    a, b = _cmul(o1, 2 * math.pi * j / n), _cmul(o3, 6 * math.pi * j / n)
    s, d = _cadd(a, b), _csub(a, b)
    i_d = (_neg(d[1]), d[0])
    return _cadd(e0, s), _cadd(e1, i_d), _csub(e0, s), _csub(e1, i_d)


def _fft(z):
    n = len(z)
    if n == 1:
        return list(z)
    if n == 2:
        return [_cadd(z[0], z[1]), _csub(z[0], z[1])]
    q = n // 4
    steps = [_dif_step(*z[j::q], j, n) for j in range(q)]
    out = [None] * n
    out[0::2] = _fft([s[0] for s in steps] + [s[1] for s in steps])
    out[1::4] = _fft([s[2] for s in steps])
    out[3::4] = _fft([s[3] for s in steps])
    return out


def _ifft(z):
    n = len(z)
    if n == 1:
        return list(z)
    if n == 2:
        return [_cadd(z[0], z[1]), _csub(z[0], z[1])]
    q = n // 4
    e, o1, o3 = _ifft(z[0::2]), _ifft(z[1::4]), _ifft(z[3::4])
    out = [None] * n
    for j in range(q):
        out[j::q] = _dit_step(e[j], e[j + q], o1[j], o3[j], j, n)
    return out


_SUBS = ((0, 8, 0, 4), (8, 8, 1, 4), (16, 8, 3, 4), (24, 4, 2, 8), (28, 4, 6, 8))


def _fwd_first(j, xs):
    z = [_cmul(((1, x), None), -2 * math.pi * (j + 4 * m) / (4 * M1)) for m, x in enumerate(xs)]
    lo, hi = _dif_step(*z[0::2], j, 32), _dif_step(*z[1::2], j + 4, 32)
    mid = _dif_step(lo[0], hi[0], lo[1], hi[1], j, 16)
    return {j: mid[0], j + 4: mid[1], 8 + j: lo[2], 12 + j: hi[2],
            16 + j: lo[3], 20 + j: hi[3], 24 + j: mid[2], 28 + j: mid[3]}


def _inv_last(j, w):
    mid = _dit_step(w[j], w[j + 4], w[24 + j], w[28 + j], j, 16)
    lo = _dit_step(mid[0], mid[2], w[8 + j], w[16 + j], j, 32)
    hi = _dit_step(mid[1], mid[3], w[12 + j], w[20 + j], j + 4, 32)
    z = [None] * 8
    z[0::2], z[1::2] = lo, hi
    return [_cmul(v, 2 * math.pi * (j + 4 * m) / (4 * M1))[0] for m, v in enumerate(z)]


def _slots(j):
    return (j, j + 4, 8 + j, 12 + j, 16 + j, 20 + j, 24 + j, 28 + j)


def _codelet_signs():
    one = (1, 1.0)
    mid = {}
    for j in range(4):
        mid.update(_fwd_first(j, [1.0] * 8))
    mid = {s: (v[0][0], v[1][0]) for s, v in mid.items()}
    out = {}
    for s0, n, k0, dk in _SUBS:
        ys = _fft([((mid[s0 + i][0], 1.0), (mid[s0 + i][1], 1.0)) for i in range(n)])
        out.update({k0 + dk * i: (y[0][0], y[1][0]) for i, y in enumerate(ys)})
    imid = {}
    for s0, n, _, _ in _SUBS:
        imid.update({s0 + i: (w[0][0], w[1][0]) for i, w in enumerate(_ifft([(one, one)] * n))})
    return mid, out, imid


_FWD_MID_SIGNS, _FWD_SIGNS, _INV_MID_SIGNS = _codelet_signs()


class _Pacer:
    def __init__(self, never, blocks, slots, lead=0, free=0, lag=2):
        self.never, self.blocks, self.slots, self.lag = never, list(blocks), slots - lead, lag
        self.total = sum(b[0] for b in self.blocks) - free
        self.slot, self.spent, self.results = -lead, 0, []

    def note(self, result):
        self.results.append(result[:8])

    def _run_block(self):
        cost, fn, release, word = self.blocks.pop(0)
        self.spent += cost
        if release is not None and len(self.results) >= self.lag > 0:
            release(self.results[-self.lag])
        fn()
        return word

    def pace(self, x, every):
        parts = [x[8 * r:8 * r + 8] for r in range(x.shape[0] // 8)]
        for r in range(0, len(parts), every):
            self.slot += 1
            words = []
            while self.blocks and ((self.spent + self.blocks[0][0] / 2) * self.slots
                                   <= self.total * min(self.slot, self.slots)):
                word = self._run_block()
                if word not in words:
                    words.append(word)
            for word in words:
                parts[r] = jnp.where(self.never, word(), parts[r])
        return jnp.concatenate(parts, axis=0)

    def run(self, pieces):
        for piece in pieces:
            piece(self)
        while self.blocks:
            self._run_block()


def _pack_rows(m):
    b = np.asarray(m, np.float32).astype(ml_dtypes.bfloat16).view(np.uint16).astype(np.uint32)
    return np.ascontiguousarray(b[..., 0::2, :] | (b[..., 1::2, :] << 16))


def _dft_tables():
    r = np.arange(128)
    part = (r // 8) % 2
    nat = 8 * (r // 16) + r % 8
    eo = 16 * (r // 32) + 2 * (r % 8) + (r // 16) % 2
    fwd = np.zeros((M1, 128, 128))
    inv = np.zeros((M1, 128, 128))
    for k1 in range(M1):
        freq = k1 + M1 * nat + 0.25
        ph = 2 * np.pi * freq[:, None] * eo[None, :] / S
        same = part[:, None] == part[None, :]
        cross = np.where(part[:, None] == 0, 1.0, -1.0)
        sg = np.where(part == 0, _FWD_SIGNS[k1][0], _FWD_SIGNS[k1][1])
        fwd[k1] = np.where(same, np.cos(ph), cross * np.sin(ph)) * sg[None, :]
        ph = 2 * np.pi * nat[:, None] * freq[None, :] / S
        inv[k1] = np.where(same, np.cos(ph), -cross * np.sin(ph)) / S
    return _pack_rows(fwd), _pack_rows(inv)


_G_FWD, _G_INV = _dft_tables()


def _pk(x):
    return pltpu.bitcast(x, u32)


def _upk(x):
    return pltpu.bitcast(x, bf16)


def _even(x):
    return pltpu.bitcast(x << 16, f32)


def _odd(x):
    return pltpu.bitcast(x & jnp.uint32(0xFFFF0000), f32)


def _dot(a, b):
    return lax.dot_general(a, b, (((1,), (0,)), ((), ())), preferred_element_type=f32)


def _dot_t(a, b):
    return lax.dot_general(a, b, (((1,), (1,)), ((), ())), preferred_element_type=f32)


def _phi(t):
    return jnp.where(t > 0, t + 1.0, jnp.exp2(t * LOG2E))


def _recip(x):
    r = pltpu.reciprocal(x, approx=True)
    return r * (2.0 - x * r)


def _ds(start, size, align=8):
    return pl.ds(pl.multiple_of(start, align), size)


def _kernel(
    q_hbm, k_hbm, v_hbm, shift_hbm, h_hbm, d_hbm,
    x_hbm, wq_hbm, wk_hbm, wv_hbm, wo_hbm, beta_hbm, gf_hbm, gi_hbm,
    out_hbm,
    x_b, wq_b, wk_b, wv_b, wo_b, k_b, v_b, h_b, q_b, gf_v, gi_v,
    oa0_b, oa1_b, oa2_b, oa3_b, oa4_b, ob_b,
    wt_v, ht_v, mx_v, mh_v, kv_v, par_v, yx_b, yh_b, u0_v, u1_v, u2_v, u3_v, u4_v,
    k0_b, k1_b, k2_b, k3_b, kg_v, qt_b, pqt_b, vt_v, ot_b, on0_v, on1_v, on2_v, on3_v,
    sa0_v, sa1_v, sa2_v, sa3_v, sb0_v, sb1_v, sb2_v, sb3_v,
    mem_v, gate_v, mask_v, first_q, late_v, shift_ref, d_ref, beta_ref, zero_s, sems,
):
    u_v = (u0_v, u1_v, u2_v, u3_v, u4_v)
    kt_b = (k0_b, k1_b, k2_b, k3_b)
    s_v = ((sa0_v, sa1_v, sa2_v, sa3_v), (sb0_v, sb1_v, sb2_v, sb3_v))
    oa_b = (oa0_b, oa1_b, oa2_b, oa3_b, oa4_b)
    x_v, wq_v, wk_v, wv_v, wo_v = (r.bitcast(u32) for r in (x_b, wq_b, wk_b, wv_b, wo_b))
    k_v, v_v, h_v, q_v = (r.bitcast(u32) for r in (k_b, v_b, h_b, q_b))
    yx_v, yh_v = (r.bitcast(u32) for r in (yx_b, yh_b))
    oa_v = [r.bitcast(u32) for r in oa_b]
    kt_v = [r.bitcast(u32) for r in kt_b]
    qt_v, pqt_v, ot_v = (r.bitcast(u32) for r in (qt_b, pqt_b, ot_b))

    n_sem = [0]

    def group(pairs):
        sem = sems.at[n_sem[0]]
        n_sem[0] += 1
        return [pltpu.make_async_copy(src, dst, sem) for src, dst in pairs]

    def cols(t):
        return pl.ds(128 * t, 128)

    def weight(hbm, buf):
        return group([(hbm.at[:, cols(t)], buf.at[t]) for t in range(NT)])

    def xrows(r0, n):
        return group([(x_hbm.at[pl.ds(r0, n), cols(t)], x_b.at[t, pl.ds(r0, n)]) for t in range(NT)])

    c_wk = [group([(wk_hbm.at[:, cols(t)], wk_b.at[t])]) for t in range(NT)]
    c_wq, c_wv, c_wo = (weight(a, b) for a, b in ((wq_hbm, wq_b), (wv_hbm, wv_b), (wo_hbm, wo_b)))
    c_x = [xrows(128 * t0, 128 * (t1 - t0)) for t0, t1 in X_CHUNKS]
    c_h = [group([(h_hbm.at[cols(t)], h_b.at[t])]) for t in range(NT)]
    c_kv = [group([(k_hbm.at[:, cols(t)], k_b.at[t, pl.ds(16, S)]),
                   (v_hbm.at[:, cols(t)], v_b.at[t])]) for t in range(NT)]
    c_g = group([(gf_hbm, gf_v), (gi_hbm, gi_v)])
    c_q = group([(q_hbm.at[:, cols(t)], q_b.at[t]) for t in range(NT)])
    c_oa = [group([(oa_b[t].at[0], out_hbm.at[:, cols(t)])]) for t in range(NT)]
    c_ob = [group([(ob_b.at[t, pl.ds(128 * t0, 128 * (t1 - t0))],
                    out_hbm.at[pl.ds(128 * t0, 128 * (t1 - t0)), cols(NT + t)]) for t in range(NT)])
            for t0, t1 in OUT_CHUNKS]

    def start(cs):
        for c in cs:
            c.start()

    def wait(cs):
        for c in cs:
            c.wait()

    def wait_when(cond, cs):
        pl.when(cond)(lambda: wait(cs))

    c_par = group([(shift_hbm, shift_ref), (d_hbm, d_ref), (beta_hbm, beta_ref)])
    start(c_x[0] + c_wk[0] + c_wk[1])

    sub8 = lax.broadcasted_iota(i32, (8, 128), 0)
    lane8 = lax.broadcasted_iota(i32, (8, 128), 1)

    zero_s[0] = 0
    zero_s[1] = 0
    zero_s[2] = 0

    def unpack_parameters():
        taps = shift_ref[...].astype(f32)
        skip = d_ref[...].astype(f32).reshape(1, D)
        for t in range(NT):
            for j in range(4):
                par_v[t, j] = jnp.broadcast_to(taps[j:j + 1, 128 * t:128 * t + 128], (8, 128))
            par_v[t, 4] = jnp.where(sub8 == 0, skip[:, 128 * t:128 * t + 128], 0.0)
            k_v[t, 0:8, :] = jnp.zeros((8, 128), u32)
        beta = beta_ref[...].astype(f32).reshape(1, 4 * NG)
        gate = 1.0 / (1.0 + jnp.exp(-beta))
        for h in range(4 * NG):
            gate_v[h] = jnp.broadcast_to(gate[:, h:h + 1], (8, 128))


    def key_buffer(tile):
        n = max(i for i, first in enumerate(K_FIRST) if first <= tile)
        return n, K_FIRST[n]

    def project_k(tile, ft, pace):
        parts = [x_v[kt, pl.ds(64 * tile, 64), :] for kt in range(NT)]
        parts[0] = pace.pace(parts[0], PACE0)
        k = _dot(_upk(jnp.concatenate(parts, axis=1)), _upk(wk_v[ft]))
        pace.note(k)
        n, first = key_buffer(tile)
        kt_b[n][ft, pl.ds(128 * (tile - first), 128), :] = k.astype(bf16)

    def project_qv(tile, ft, half, pace):
        xt = _upk(jnp.concatenate([x_v[kt, _ds(tile * 64, 64), :] for kt in range(NT)], axis=1))
        parts = [wt_v[ft, kt, 64 * half:64 * half + 64, :] for kt in range(NT)]
        parts[0] = pace.pace(parts[0], PACE1)
        y = _dot_t(_upk(jnp.concatenate(parts, axis=1)), xt)
        pace.note(y)
        rows = pl.ds(128 * ft, 128)
        if half == 0:
            qt_b[tile, rows, :] = (y * Q_SCALE).astype(bf16)
            pqt_b[tile, rows, :] = _phi(y).astype(bf16)
        else:
            vt_v[tile, rows, :] = y

    class Spare:
        def __init__(self, view, *idx):
            self.view, self.idx = view, idx
            view[(*idx, slice(0, 8), slice(None))] = jnp.zeros((8, 128), view.dtype)

        def word(self):
            return pltpu.bitcast(self.view[(*self.idx, _ds(zero_s[2], 8), slice(None))], u32)

        def release(self, value):
            self.view[(*self.idx, _ds(zero_s[2] + 8, 8), slice(None))] = pltpu.bitcast(value, self.view.dtype)

    sp_ht, sp_k, sp_kv = Spare(ht_v, NT), Spare(k_v, NT), Spare(kv_v, 2)
    sp_mx, sp_mh, sp_yx, sp_yh = Spare(mx_v, 2), Spare(mh_v, 2), Spare(yx_v, NT, 0), Spare(yh_v, NT, 0)
    sp_oa, sp_kt, sp_kg = [Spare(r, 1) for r in oa_v], [Spare(r, NT) for r in kt_v], Spare(kg_v, NG)
    sp_u, sp_wt = [Spare(u, 0, M1) for u in u_v], Spare(wt_v, NT, 0)

    heads = [(r, Spare(r, NT)) for r in (on0_v, on1_v, on2_v, on3_v)]

    def block(cost, src, dst, fn, *args):
        return (cost, functools.partial(fn, *args), src.release if src else None, dst.word)

    def transpose_filter(ct):
        def one(t):
            ht_v[ct, pl.ds(64 * t, 64), :] = _pk(_upk(h_v[ct, :, pl.ds(128 * t, 128)]).T)

        return [block(20, None, sp_ht, one, t) for t in range(S // 128)]

    def transpose_weight(half, w_v):
        def one(ft, kt):
            wt_v[ft, kt, 64 * half:64 * half + 64, :] = _pk(_upk(w_v[ft, 64 * kt:64 * kt + 64, :]).T)

        return [block(20, None, sp_wt, one, ft, kt) for ft in range(NT) for kt in range(NT)]

    def align_keys(tile0, tile1):
        def one(r):
            n, first = key_buffer(r // 64)
            rows = pl.ds(r - 64 * first, 16)
            lane = lax.broadcasted_iota(i32, (16, 128), 1)
            for g in range(NG):
                t, off = divmod(80 * g, 128)
                x = kt_v[n][t, rows, :]
                if off > 48:
                    x = jnp.where(lane >= off, x, kt_v[n][t + 1, rows, :])
                kg_v[g, pl.ds(r, 16), :] = pltpu.roll(x, 128 - off, 1) if off else x

        return [block(20, sp_kt[key_buffer(r // 64)[0]], sp_kg, one, r) for r in range(64 * tile0, 64 * tile1, 16)]

    def merge(xs, ys):
        keyed = [((i + 0.5) / len(bs), n, b) for n, bs in enumerate((xs, ys)) for i, b in enumerate(bs)]
        return [b for _, _, b in sorted(keyed, key=lambda e: e[:2])]

    def forward_unit(ct, bb):
        r0 = pl.multiple_of(bb * 8, 8)

        def short_conv(n1):
            w = [par_v[ct, j] for j in range(4)]
            base = r0 + 32 * n1
            p0, p1, p2 = (k_v[ct, pl.ds(base + 8 - j, 8), :] for j in range(3))
            e0, o0, e1, o1, o2 = _even(p0), _odd(p0), _even(p1), _odd(p1), _odd(p2)
            vv = v_v[ct, _ds(base, 8), :]
            return ((w[0] * e0 + w[1] * o1 + w[2] * e1 + w[3] * o2) * _even(vv),
                    (w[0] * o0 + w[1] * e0 + w[2] * o1 + w[3] * e1) * _odd(vv))

        def park(mid, par, vals):
            for s, (re, im) in vals.items():
                mid[par, pl.ds(16 * s, 8), :] = re[1]
                mid[par, pl.ds(16 * s + 8, 8), :] = im[1]

        def conv(n1s):
            for n1 in n1s:
                for par, y in enumerate(short_conv(n1)):
                    kv_v[par, pl.ds(8 * n1, 8), :] = y

        def first_x(j, par):
            xs = [kv_v[par, _ds(8 * (j + 4 * m) + zero_s[2], 8), :] for m in range(8)]
            park(mx_v, par, _fwd_first(j, xs))

        def first_h(j, par):
            xs = [(_odd if par else _even)(ht_v[ct, _ds(r0 + 32 * (j + 4 * m), 8), :]) for m in range(8)]
            if par == 0 and j == 0:
                xs[0] = xs[0] + jnp.where(bb == 0, par_v[ct, 4], 0.0)
            park(mh_v, par, _fwd_first(j, xs))

        def second(mid, dst, par, subs):
            for s0, n, k0, dk in subs:
                zs = [((_FWD_MID_SIGNS[s][0], mid[par, _ds(16 * s + zero_s[2], 8), :]),
                       (_FWD_MID_SIGNS[s][1], mid[par, _ds(16 * s + 8 + zero_s[2], 8), :]))
                      for s in range(s0, s0 + n)]
                for i, (re, im) in enumerate(_fft(zs)):
                    y = jnp.concatenate([re[1], im[1]], axis=0).astype(bf16)
                    dst[ct, k0 + dk * i, _ds(bb * 32 + 16 * par, 16, 16), :] = y

        def seconds(mid, dst, sp_src, sp_dst):
            return [block(64 if len(subs) == 1 else 40, sp_src, sp_dst, second, mid, dst, par, subs)
                    for par in range(2) for subs in (_SUBS[0:1], _SUBS[1:2], _SUBS[2:3], _SUBS[3:5])]

        def firsts(fn, sp_src, sp_dst):
            return [block(95, sp_src, sp_dst, fn, j, par) for par in range(2) for j in range(4)]

        convs = [block(46, sp_k, sp_kv, conv, range(n, n + 2)) for n in range(0, M1, 2)]
        return (firsts(first_h, sp_ht, sp_mh) + convs + seconds(mh_v, yh_b, sp_mh, sp_yh)
                + firsts(first_x, sp_kv, sp_mx) + seconds(mx_v, yx_b, sp_mx, sp_yx))

    def forward(ct):
        return [b for bb in range(4) for b in forward_unit(ct, bb)]

    def pacer(blocks, slots, lead=0, free=0, lag=0):
        return _Pacer(sub8 < zero_s[2], blocks, slots, lead, free, lag)

    def phase0():
        def run(blocks, chunk, fts, lead=0):
            todo = [functools.partial(project_k, tile, ft) for ft in fts for tile in range(*X_CHUNKS[chunk])]
            pacer(blocks, len(todo) * 8 // PACE0, lead).run(todo)

        for cs in (*c_wk[2:], c_par):
            start(cs)
        wait(c_x[0] + c_wk[0] + c_wk[1])
        for cs in (c_x[1], c_x[2], c_wq):
            start(cs)
        run([], 0, range(2))
        wait(c_wk[2] + c_wk[3] + c_wk[4] + c_par)
        for cs in (c_x[3], c_wv, c_h[0], c_kv[0], c_h[1]):
            start(cs)
        unpack_parameters()
        run([], 0, range(2, NT))
        wait(c_x[1])
        for cs in (c_kv[1], c_h[2], c_kv[2], c_h[3], c_kv[3], c_h[4], c_kv[4], c_g, c_q, c_wo):
            start(cs)
        run(align_keys(0, 2), 1, range(NT))
        wait(c_x[2] + c_wq)
        run(merge(transpose_weight(0, wq_v), align_keys(2, 6)), 2, range(NT), 2)
        wait(c_x[3] + c_wv + c_h[0])
        turns = transpose_weight(1, wv_v) + transpose_filter(0)
        run(merge(turns, align_keys(6, 12)), 3, range(NT), 2)

    def phase1(ct, c):
        for t in range(NT - 1):
            wait_when(ct == t, c_kv[t] + c_h[t + 1])
        blocks = merge(forward(ct), transpose_filter(ct + 1))
        pieces = [functools.partial(project_qv, 4 * ct + j, ft, half)
                  for j in range(4) for ft in range(NT) for half in range(2)]
        pacer(blocks, len(pieces) * 8 // PACE1, LEAD1, FREE1, LAG1).run(pieces)
        return c

    def spectral(ct, u_out, z):
        zs = {}

        def fwd(k1, pace):
            g = _upk(pace.pace(gf_v[k1], PACE2))
            x = _dot(g, _upk(yx_v[ct, k1]))
            h = _dot(g, _upk(yh_v[ct, k1]))
            rows = []
            for a in range(8):
                xr, xi = x[16 * a:16 * a + 8], x[16 * a + 8:16 * a + 16]
                hr, hi = h[16 * a:16 * a + 8], h[16 * a + 8:16 * a + 16]
                rows += [xr * hr - xi * hi, xr * hi + xi * hr]
            pace.note(x)
            zs[k1] = jnp.concatenate(rows, axis=0).astype(bf16)

        def inv(k1, pace):
            u_out[z, k1] = _dot(_upk(pace.pace(gi_v[k1], PACE2)), zs.pop(k1))

        pieces = []
        for k1 in range(M1 + LOOK2):
            if k1 < M1:
                pieces.append(functools.partial(fwd, k1))
            if k1 >= LOOK2:
                pieces.append(functools.partial(inv, k1 - LOOK2))
        return pieces

    def inverse(ct, z):
        u_in = u_v[ct]

        def first(mid, a, subs):
            for s0, n, k0, dk in subs:
                zs = [((1, u_in[z, k, 16 * a:16 * a + 8, :]), (1, u_in[z, k, 16 * a + 8:16 * a + 16, :]))
                      for k in range(k0, M1, dk)]
                for i, (re, im) in enumerate(_ifft(zs)):
                    mid[a % 2, pl.ds(16 * (s0 + i), 8), :] = re[1]
                    mid[a % 2, pl.ds(16 * (s0 + i) + 8, 8), :] = im[1]

        def last(mid, bb, j, par):
            w = {s: ((_INV_MID_SIGNS[s][0], mid[par, _ds(16 * s + zero_s[2], 8), :]),
                     (_INV_MID_SIGNS[s][1], mid[par, _ds(16 * s + 8 + zero_s[2], 8), :]))
                 for s in _slots(j)}
            for m, (sign, y) in enumerate(_inv_last(j, w)):
                n1 = j + 4 * m
                if par == 0:
                    kv_v[0, pl.ds(8 * n1, 8), :] = y
                    continue
                gate_q = _upk(q_v[ct, pl.ds(32 * n1 + 8 * bb, 8), :]).astype(f32)
                y = jnp.concatenate([kv_v[0, _ds(8 * n1 + zero_s[2], 8), :], y], axis=0) * gate_q
                oa_b[ct][0, pl.ds(64 * n1 + 16 * bb, 16), :] = (y if sign > 0 else -y).astype(bf16)

        blocks = []
        for bb in range(4):
            mid, sp_mid = (mh_v, sp_mh) if bb % 2 else (mx_v, sp_mx)
            blocks += [block(56 if len(subs) == 1 else 32, sp_u[ct], sp_mid, first, mid, a, subs)
                       for a in (2 * bb, 2 * bb + 1)
                       for subs in (_SUBS[0:1], _SUBS[1:2], _SUBS[2:3], _SUBS[3:5])]
            blocks += [block(125 if par else 85, sp_mid, sp_oa[ct] if par else sp_kv, last, mid, bb, j, par)
                       for par in range(2) for j in range(4)]
        return blocks

    def stream(cts, z):
        return [piece for ct in cts for piece in spectral(ct, u_v[ct], z)]

    prow = lax.broadcasted_iota(i32, (16, 128), 0)
    steps = [(j, t) for j in (3, 2, 1, 0) for t in range(j + 1)]

    def fill_masks():
        key = lax.broadcasted_iota(i32, (64, 128), 0)
        lane = lax.broadcasted_iota(i32, (64, 128), 1)
        for n, query in enumerate((lane, (lane + 64) & 127, lane & 63)):
            mask_v[n] = jnp.where(key <= query, 0.0, -1e9 * LOG2E).astype(f32)

    def head_queries(unit, j):
        out = []
        for i in range(4):
            own = (prow >= 2 * i) & (prow < 2 * i + 10)
            w = qt_v[4 * (unit >> 3) + j, _ds(40 * (unit & 7) + 8 * i, 16), :]
            out.append(jnp.where(own, pltpu.roll(w, 64, 1) if i % 2 else w, jnp.uint32(0)))
        return out

    def prepare_queries(unit):
        for i, w in enumerate(head_queries(unit, 3)):
            first_q[i] = w

    def write_heads(unit, j, local, stored):
        low = sub8 < 4
        gates = [gate_v[4 * (unit & 7) + i] for i in range(4)]
        rows = []
        for i in (0, 2):
            a, b = local[24 * i:24 * i + 24], pltpu.roll(local[24 * i + 24:24 * i + 48], 64, 1)
            inv = _recip(jnp.where(low, b[0:8], a[16:24])) * (1.0 - jnp.where(low, gates[i + 1], gates[i]))
            swap = pltpu.roll(inv, 4, 0)
            first, second = jnp.where(low, swap, inv), jnp.where(low, inv, swap)
            rows += [a[0:8] * first, a[8:16] * first, jnp.where(low, a[16:24], b[0:8]) * swap,
                     b[8:16] * second, b[16:24] * second]
        if stored is not None:
            for n in range(2):
                inv = _recip(stored[80 + 8 * n:88 + 8 * n] + 1e-6)
                swap = pltpu.roll(inv, 4, 0)
                scales = [jnp.where(low, inv, swap)] * 2 + [inv] + [jnp.where(low, swap, inv)] * 2
                for b in range(5):
                    rows[5 * n + b] = rows[5 * n + b] + stored[40 * n + 8 * b:40 * n + 8 * b + 8] * scales[b]
        ot_b[4 * (unit >> 3) + j, _ds(80 * (unit & 7), 80, 16), :] = jnp.concatenate(rows, axis=0).astype(bf16)

    def attend(uq, s_out, zo, up, s_in, zi, memory, pace=None, first=False, final=False, filler=None,
               late=None):
        low, left = sub8 < 4, lane8 < 64
        if uq is not None:
            sq, gq = uq >> 3, uq & 7
        if up is not None:
            sp, gp = up >> 3, up & 7
            gates = [gate_v[4 * gp + i] for i in range(4)]
        weights, run_max, acc = {}, {}, {}

        def stack(*parts):
            rows = sum(x.shape[0] for x in parts)
            return jnp.concatenate([x for x in parts if x.shape[0]] + [jnp.zeros((64 - rows, 128), u32)], axis=0)

        def q_weights(j):
            if j not in weights:
                if first and j == 3:
                    qw = [first_q[i] for i in range(4)]
                else:
                    qw = head_queries(uq, j)
                single = [stack(jnp.zeros((8 * i, 128), u32), qw[i]) for i in range(4)]
                shared = []
                for i in (0, 2):
                    a, b = qw[i], qw[i + 1]
                    shared.append(stack(jnp.zeros((8 * i, 128), u32), jnp.where(left, 0, a[:8]),
                                        jnp.where(left, b[:8], a[8:]), jnp.where(left, b[8:], 0)))
                weights[j] = (_upk(jnp.concatenate(single, axis=1)), [_upk(w) for w in shared])
            return weights[j]

        def keys(t, r0, n):
            x = kg_v[gq, _ds(256 * sq + 64 * t + r0 // 2, n // 2), :]
            return _upk(pace.pace(x, 2) if pace else x)

        def column_max(x):
            return jnp.max(x.reshape(x.shape[0] // 8, 8, 128), axis=0)

        def reduce_max(x):
            return jnp.broadcast_to(jnp.max(x, axis=0, keepdims=True), (8, 128))

        def score(j, t):
            single, shared = q_weights(j)
            if t < j:
                return _dot(keys(t, 0, 128), single), None
            main = _dot(keys(t, 0, 64), single)
            tail = [jnp.concatenate([_dot(keys(t, r, 32), w) for r in (64, 96)], axis=0) for w in shared]
            return main, tail

        def keep(j, t, main, tail):
            if pace:
                pace.note(main[:, :128])
            if tail is not None:
                tail = [x + mask_v[2] for x in tail]
                for n, x in enumerate(tail):
                    s_out[j][zo, 2 * n, pl.ds(128 * j + 64, 64)] = x
                tail = [column_max(x) for x in tail]
            for i in range(4):
                st = main[:, 128 * i:128 * i + 128]
                if t == j:
                    st = st + mask_v[i % 2]
                    s_out[j][zo, i, pl.ds(128 * j, 64)] = st
                else:
                    s_out[j][zo, i, pl.ds(128 * t, 128)] = st
                mx = column_max(st)
                run_max[j, i] = mx if t == 0 else jnp.maximum(run_max[j, i], mx)
                if t == j:
                    mine = left if i % 2 else ~left
                    mx = jnp.where(mine, jnp.maximum(run_max[j, i], tail[i // 2]), run_max[j, i])
                    s_out[j][zo, i, pl.ds(128 * j + 128, 8)] = reduce_max(mx) if j else mx

        def expo(x, m):
            return jnp.exp2(x.reshape(x.shape[0] // 8, 8, 128) - m[None]).reshape(x.shape).astype(bf16)

        def probs(j, t):
            m = [s_in[j][zi, i, pl.ds(128 * j + 128, 8)] for i in range(4)]
            if j == 0:
                m = [reduce_max(x) for x in m]
            if t < j:
                return [expo(s_in[j][zi, i, pl.ds(128 * t, 128)], m[i]) for i in range(4)]
            ps = []
            half = lax.broadcasted_iota(i32, (32, 128), 1) < 64
            for i in (0, 2):
                tail = _pk(expo(s_in[j][zi, i, pl.ds(128 * j + 64, 64)], jnp.where(left, m[i + 1], m[i])))
                for n, part in enumerate((jnp.where(half, 0, tail), jnp.where(half, tail, 0))):
                    main = expo(s_in[j][zi, i + n, pl.ds(128 * j, 64)], m[i + n])
                    ps.append(jnp.concatenate([main, _upk(part)], axis=0))
            return ps

        def v_rows(i, t):
            r0 = (0, 16, 40, 56)[i]
            v = [vt_v[4 * sp + t, _ds(80 * gp + r0 + 8 * b, 8), :] for b in range(3)]
            if i % 2:
                v[0] = jnp.where(low, 1.0, v[0])
            else:
                v[2] = jnp.where(low, v[2], 1.0)
            return jnp.concatenate(v, axis=0)

        mem = {}

        def memory_update(t):
            tile = 4 * (sp - 1) + t
            pk_t = _phi(_upk(kg_v[gp, _ds(tile * 64, 64), :]).astype(f32)).astype(bf16)
            lhs = jnp.concatenate([vt_v[tile, _ds(80 * gp, 80), :], jnp.ones((8, 128), f32)], axis=0)
            d = _dot(lhs, pk_t)
            mem["sum"] = d if t == 0 else mem["sum"] + d
            if t < 3:
                return
            m = mem_v[gp] + mem["sum"]
            mem_v[gp] = m
            own = [(lane8 >= DH * i) & (lane8 < DH * i + DH) for i in range(4)]
            rows = []
            for r in range(10):
                lo, hi = (8 * r) // DH, (8 * r + 7) // DH
                blk = m[8 * r:8 * r + 8]
                a = jnp.where(own[lo], blk * gates[lo], 0.0)
                if hi != lo:
                    a = jnp.where(low, a, jnp.where(own[hi], blk * gates[hi], 0.0))
                rows.append(a)
            rows += [jnp.where((low & own[i]) | (~low & own[i + 1]), m[80:88], 0.0) for i in (0, 2)]
            mem["lhs"] = jnp.concatenate(rows, axis=0).astype(bf16)

        def memory_read(j):
            w = jnp.concatenate([pqt_v[4 * sp + j, _ds(40 * gp, 40), :], jnp.zeros((24, 128), u32)], axis=0)
            return _dot(mem["lhs"], _upk(w))

        def finish(j):
            local = jnp.concatenate([acc[j, i] for i in range(4)], axis=0)
            stored = memory_read(j) if memory else None
            if final and j == 0 and filler is None:
                late_v[0:96] = local
                late_v[96:192] = stored if memory else jnp.zeros((96, 128), f32)
            else:
                write_heads(up, j, local, stored)

        def weigh(j, t, ps):
            for i in range(4):
                d = _dot(v_rows(i, t), ps[i])
                acc[j, i] = d if t == 0 else acc[j, i] + d
            if t == j:
                finish(j)

        def update(n):
            if late is not None and n == 0:
                late()
            for t in range(4):
                if memory and UPDATE3[t] == n:
                    memory_update(t)

        for n, (j, t) in enumerate(steps):
            if up is None:
                keep(j, t, *score(j, t))
            elif uq is None:
                filler()
                update(n)
                weigh(j, t, probs(j, t))
            else:
                scores = score(j, t)
                update(n)
                ps = probs(j, t)
                keep(j, t, *scores)
                weigh(j, t, ps)

    def phase2():
        wait(c_kv[NT - 1] + c_g + c_q + c_wo)
        mem_v[...] = jnp.zeros(mem_v.shape, f32)
        z0, z1 = zero_s[0], zero_s[1]
        slots = 64 * 8 // PACE2
        pacer(forward(NT - 1), NF2 * slots, LEAD2, 0, LAG2).run(stream(range(NF2), z0))
        blocks = merge([b for ct in range(NI2) for b in inverse(ct, z1)], align_keys(12, 16))
        pacer(blocks, (NT - NF2) * slots + 36, 0, FREE2, LAG2).run(
            stream(range(NF2, NT), z0) + [lambda p: attend(0, s_v[0], z0, None, None, None, False, p)])
        prepare_queries(1)
        late_v[...] = jnp.ones(late_v.shape, f32)
        start([c for ct in range(NI2) for c in c_oa[ct]])

    def attend_units(memory, filler=None):
        def body(i, c):
            prev = jnp.where(i > 0, 2 * i - 1, 4 * NG)
            late = functools.partial(write_heads, prev, 0, late_v[0:96], late_v[96:192] if memory else None)
            for n in range(2):
                unit, final = 2 * i + n, n == 1
                attend(None if filler and final else unit + 1, s_v[1 - n % 2], zero_s[0],
                       unit, s_v[n % 2], zero_s[1], memory, first=n == 0, final=final, filler=filler,
                       late=late if n == 0 else None)
            if filler is None:
                prepare_queries(2 * i + 3)
            return c
        return body

    def transpose_heads(tile):
        on_v, sp_on = heads[tile // 4]

        def one(ft):
            rows = pl.ds(64 * (tile % 4), 64)
            on_v[ft, rows, :] = _pk(_upk(ot_v[tile, 64 * ft:64 * ft + 64, :]).T)

        return [block(20, None, sp_on, one, ft) for ft in range(NT)]

    def out_project(tile, nt, pace):
        on_v = heads[tile // 4][0]
        parts = [on_v[ft, _ds(64 * (tile % 4) + zero_s[0], 64), :] for ft in range(NT)]
        parts[0] = pace.pace(parts[0], PACE4)
        y = _dot(_upk(jnp.concatenate(parts, axis=1)), _upk(wo_v[nt]))
        pace.note(y)
        ob_b[nt, pl.ds(128 * tile, 128), :] = y.astype(bf16)

    def phase4():
        cts = list(range(NI2, NT))
        for n, (t0, t1) in enumerate(OUT_CHUNKS):
            nxt = OUT_CHUNKS[n + 1] if n + 1 < len(OUT_CHUNKS) else (0, 0)
            blocks = [b for t in range(*nxt) for b in transpose_heads(t)]
            mine = cts[HOST4[n]:HOST4[n + 1]]
            blocks = merge(blocks, [b for ct in mine for b in inverse(ct, zero_s[1])])
            pace = pacer(blocks, (t1 - t0) * NT * 8 // PACE4, 0)
            pieces = [functools.partial(out_project, t, nt) for t in range(t0, t1) for nt in range(NT)]
            if n == 0:
                count = itertools.count()
                attend_units(True, lambda: pieces.pop(0)(pace) if next(count) < FILL4 else None)(
                    2 * NG - 1, 0)
            pace.run(pieces)
            start([c for ct in mine for c in c_oa[ct]] + c_ob[n])

    fill_masks()
    phase0()
    lax.fori_loop(0, NT - 1, phase1, 0)
    phase2()
    lax.fori_loop(0, NG // 2, attend_units(False), 0)
    lax.fori_loop(NG // 2, 2 * NG - 1, attend_units(True), 0)
    for tile in range(*OUT_CHUNKS[0]):
        for b in transpose_heads(tile):
            b[1]()
    phase4()
    for cs in c_oa + c_ob:
        wait(cs)


@jax.jit
def pallas_concat_heads__ssm_conv_h3__memory_aug_infini_attn__prompt_kernel(
    A_q: jax.Array,
    A_k: jax.Array,
    A_v: jax.Array,
    A_shift_k: jax.Array,
    A_ssm_k: jax.Array,
    A_ssm_D: jax.Array,
    B_x: jax.Array,
    B_wq: jax.Array,
    B_wk: jax.Array,
    B_wv: jax.Array,
    B_wo: jax.Array,
    B_beta: jax.Array,
):
    hbm = pl.BlockSpec(memory_space=pl.ANY)
    V = pltpu.VMEM
    scratch = [
        V((NT, S, 128), bf16),
        V((NT, D, 128), bf16), V((NT, D, 128), bf16),
        V((NT, D, 128), bf16), V((NT, D, 128), bf16),
        V((NT + 1, S + 16, 128), bf16), V((NT, S, 128), bf16),
        V((NT, 128, S), bf16), V((NT, S, 128), bf16),
        V((M1, 64, 128), u32), V((M1, 64, 128), u32),
        *[V((2, S, 128), bf16)] * NT, V((NT, S, 128), bf16),
        V((NT + 1, NT, 128, 128), u32),
        V((NT + 1, S // 2, 128), u32),
        V((3, 16 * M1, 128), f32), V((3, 16 * M1, 128), f32),
        V((3, 8 * M1, 128), f32),
        V((NT, 5, 8, 128), f32),
        V((NT + 1, M1, 128, 128), bf16), V((NT + 1, M1, 128, 128), bf16),
        *[V((1, M1 + 1, 128, 128), f32)] * NT,
        *[V((NT + 1, 128 * n, 128), bf16) for n in (2, 4, 6, 4)],
        V((NG + 1, S // 2, 128), u32),
        V((16, D, 128), bf16), V((16, D, 128), bf16),
        V((16, D, 128), f32), V((17, D, 128), bf16),
        *[V((NT + 1, SEG // 2, 128), u32)] * 4,
        *[V((1, 4, 128 * j + 136, 128), f32) for j in range(4)] * 2,
        V((NG, 88, 128), f32),
        V((4 * NG, 8, 128), f32),
        V((3, 64, 128), f32),
        V((4, 16, 128), u32),
        V((192, 128), f32),
        V((4, D), bf16), V((D,), bf16), V((4 * NG,), bf16),
        pltpu.SMEM((3,), i32),
        pltpu.SemaphoreType.DMA((40,)),
    ]
    out = pl.pallas_call(
        _kernel,
        out_shape=jax.ShapeDtypeStruct((S, 2 * D), bf16),
        in_specs=[hbm] * 14,
        out_specs=hbm,
        scratch_shapes=scratch,
        compiler_params=pltpu.CompilerParams(vmem_limit_bytes=110 * 2**20),
    )(
        A_q.reshape(S, D), A_k.reshape(S, D), A_v.reshape(S, D), A_shift_k.T, A_ssm_k, A_ssm_D,
        B_x.reshape(S, D), B_wq, B_wk, B_wv, B_wo, B_beta, _G_FWD, _G_INV,
    )
    return out.reshape(1, S, 2 * D)
```

```python
import functools
import itertools
import math

import jax
import jax.numpy as jnp
import ml_dtypes
import numpy as np
from jax import lax
from jax.experimental import pallas as pl
from jax.experimental.pallas import tpu as pltpu

S = 2048
D = 640
NT = D // 128
DH = 20
NG = 8
SEG = 512
M1, M2 = 32, 64

bf16 = jnp.bfloat16
f32 = jnp.float32
u32 = jnp.uint32
i32 = jnp.int32

LOG2E = math.log2(math.e)
Q_SCALE = DH ** -0.5 * LOG2E

X_CHUNKS = ((0, 2), (2, 6), (6, 12), (12, 16))
K_FIRST = (0, 2, 6, 12)
PACE0 = 8
PACE1, LEAD1, FREE1, LAG1 = 1, 4, 150, 2
PACE2, LEAD2, FREE2, LAG2 = 4, 4, 400, 4
LOOK2 = 5
NF2, NI2 = 3, 2
UPDATE3 = (0, 1, 2, 2)
PACE4 = 4
FILL4 = 10
OUT_CHUNKS = ((0, 4), (4, 8), (8, 12), (12, 15), (15, 16))
HOST4 = (0, 1, 2, 3, 3, 3)


def _neg(a):
    return None if a is None else (-a[0], a[1])


def _add(a, b):
    if a is None:
        return b
    if b is None:
        return a
    if a[0] == b[0]:
        return (a[0], a[1] + b[1])
    if a[0] > 0:
        return (1, a[1] - b[1])
    return (1, b[1] - a[1])


def _sub(a, b):
    return _add(a, _neg(b))


def _scale(a, c):
    if a is None or abs(c) < 1e-12:
        return None
    if abs(abs(c) - 1.0) < 1e-12:
        return a if c > 0 else _neg(a)
    return (a[0], a[1] * float(c))


def _cmul(z, ang):
    c, s = math.cos(ang), math.sin(ang)
    x, y = z
    if x is not None and y is not None and abs(abs(c) - abs(s)) < 1e-12:
        r = 1.0 if c * s > 0 else -1.0
        if r > 0:
            return (_scale(_sub(x, y), c), _scale(_add(y, x), c))
        return (_scale(_add(x, y), c), _scale(_sub(y, x), c))
    return (_sub(_scale(x, c), _scale(y, s)), _add(_scale(y, c), _scale(x, s)))


def _cadd(a, b):
    return (_add(a[0], b[0]), _add(a[1], b[1]))


def _csub(a, b):
    return (_sub(a[0], b[0]), _sub(a[1], b[1]))


def _dif_step(a, b, c, d, j, n):
    t1, t2 = _csub(a, c), _csub(b, d)
    mi_t2 = (t2[1], _neg(t2[0]))
    return (_cadd(a, c), _cadd(b, d),
            _cmul(_cadd(t1, mi_t2), -2 * math.pi * j / n),
            _cmul(_csub(t1, mi_t2), -6 * math.pi * j / n))


def _dit_step(e0, e1, o1, o3, j, n):
    a, b = _cmul(o1, 2 * math.pi * j / n), _cmul(o3, 6 * math.pi * j / n)
    s, d = _cadd(a, b), _csub(a, b)
    i_d = (_neg(d[1]), d[0])
    return _cadd(e0, s), _cadd(e1, i_d), _csub(e0, s), _csub(e1, i_d)


def _fft(z):
    n = len(z)
    if n == 1:
        return list(z)
    if n == 2:
        return [_cadd(z[0], z[1]), _csub(z[0], z[1])]
    q = n // 4
    steps = [_dif_step(*z[j::q], j, n) for j in range(q)]
    out = [None] * n
    out[0::2] = _fft([s[0] for s in steps] + [s[1] for s in steps])
    out[1::4] = _fft([s[2] for s in steps])
    out[3::4] = _fft([s[3] for s in steps])
    return out


def _ifft(z):
    n = len(z)
    if n == 1:
        return list(z)
    if n == 2:
        return [_cadd(z[0], z[1]), _csub(z[0], z[1])]
    q = n // 4
    e, o1, o3 = _ifft(z[0::2]), _ifft(z[1::4]), _ifft(z[3::4])
    out = [None] * n
    for j in range(q):
        out[j::q] = _dit_step(e[j], e[j + q], o1[j], o3[j], j, n)
    return out


_SUBS = ((0, 8, 0, 4), (8, 8, 1, 4), (16, 8, 3, 4), (24, 4, 2, 8), (28, 4, 6, 8))


def _fwd_first(j, xs):
    z = [_cmul(((1, x), None), -2 * math.pi * (j + 4 * m) / (4 * M1)) for m, x in enumerate(xs)]
    lo, hi = _dif_step(*z[0::2], j, 32), _dif_step(*z[1::2], j + 4, 32)
    mid = _dif_step(lo[0], hi[0], lo[1], hi[1], j, 16)
    return {j: mid[0], j + 4: mid[1], 8 + j: lo[2], 12 + j: hi[2],
            16 + j: lo[3], 20 + j: hi[3], 24 + j: mid[2], 28 + j: mid[3]}


def _inv_last(j, w):
    mid = _dit_step(w[j], w[j + 4], w[24 + j], w[28 + j], j, 16)
    lo = _dit_step(mid[0], mid[2], w[8 + j], w[16 + j], j, 32)
    hi = _dit_step(mid[1], mid[3], w[12 + j], w[20 + j], j + 4, 32)
    z = [None] * 8
    z[0::2], z[1::2] = lo, hi
    return [_cmul(v, 2 * math.pi * (j + 4 * m) / (4 * M1))[0] for m, v in enumerate(z)]


def _slots(j):
    return (j, j + 4, 8 + j, 12 + j, 16 + j, 20 + j, 24 + j, 28 + j)


def _codelet_signs():
    one = (1, 1.0)
    mid = {}
    for j in range(4):
        mid.update(_fwd_first(j, [1.0] * 8))
    mid = {s: (v[0][0], v[1][0]) for s, v in mid.items()}
    out = {}
    for s0, n, k0, dk in _SUBS:
        ys = _fft([((mid[s0 + i][0], 1.0), (mid[s0 + i][1], 1.0)) for i in range(n)])
        out.update({k0 + dk * i: (y[0][0], y[1][0]) for i, y in enumerate(ys)})
    imid = {}
    for s0, n, _, _ in _SUBS:
        imid.update({s0 + i: (w[0][0], w[1][0]) for i, w in enumerate(_ifft([(one, one)] * n))})
    return mid, out, imid


_FWD_MID_SIGNS, _FWD_SIGNS, _INV_MID_SIGNS = _codelet_signs()


class _Pacer:
    def __init__(self, never, blocks, slots, lead=0, free=0, lag=2):
        self.never, self.blocks, self.slots, self.lag = never, list(blocks), slots - lead, lag
        self.total = sum(b[0] for b in self.blocks) - free
        self.slot, self.spent, self.results = -lead, 0, []

    def note(self, result):
        self.results.append(result[:8])

    def _run_block(self):
        cost, fn, release, word = self.blocks.pop(0)
        self.spent += cost
        if release is not None and len(self.results) >= self.lag > 0:
            release(self.results[-self.lag])
        fn()
        return word

    def pace(self, x, every):
        parts = [x[8 * r:8 * r + 8] for r in range(x.shape[0] // 8)]
        for r in range(0, len(parts), every):
            self.slot += 1
            words = []
            while self.blocks and ((self.spent + self.blocks[0][0] / 2) * self.slots
                                   <= self.total * min(self.slot, self.slots)):
                word = self._run_block()
                if word not in words:
                    words.append(word)
            for word in words:
                parts[r] = jnp.where(self.never, word(), parts[r])
        return jnp.concatenate(parts, axis=0)

    def run(self, pieces):
        for piece in pieces:
            piece(self)
        while self.blocks:
            self._run_block()


def _pack_rows(m):
    b = np.asarray(m, np.float32).astype(ml_dtypes.bfloat16).view(np.uint16).astype(np.uint32)
    return np.ascontiguousarray(b[..., 0::2, :] | (b[..., 1::2, :] << 16))


def _dft_tables():
    r = np.arange(128)
    part = (r // 8) % 2
    nat = 8 * (r // 16) + r % 8
    eo = 16 * (r // 32) + 2 * (r % 8) + (r // 16) % 2
    fwd = np.zeros((M1, 128, 128))
    inv = np.zeros((M1, 128, 128))
    for k1 in range(M1):
        freq = k1 + M1 * nat + 0.25
        ph = 2 * np.pi * freq[:, None] * eo[None, :] / S
        same = part[:, None] == part[None, :]
        cross = np.where(part[:, None] == 0, 1.0, -1.0)
        sg = np.where(part == 0, _FWD_SIGNS[k1][0], _FWD_SIGNS[k1][1])
        fwd[k1] = np.where(same, np.cos(ph), cross * np.sin(ph)) * sg[None, :]
        ph = 2 * np.pi * nat[:, None] * freq[None, :] / S
        inv[k1] = np.where(same, np.cos(ph), -cross * np.sin(ph)) / S
    return _pack_rows(fwd), _pack_rows(inv)


_G_FWD, _G_INV = _dft_tables()


def _pk(x):
    return pltpu.bitcast(x, u32)


def _upk(x):
    return pltpu.bitcast(x, bf16)


def _even(x):
    return pltpu.bitcast(x << 16, f32)


def _odd(x):
    return pltpu.bitcast(x & jnp.uint32(0xFFFF0000), f32)


def _dot(a, b):
    return lax.dot_general(a, b, (((1,), (0,)), ((), ())), preferred_element_type=f32)


def _dot_t(a, b):
    return lax.dot_general(a, b, (((1,), (1,)), ((), ())), preferred_element_type=f32)


def _phi(t):
    return jnp.where(t > 0, t + 1.0, jnp.exp2(t * LOG2E))


def _recip(x):
    r = pltpu.reciprocal(x, approx=True)
    return r * (2.0 - x * r)


def _ds(start, size, align=8):
    return pl.ds(pl.multiple_of(start, align), size)


def _kernel(
    q_hbm, k_hbm, v_hbm, shift_hbm, h_hbm, d_hbm,
    x_hbm, wq_hbm, wk_hbm, wv_hbm, wo_hbm, beta_hbm, gf_hbm, gi_hbm,
    out_hbm,
    x_b, wq_b, wk_b, wv_b, wo_b, k_b, v_b, h_b, q_b, gf_v, gi_v,
    oa0_b, oa1_b, oa2_b, oa3_b, oa4_b, ob_b,
    wt_v, ht_v, mx_v, mh_v, kv_v, par_v, yx_b, yh_b, u0_v, u1_v, u2_v, u3_v, u4_v,
    k0_b, k1_b, k2_b, k3_b, kg_v, qt_b, pqt_b, vt_v, ot_b, on0_v, on1_v, on2_v, on3_v,
    sa0_v, sa1_v, sa2_v, sa3_v, sb0_v, sb1_v, sb2_v, sb3_v,
    mem_v, gate_v, mask_v, first_q, late_v, shift_ref, d_ref, beta_ref, zero_s, sems,
):
    u_v = (u0_v, u1_v, u2_v, u3_v, u4_v)
    kt_b = (k0_b, k1_b, k2_b, k3_b)
    s_v = ((sa0_v, sa1_v, sa2_v, sa3_v), (sb0_v, sb1_v, sb2_v, sb3_v))
    oa_b = (oa0_b, oa1_b, oa2_b, oa3_b, oa4_b)
    x_v, wq_v, wk_v, wv_v, wo_v = (r.bitcast(u32) for r in (x_b, wq_b, wk_b, wv_b, wo_b))
    k_v, v_v, h_v, q_v = (r.bitcast(u32) for r in (k_b, v_b, h_b, q_b))
    yx_v, yh_v = (r.bitcast(u32) for r in (yx_b, yh_b))
    oa_v = [r.bitcast(u32) for r in oa_b]
    kt_v = [r.bitcast(u32) for r in kt_b]
    qt_v, pqt_v, ot_v = (r.bitcast(u32) for r in (qt_b, pqt_b, ot_b))

    n_sem = [0]

    def group(pairs):
        sem = sems.at[n_sem[0]]
        n_sem[0] += 1
        return [pltpu.make_async_copy(src, dst, sem) for src, dst in pairs]

    def cols(t):
        return pl.ds(128 * t, 128)

    def weight(hbm, buf):
        return group([(hbm.at[:, cols(t)], buf.at[t]) for t in range(NT)])

    def xrows(r0, n):
        return group([(x_hbm.at[pl.ds(r0, n), cols(t)], x_b.at[t, pl.ds(r0, n)]) for t in range(NT)])

    c_wk = [group([(wk_hbm.at[:, cols(t)], wk_b.at[t])]) for t in range(NT)]
    c_wq, c_wv, c_wo = (weight(a, b) for a, b in ((wq_hbm, wq_b), (wv_hbm, wv_b), (wo_hbm, wo_b)))
    c_x = [xrows(128 * t0, 128 * (t1 - t0)) for t0, t1 in X_CHUNKS]
    c_h = [group([(h_hbm.at[cols(t)], h_b.at[t])]) for t in range(NT)]
    c_kv = [group([(k_hbm.at[:, cols(t)], k_b.at[t, pl.ds(16, S)]),
                   (v_hbm.at[:, cols(t)], v_b.at[t])]) for t in range(NT)]
    c_g = group([(gf_hbm, gf_v), (gi_hbm, gi_v)])
    c_q = group([(q_hbm.at[:, cols(t)], q_b.at[t]) for t in range(NT)])
    c_oa = [group([(oa_b[t].at[0], out_hbm.at[:, cols(t)])]) for t in range(NT)]
    c_ob = [group([(ob_b.at[t, pl.ds(128 * t0, 128 * (t1 - t0))],
                    out_hbm.at[pl.ds(128 * t0, 128 * (t1 - t0)), cols(NT + t)]) for t in range(NT)])
            for t0, t1 in OUT_CHUNKS]

    def start(cs):
        for c in cs:
            c.start()

    def wait(cs):
        for c in cs:
            c.wait()

    def wait_when(cond, cs):
        pl.when(cond)(lambda: wait(cs))

    c_par = group([(shift_hbm, shift_ref), (d_hbm, d_ref), (beta_hbm, beta_ref)])
    start(c_x[0] + c_wk[0] + c_wk[1])

    sub8 = lax.broadcasted_iota(i32, (8, 128), 0)
    lane8 = lax.broadcasted_iota(i32, (8, 128), 1)

    zero_s[0] = 0
    zero_s[1] = 0
    zero_s[2] = 0

    def unpack_parameters():
        taps = shift_ref[...].astype(f32)
        skip = d_ref[...].astype(f32).reshape(1, D)
        for t in range(NT):
            for j in range(4):
                par_v[t, j] = jnp.broadcast_to(taps[j:j + 1, 128 * t:128 * t + 128], (8, 128))
            par_v[t, 4] = jnp.where(sub8 == 0, skip[:, 128 * t:128 * t + 128], 0.0)
            k_v[t, 0:8, :] = jnp.zeros((8, 128), u32)
        beta = beta_ref[...].astype(f32).reshape(1, 4 * NG)
        gate = 1.0 / (1.0 + jnp.exp(-beta))
        for h in range(4 * NG):
            gate_v[h] = jnp.broadcast_to(gate[:, h:h + 1], (8, 128))


    def key_buffer(tile):
        n = max(i for i, first in enumerate(K_FIRST) if first <= tile)
        return n, K_FIRST[n]

    def project_k(tile, ft, pace):
        parts = [x_v[kt, pl.ds(64 * tile, 64), :] for kt in range(NT)]
        parts[0] = pace.pace(parts[0], PACE0)
        k = _dot(_upk(jnp.concatenate(parts, axis=1)), _upk(wk_v[ft]))
        pace.note(k)
        n, first = key_buffer(tile)
        kt_b[n][ft, pl.ds(128 * (tile - first), 128), :] = k.astype(bf16)

    def project_qv(tile, ft, half, pace):
        xt = _upk(jnp.concatenate([x_v[kt, _ds(tile * 64, 64), :] for kt in range(NT)], axis=1))
        parts = [wt_v[ft, kt, 64 * half:64 * half + 64, :] for kt in range(NT)]
        parts[0] = pace.pace(parts[0], PACE1)
        y = _dot_t(_upk(jnp.concatenate(parts, axis=1)), xt)
        pace.note(y)
        rows = pl.ds(128 * ft, 128)
        if half == 0:
            qt_b[tile, rows, :] = (y * Q_SCALE).astype(bf16)
            pqt_b[tile, rows, :] = _phi(y).astype(bf16)
        else:
            vt_v[tile, rows, :] = y

    class Spare:
        def __init__(self, view, *idx):
            self.view, self.idx = view, idx
            view[(*idx, slice(0, 8), slice(None))] = jnp.zeros((8, 128), view.dtype)

        def word(self):
            return pltpu.bitcast(self.view[(*self.idx, _ds(zero_s[2], 8), slice(None))], u32)

        def release(self, value):
            self.view[(*self.idx, _ds(zero_s[2] + 8, 8), slice(None))] = pltpu.bitcast(value, self.view.dtype)

    sp_ht, sp_k, sp_kv = Spare(ht_v, NT), Spare(k_v, NT), Spare(kv_v, 2)
    sp_mx, sp_mh, sp_yx, sp_yh = Spare(mx_v, 2), Spare(mh_v, 2), Spare(yx_v, NT, 0), Spare(yh_v, NT, 0)
    sp_oa, sp_kt, sp_kg = [Spare(r, 1) for r in oa_v], [Spare(r, NT) for r in kt_v], Spare(kg_v, NG)
    sp_u, sp_wt = [Spare(u, 0, M1) for u in u_v], Spare(wt_v, NT, 0)

    heads = [(r, Spare(r, NT)) for r in (on0_v, on1_v, on2_v, on3_v)]

    def block(cost, src, dst, fn, *args):
        return (cost, functools.partial(fn, *args), src.release if src else None, dst.word)

    def transpose_filter(ct):
        def one(t):
            ht_v[ct, pl.ds(64 * t, 64), :] = _pk(_upk(h_v[ct, :, pl.ds(128 * t, 128)]).T)

        return [block(20, None, sp_ht, one, t) for t in range(S // 128)]

    def transpose_weight(half, w_v):
        def one(ft, kt):
            wt_v[ft, kt, 64 * half:64 * half + 64, :] = _pk(_upk(w_v[ft, 64 * kt:64 * kt + 64, :]).T)

        return [block(20, None, sp_wt, one, ft, kt) for ft in range(NT) for kt in range(NT)]

    def align_keys(tile0, tile1):
        def one(r):
            n, first = key_buffer(r // 64)
            rows = pl.ds(r - 64 * first, 16)
            lane = lax.broadcasted_iota(i32, (16, 128), 1)
            for g in range(NG):
                t, off = divmod(80 * g, 128)
                x = kt_v[n][t, rows, :]
                if off > 48:
                    x = jnp.where(lane >= off, x, kt_v[n][t + 1, rows, :])
                kg_v[g, pl.ds(r, 16), :] = pltpu.roll(x, 128 - off, 1) if off else x

        return [block(20, sp_kt[key_buffer(r // 64)[0]], sp_kg, one, r) for r in range(64 * tile0, 64 * tile1, 16)]

    def merge(xs, ys):
        keyed = [((i + 0.5) / len(bs), n, b) for n, bs in enumerate((xs, ys)) for i, b in enumerate(bs)]
        return [b for _, _, b in sorted(keyed, key=lambda e: e[:2])]

    def forward_unit(ct, bb):
        r0 = pl.multiple_of(bb * 8, 8)

        def short_conv(n1):
            w = [par_v[ct, j] for j in range(4)]
            base = r0 + 32 * n1
            p0, p1, p2 = (k_v[ct, pl.ds(base + 8 - j, 8), :] for j in range(3))
            e0, o0, e1, o1, o2 = _even(p0), _odd(p0), _even(p1), _odd(p1), _odd(p2)
            vv = v_v[ct, _ds(base, 8), :]
            return ((w[0] * e0 + w[1] * o1 + w[2] * e1 + w[3] * o2) * _even(vv),
                    (w[0] * o0 + w[1] * e0 + w[2] * o1 + w[3] * e1) * _odd(vv))

        def park(mid, par, vals):
            for s, (re, im) in vals.items():
                mid[par, pl.ds(16 * s, 8), :] = re[1]
                mid[par, pl.ds(16 * s + 8, 8), :] = im[1]

        def conv(n1s):
            for n1 in n1s:
                for par, y in enumerate(short_conv(n1)):
                    kv_v[par, pl.ds(8 * n1, 8), :] = y

        def first_x(j, par):
            xs = [kv_v[par, _ds(8 * (j + 4 * m) + zero_s[2], 8), :] for m in range(8)]
            park(mx_v, par, _fwd_first(j, xs))

        def first_h(j, par):
            xs = [(_odd if par else _even)(ht_v[ct, _ds(r0 + 32 * (j + 4 * m), 8), :]) for m in range(8)]
            if par == 0 and j == 0:
                xs[0] = xs[0] + jnp.where(bb == 0, par_v[ct, 4], 0.0)
            park(mh_v, par, _fwd_first(j, xs))

        def second(mid, dst, par, subs):
            for s0, n, k0, dk in subs:
                zs = [((_FWD_MID_SIGNS[s][0], mid[par, _ds(16 * s + zero_s[2], 8), :]),
                       (_FWD_MID_SIGNS[s][1], mid[par, _ds(16 * s + 8 + zero_s[2], 8), :]))
                      for s in range(s0, s0 + n)]
                for i, (re, im) in enumerate(_fft(zs)):
                    y = jnp.concatenate([re[1], im[1]], axis=0).astype(bf16)
                    dst[ct, k0 + dk * i, _ds(bb * 32 + 16 * par, 16, 16), :] = y

        def seconds(mid, dst, sp_src, sp_dst):
            return [block(64 if len(subs) == 1 else 40, sp_src, sp_dst, second, mid, dst, par, subs)
                    for par in range(2) for subs in (_SUBS[0:1], _SUBS[1:2], _SUBS[2:3], _SUBS[3:5])]

        def firsts(fn, sp_src, sp_dst):
            return [block(95, sp_src, sp_dst, fn, j, par) for par in range(2) for j in range(4)]

        convs = [block(46, sp_k, sp_kv, conv, range(n, n + 2)) for n in range(0, M1, 2)]
        return (firsts(first_h, sp_ht, sp_mh) + convs + seconds(mh_v, yh_b, sp_mh, sp_yh)
                + firsts(first_x, sp_kv, sp_mx) + seconds(mx_v, yx_b, sp_mx, sp_yx))

    def forward(ct):
        return [b for bb in range(4) for b in forward_unit(ct, bb)]

    def pacer(blocks, slots, lead=0, free=0, lag=0):
        return _Pacer(sub8 < zero_s[2], blocks, slots, lead, free, lag)

    def phase0():
        def run(blocks, chunk, fts, lead=0):
            todo = [functools.partial(project_k, tile, ft) for ft in fts for tile in range(*X_CHUNKS[chunk])]
            pacer(blocks, len(todo) * 8 // PACE0, lead).run(todo)

        for cs in (*c_wk[2:], c_par, c_x[1]):
            start(cs)
        wait(c_x[0] + c_wk[0] + c_wk[1])
        run([], 0, range(2))
        start(c_x[2] + c_wq)
        wait(c_wk[2] + c_wk[3] + c_wk[4] + c_par)
        unpack_parameters()
        run([], 0, range(2, NT))
        for cs in (c_x[3], c_wv, c_h[0], c_kv[0], c_h[1]):
            start(cs)
        wait(c_x[1])
        run(align_keys(0, 2), 1, range(NT))
        for cs in (c_kv[1], c_h[2], c_kv[2], c_h[3], c_kv[3], c_h[4], c_kv[4], c_g, c_q, c_wo):
            start(cs)
        wait(c_x[2] + c_wq)
        run(merge(transpose_weight(0, wq_v), align_keys(2, 6)), 2, range(NT), 2)
        wait(c_x[3] + c_wv + c_h[0])
        turns = transpose_weight(1, wv_v) + transpose_filter(0)
        run(merge(turns, align_keys(6, 12)), 3, range(NT), 2)

    def phase1(ct):
        blocks = merge(forward(ct), transpose_filter(ct + 1))
        pieces = [functools.partial(project_qv, 4 * ct + j, ft, half)
                  for j in range(4) for ft in range(NT) for half in range(2)]
        pacer(blocks, len(pieces) * 8 // PACE1, LEAD1, FREE1, LAG1).run(pieces)

    def spectral(ct, u_out, z):
        zs = {}

        def fwd(k1, pace):
            g = _upk(pace.pace(gf_v[k1], PACE2))
            x = _dot(g, _upk(yx_v[ct, k1]))
            h = _dot(g, _upk(yh_v[ct, k1]))
            rows = []
            for a in range(8):
                xr, xi = x[16 * a:16 * a + 8], x[16 * a + 8:16 * a + 16]
                hr, hi = h[16 * a:16 * a + 8], h[16 * a + 8:16 * a + 16]
                rows += [xr * hr - xi * hi, xr * hi + xi * hr]
            pace.note(x)
            zs[k1] = jnp.concatenate(rows, axis=0).astype(bf16)

        def inv(k1, pace):
            u_out[z, k1] = _dot(_upk(pace.pace(gi_v[k1], PACE2)), zs.pop(k1))

        pieces = []
        for k1 in range(M1 + LOOK2):
            if k1 < M1:
                pieces.append(functools.partial(fwd, k1))
            if k1 >= LOOK2:
                pieces.append(functools.partial(inv, k1 - LOOK2))
        return pieces

    def inverse(ct, z):
        u_in = u_v[ct]

        def first(mid, a, subs):
            for s0, n, k0, dk in subs:
                zs = [((1, u_in[z, k, 16 * a:16 * a + 8, :]), (1, u_in[z, k, 16 * a + 8:16 * a + 16, :]))
                      for k in range(k0, M1, dk)]
                for i, (re, im) in enumerate(_ifft(zs)):
                    mid[a % 2, pl.ds(16 * (s0 + i), 8), :] = re[1]
                    mid[a % 2, pl.ds(16 * (s0 + i) + 8, 8), :] = im[1]

        def last(mid, bb, j, par):
            w = {s: ((_INV_MID_SIGNS[s][0], mid[par, _ds(16 * s + zero_s[2], 8), :]),
                     (_INV_MID_SIGNS[s][1], mid[par, _ds(16 * s + 8 + zero_s[2], 8), :]))
                 for s in _slots(j)}
            for m, (sign, y) in enumerate(_inv_last(j, w)):
                n1 = j + 4 * m
                if par == 0:
                    kv_v[0, pl.ds(8 * n1, 8), :] = y
                    continue
                gate_q = _upk(q_v[ct, pl.ds(32 * n1 + 8 * bb, 8), :]).astype(f32)
                y = jnp.concatenate([kv_v[0, _ds(8 * n1 + zero_s[2], 8), :], y], axis=0) * gate_q
                oa_b[ct][0, pl.ds(64 * n1 + 16 * bb, 16), :] = (y if sign > 0 else -y).astype(bf16)

        blocks = []
        for bb in range(4):
            mid, sp_mid = (mh_v, sp_mh) if bb % 2 else (mx_v, sp_mx)
            blocks += [block(56 if len(subs) == 1 else 32, sp_u[ct], sp_mid, first, mid, a, subs)
                       for a in (2 * bb, 2 * bb + 1)
                       for subs in (_SUBS[0:1], _SUBS[1:2], _SUBS[2:3], _SUBS[3:5])]
            blocks += [block(125 if par else 85, sp_mid, sp_oa[ct] if par else sp_kv, last, mid, bb, j, par)
                       for par in range(2) for j in range(4)]
        return blocks

    def stream(cts, z):
        return [piece for ct in cts for piece in spectral(ct, u_v[ct], z)]

    prow = lax.broadcasted_iota(i32, (16, 128), 0)
    steps = [(j, t) for j in (3, 2, 1, 0) for t in range(j + 1)]

    def fill_masks():
        key = lax.broadcasted_iota(i32, (64, 128), 0)
        lane = lax.broadcasted_iota(i32, (64, 128), 1)
        for n, query in enumerate((lane, (lane + 64) & 127, lane & 63)):
            mask_v[n] = jnp.where(key <= query, 0.0, -1e9 * LOG2E).astype(f32)

    def head_queries(unit, j):
        out = []
        for i in range(4):
            own = (prow >= 2 * i) & (prow < 2 * i + 10)
            w = qt_v[4 * (unit >> 3) + j, _ds(40 * (unit & 7) + 8 * i, 16), :]
            out.append(jnp.where(own, pltpu.roll(w, 64, 1) if i % 2 else w, jnp.uint32(0)))
        return out

    def prepare_queries(unit):
        for i, w in enumerate(head_queries(unit, 3)):
            first_q[i] = w

    def write_heads(unit, j, local, stored):
        low = sub8 < 4
        gates = [gate_v[4 * (unit & 7) + i] for i in range(4)]
        rows = []
        for i in (0, 2):
            a, b = local[24 * i:24 * i + 24], pltpu.roll(local[24 * i + 24:24 * i + 48], 64, 1)
            inv = _recip(jnp.where(low, b[0:8], a[16:24])) * (1.0 - jnp.where(low, gates[i + 1], gates[i]))
            swap = pltpu.roll(inv, 4, 0)
            first, second = jnp.where(low, swap, inv), jnp.where(low, inv, swap)
            rows += [a[0:8] * first, a[8:16] * first, jnp.where(low, a[16:24], b[0:8]) * swap,
                     b[8:16] * second, b[16:24] * second]
        if stored is not None:
            for n in range(2):
                inv = _recip(stored[80 + 8 * n:88 + 8 * n] + 1e-6)
                swap = pltpu.roll(inv, 4, 0)
                scales = [jnp.where(low, inv, swap)] * 2 + [inv] + [jnp.where(low, swap, inv)] * 2
                for b in range(5):
                    rows[5 * n + b] = rows[5 * n + b] + stored[40 * n + 8 * b:40 * n + 8 * b + 8] * scales[b]
        ot_b[4 * (unit >> 3) + j, _ds(80 * (unit & 7), 80, 16), :] = jnp.concatenate(rows, axis=0).astype(bf16)

    def attend(uq, s_out, zo, up, s_in, zi, memory, pace=None, first=False, final=False, filler=None,
               late=None):
        low, left = sub8 < 4, lane8 < 64
        if uq is not None:
            sq, gq = uq >> 3, uq & 7
        if up is not None:
            sp, gp = up >> 3, up & 7
            gates = [gate_v[4 * gp + i] for i in range(4)]
        weights, run_max, acc = {}, {}, {}

        def stack(*parts):
            rows = sum(x.shape[0] for x in parts)
            return jnp.concatenate([x for x in parts if x.shape[0]] + [jnp.zeros((64 - rows, 128), u32)], axis=0)

        def q_weights(j):
            if j not in weights:
                if first and j == 3:
                    qw = [first_q[i] for i in range(4)]
                else:
                    qw = head_queries(uq, j)
                single = [stack(jnp.zeros((8 * i, 128), u32), qw[i]) for i in range(4)]
                shared = []
                for i in (0, 2):
                    a, b = qw[i], qw[i + 1]
                    shared.append(stack(jnp.zeros((8 * i, 128), u32), jnp.where(left, 0, a[:8]),
                                        jnp.where(left, b[:8], a[8:]), jnp.where(left, b[8:], 0)))
                weights[j] = (_upk(jnp.concatenate(single, axis=1)), [_upk(w) for w in shared])
            return weights[j]

        def keys(t, r0, n):
            x = kg_v[gq, _ds(256 * sq + 64 * t + r0 // 2, n // 2), :]
            return _upk(pace.pace(x, 2) if pace else x)

        def column_max(x):
            return jnp.max(x.reshape(x.shape[0] // 8, 8, 128), axis=0)

        def reduce_max(x):
            return jnp.broadcast_to(jnp.max(x, axis=0, keepdims=True), (8, 128))

        def score(j, t):
            single, shared = q_weights(j)
            if t < j:
                return _dot(keys(t, 0, 128), single), None
            main = _dot(keys(t, 0, 64), single)
            tail = [jnp.concatenate([_dot(keys(t, r, 32), w) for r in (64, 96)], axis=0) for w in shared]
            return main, tail

        def keep(j, t, main, tail):
            if pace:
                pace.note(main[:, :128])
            if tail is not None:
                tail = [x + mask_v[2] for x in tail]
                for n, x in enumerate(tail):
                    s_out[j][zo, 2 * n, pl.ds(128 * j + 64, 64)] = x
                tail = [column_max(x) for x in tail]
            for i in range(4):
                st = main[:, 128 * i:128 * i + 128]
                if t == j:
                    st = st + mask_v[i % 2]
                    s_out[j][zo, i, pl.ds(128 * j, 64)] = st
                else:
                    s_out[j][zo, i, pl.ds(128 * t, 128)] = st
                mx = column_max(st)
                run_max[j, i] = mx if t == 0 else jnp.maximum(run_max[j, i], mx)
                if t == j:
                    mine = left if i % 2 else ~left
                    mx = jnp.where(mine, jnp.maximum(run_max[j, i], tail[i // 2]), run_max[j, i])
                    s_out[j][zo, i, pl.ds(128 * j + 128, 8)] = reduce_max(mx) if j else mx

        def expo(x, m):
            return jnp.exp2(x.reshape(x.shape[0] // 8, 8, 128) - m[None]).reshape(x.shape).astype(bf16)

        def probs(j, t):
            m = [s_in[j][zi, i, pl.ds(128 * j + 128, 8)] for i in range(4)]
            if j == 0:
                m = [reduce_max(x) for x in m]
            if t < j:
                return [expo(s_in[j][zi, i, pl.ds(128 * t, 128)], m[i]) for i in range(4)]
            ps = []
            half = lax.broadcasted_iota(i32, (32, 128), 1) < 64
            for i in (0, 2):
                tail = _pk(expo(s_in[j][zi, i, pl.ds(128 * j + 64, 64)], jnp.where(left, m[i + 1], m[i])))
                for n, part in enumerate((jnp.where(half, 0, tail), jnp.where(half, tail, 0))):
                    main = expo(s_in[j][zi, i + n, pl.ds(128 * j, 64)], m[i + n])
                    ps.append(jnp.concatenate([main, _upk(part)], axis=0))
            return ps

        def v_rows(i, t):
            r0 = (0, 16, 40, 56)[i]
            v = [vt_v[4 * sp + t, _ds(80 * gp + r0 + 8 * b, 8), :] for b in range(3)]
            if i % 2:
                v[0] = jnp.where(low, 1.0, v[0])
            else:
                v[2] = jnp.where(low, v[2], 1.0)
            return jnp.concatenate(v, axis=0)

        mem = {}

        def memory_update(t):
            tile = 4 * (sp - 1) + t
            pk_t = _phi(_upk(kg_v[gp, _ds(tile * 64, 64), :]).astype(f32)).astype(bf16)
            lhs = jnp.concatenate([vt_v[tile, _ds(80 * gp, 80), :], jnp.ones((8, 128), f32)], axis=0)
            d = _dot(lhs, pk_t)
            mem["sum"] = d if t == 0 else mem["sum"] + d
            if t < 3:
                return
            m = mem_v[gp] + mem["sum"]
            mem_v[gp] = m
            own = [(lane8 >= DH * i) & (lane8 < DH * i + DH) for i in range(4)]
            rows = []
            for r in range(10):
                lo, hi = (8 * r) // DH, (8 * r + 7) // DH
                blk = m[8 * r:8 * r + 8]
                a = jnp.where(own[lo], blk * gates[lo], 0.0)
                if hi != lo:
                    a = jnp.where(low, a, jnp.where(own[hi], blk * gates[hi], 0.0))
                rows.append(a)
            rows += [jnp.where((low & own[i]) | (~low & own[i + 1]), m[80:88], 0.0) for i in (0, 2)]
            mem["lhs"] = jnp.concatenate(rows, axis=0).astype(bf16)

        def memory_read(j):
            w = jnp.concatenate([pqt_v[4 * sp + j, _ds(40 * gp, 40), :], jnp.zeros((24, 128), u32)], axis=0)
            return _dot(mem["lhs"], _upk(w))

        def finish(j):
            local = jnp.concatenate([acc[j, i] for i in range(4)], axis=0)
            stored = memory_read(j) if memory else None
            if final and j == 0 and filler is None:
                late_v[0:96] = local
                late_v[96:192] = stored if memory else jnp.zeros((96, 128), f32)
            else:
                write_heads(up, j, local, stored)

        def weigh(j, t, ps):
            for i in range(4):
                d = _dot(v_rows(i, t), ps[i])
                acc[j, i] = d if t == 0 else acc[j, i] + d
            if t == j:
                finish(j)

        def update(n):
            if late is not None and n == 0:
                late()
            for t in range(4):
                if memory and UPDATE3[t] == n:
                    memory_update(t)

        for n, (j, t) in enumerate(steps):
            if up is None:
                keep(j, t, *score(j, t))
            elif uq is None:
                filler()
                update(n)
                weigh(j, t, probs(j, t))
            else:
                scores = score(j, t)
                update(n)
                ps = probs(j, t)
                keep(j, t, *scores)
                weigh(j, t, ps)

    def phase2():
        z0, z1 = zero_s[0], zero_s[1]
        slots = 64 * 8 // PACE2
        pacer(forward(NT - 1), NF2 * slots, LEAD2, 0, LAG2).run(stream(range(NF2), z0))
        blocks = merge([b for ct in range(NI2) for b in inverse(ct, z1)], align_keys(12, 16))
        pacer(blocks, (NT - NF2) * slots + 36, 0, FREE2, LAG2).run(
            stream(range(NF2, NT), z0) + [lambda p: attend(0, s_v[0], z0, None, None, None, False, p)])
        prepare_queries(1)
        start([c for ct in range(NI2) for c in c_oa[ct]])

    def attend_units(memory, filler=None):
        def body(i, c):
            prev = jnp.where(i > 0, 2 * i - 1, 4 * NG)
            late = functools.partial(write_heads, prev, 0, late_v[0:96], late_v[96:192] if memory else None)
            for n in range(2):
                unit, final = 2 * i + n, n == 1
                attend(None if filler and final else unit + 1, s_v[1 - n % 2], zero_s[0],
                       unit, s_v[n % 2], zero_s[1], memory, first=n == 0, final=final, filler=filler,
                       late=late if n == 0 else None)
            if filler is None:
                prepare_queries(2 * i + 3)
            return c
        return body

    def transpose_heads(tile):
        on_v, sp_on = heads[tile // 4]

        def one(ft):
            rows = pl.ds(64 * (tile % 4), 64)
            on_v[ft, rows, :] = _pk(_upk(ot_v[tile, 64 * ft:64 * ft + 64, :]).T)

        return [block(20, None, sp_on, one, ft) for ft in range(NT)]

    def out_project(tile, nt, pace):
        on_v = heads[tile // 4][0]
        parts = [on_v[ft, _ds(64 * (tile % 4) + zero_s[0], 64), :] for ft in range(NT)]
        parts[0] = pace.pace(parts[0], PACE4)
        y = _dot(_upk(jnp.concatenate(parts, axis=1)), _upk(wo_v[nt]))
        pace.note(y)
        ob_b[nt, pl.ds(128 * tile, 128), :] = y.astype(bf16)

    def phase4():
        cts = list(range(NI2, NT))
        for n, (t0, t1) in enumerate(OUT_CHUNKS):
            nxt = OUT_CHUNKS[n + 1] if n + 1 < len(OUT_CHUNKS) else (0, 0)
            blocks = [b for t in range(*nxt) for b in transpose_heads(t)]
            mine = cts[HOST4[n]:HOST4[n + 1]]
            blocks = merge(blocks, [b for ct in mine for b in inverse(ct, zero_s[1])])
            pace = pacer(blocks, (t1 - t0) * NT * 8 // PACE4, 0)
            pieces = [functools.partial(out_project, t, nt) for t in range(t0, t1) for nt in range(NT)]
            if n == 0:
                count = itertools.count()
                attend_units(True, lambda: pieces.pop(0)(pace) if next(count) < FILL4 else None)(
                    2 * NG - 1, 0)
            pace.run(pieces)
            start([c for ct in mine for c in c_oa[ct]] + c_ob[n])

    fill_masks()
    mem_v[...] = jnp.zeros(mem_v.shape, f32)
    late_v[...] = jnp.ones(late_v.shape, f32)
    phase0()
    @pl.loop(0, NT - 2)
    def _(ct):
        for t in range(NT - 2):
            wait_when(ct == t, c_kv[t] + c_h[t + 1])
        phase1(ct)

    wait(c_kv[NT - 2] + c_h[NT - 1] + c_kv[NT - 1] + c_g + c_q + c_wo)
    phase1(NT - 2)
    phase2()
    lax.fori_loop(0, NG // 2, attend_units(False), 0)
    lax.fori_loop(NG // 2, 2 * NG - 1, attend_units(True), 0)
    for tile in range(*OUT_CHUNKS[0]):
        for b in transpose_heads(tile):
            b[1]()
    phase4()
    for cs in c_oa + c_ob:
        wait(cs)


@jax.jit
def pallas_concat_heads__ssm_conv_h3__memory_aug_infini_attn__prompt_kernel(
    A_q: jax.Array,
    A_k: jax.Array,
    A_v: jax.Array,
    A_shift_k: jax.Array,
    A_ssm_k: jax.Array,
    A_ssm_D: jax.Array,
    B_x: jax.Array,
    B_wq: jax.Array,
    B_wk: jax.Array,
    B_wv: jax.Array,
    B_wo: jax.Array,
    B_beta: jax.Array,
):
    hbm = pl.BlockSpec(memory_space=pl.ANY)
    V = pltpu.VMEM
    scratch = [
        V((NT, S, 128), bf16),
        V((NT, D, 128), bf16), V((NT, D, 128), bf16),
        V((NT, D, 128), bf16), V((NT, D, 128), bf16),
        V((NT + 1, S + 16, 128), bf16), V((NT, S, 128), bf16),
        V((NT, 128, S), bf16), V((NT, S, 128), bf16),
        V((M1, 64, 128), u32), V((M1, 64, 128), u32),
        *[V((2, S, 128), bf16)] * NT, V((NT, S, 128), bf16),
        V((NT + 1, NT, 128, 128), u32),
        V((NT + 1, S // 2, 128), u32),
        V((3, 16 * M1, 128), f32), V((3, 16 * M1, 128), f32),
        V((3, 8 * M1, 128), f32),
        V((NT, 5, 8, 128), f32),
        V((NT + 1, M1, 128, 128), bf16), V((NT + 1, M1, 128, 128), bf16),
        *[V((1, M1 + 1, 128, 128), f32)] * NT,
        *[V((NT + 1, 128 * n, 128), bf16) for n in (2, 4, 6, 4)],
        V((NG + 1, S // 2, 128), u32),
        V((16, D, 128), bf16), V((16, D, 128), bf16),
        V((16, D, 128), f32), V((17, D, 128), bf16),
        *[V((NT + 1, SEG // 2, 128), u32)] * 4,
        *[V((1, 4, 128 * j + 136, 128), f32) for j in range(4)] * 2,
        V((NG, 88, 128), f32),
        V((4 * NG, 8, 128), f32),
        V((3, 64, 128), f32),
        V((4, 16, 128), u32),
        V((192, 128), f32),
        V((4, D), bf16), V((D,), bf16), V((4 * NG,), bf16),
        pltpu.SMEM((3,), i32),
        pltpu.SemaphoreType.DMA((40,)),
    ]
    out = pl.pallas_call(
        _kernel,
        out_shape=jax.ShapeDtypeStruct((S, 2 * D), bf16),
        in_specs=[hbm] * 14,
        out_specs=hbm,
        scratch_shapes=scratch,
        compiler_params=pltpu.CompilerParams(vmem_limit_bytes=110 * 2**20),
    )(
        A_q.reshape(S, D), A_k.reshape(S, D), A_v.reshape(S, D), A_shift_k.T, A_ssm_k, A_ssm_D,
        B_x.reshape(S, D), B_wq, B_wk, B_wv, B_wo, B_beta, _G_FWD, _G_INV,
    )
    return out.reshape(1, S, 2 * D)
```
